```python
import jax
import jax.numpy as jnp

def _softmax(x, axis=-1):
    return jax.nn.softmax(x, axis=axis)

def _gelu(x):
    return jax.nn.gelu(x, approximate=True)

def _silu(x):
    return jax.nn.silu(x)

def _sigmoid(x):
    return jax.nn.sigmoid(x)

def _layernorm(x, axis=-1, eps=1e-05):
    m = jnp.mean(x, axis=axis, keepdims=True)
    v = jnp.var(x, axis=axis, keepdims=True)
    return (x - m) / jnp.sqrt(v + eps)

def _scatter_add(tgt, idx, src, axis=0):
    return tgt.at[idx].add(src)

def _segment_sum(src, seg, n):
    return jax.ops.segment_sum(src, seg, n)

class _Rng:

    def __init__(self, key):
        self._k = key

    def _next(self):
        self._k, sub = jax.random.split(self._k)
        return sub

    def normal(self, shape):
        return jax.random.normal(self._next(), shape, dtype=jnp.bfloat16)

    def randint(self, lo, hi, shape):
        return jax.random.randint(self._next(), shape, lo, hi, dtype=jnp.int32)

    def uniform(self, shape, lo=0.0, hi=1.0):
        return jax.random.uniform(self._next(), shape, jnp.bfloat16, lo, hi)

    def permutation(self, n):
        return jax.random.permutation(self._next(), n)
kernel_name = 'interleave_layers__memory_aug_recurrent_mem_tr__mixer_s_mlp__prompt'

def setup_inputs():
    _rng = _Rng(jax.random.key(int.from_bytes(__import__("os").urandom(4), "little")))
    _w = lambda a: (lambda t: t.astype(jnp.bfloat16) if jnp.issubdtype(t.dtype, jnp.floating) else t)(jnp.asarray(a))

    def _A_setup():
        B, S, Dm = (1, 2048, 640)
        H, Dh = (32, 192)
        M, seg = (8, 32)
        seg = min(seg, S)
        S = S // seg * seg
        return {'x': _w((lambda *s: _rng.normal(s) * 0.05)(B, S, Dm)), 'mem0': _w((lambda *s: _rng.normal(s) * 0.05)(B, M, Dm)), 'Wq': _w((lambda *s: _rng.normal(s) * 0.05)(Dm, H, Dh) * Dm ** (-0.5)), 'Wk': _w((lambda *s: _rng.normal(s) * 0.05)(Dm, H, Dh) * Dm ** (-0.5)), 'Wv': _w((lambda *s: _rng.normal(s) * 0.05)(Dm, H, Dh) * Dm ** (-0.5)), 'Wo': _w((lambda *s: _rng.normal(s) * 0.05)(H, Dh, Dm) * (H * Dh) ** (-0.5)), 'seg_len': seg}
    _A_in = _A_setup()

    def _B_setup():
        B, S, D, F = (1, 2048, 640, 1536)
        return {'x': _w((lambda *s: _rng.normal(s) * 0.05)(B, S, D)), 'w1': _w((lambda *s: _rng.normal(s) * 0.05)(D, D) * D ** (-0.5)), 'w2': _w((lambda *s: _rng.normal(s) * 0.05)(D, D) * D ** (-0.5)), 'w3': _w((lambda *s: _rng.normal(s) * 0.05)(D, F) * D ** (-0.5)), 'w4': _w((lambda *s: _rng.normal(s) * 0.05)(F, D) * F ** (-0.5))}
    _B_in = _B_setup()
    return {'A_x': _A_in['x'], 'A_mem0': _A_in['mem0'], 'A_Wq': _A_in['Wq'], 'A_Wk': _A_in['Wk'], 'A_Wv': _A_in['Wv'], 'A_Wo': _A_in['Wo'], 'A_seg_len': _A_in['seg_len'], 'B_x': _B_in['x'], 'B_w1': _B_in['w1'], 'B_w2': _B_in['w2'], 'B_w3': _B_in['w3'], 'B_w4': _B_in['w4']}

def reference(A_x, A_mem0, A_Wq, A_Wk, A_Wv, A_Wo, A_seg_len, B_x, B_w1, B_w2, B_w3, B_w4):

    def _A_ref(x, mem0, Wq, Wk, Wv, Wo, seg_len):
        B, S, Dm = x.shape
        H, Dh = (Wq.shape[1], Wq.shape[2])
        M = mem0.shape[1]
        scale = Dh ** (-0.5)
        n_seg = S // seg_len
        L = M + seg_len
        idx = jnp.arange(L)
        mask = (idx[:, None] < M) | (idx[:, None] >= idx[None, :])
        mem = mem0
        outs = []
        for s in range(n_seg):
            xs = x[:, s * seg_len:(s + 1) * seg_len, :].copy()
            h = jnp.concatenate([mem, xs], axis=1)
            q = jnp.einsum('btd,dhe->bhte', h, Wq)
            k = jnp.einsum('btd,dhe->bhte', h, Wk)
            v = jnp.einsum('btd,dhe->bhte', h, Wv)
            scores = jnp.einsum('bhqe,bhke->bhqk', q, k) * scale
            scores = jnp.where(mask[None, None], scores, -1000000000.0)
            p = _softmax(scores, axis=-1)
            o = jnp.einsum('bhqk,bhke->bhqe', p, v)
            o = jnp.einsum('bhte,hed->btd', o, Wo)
            mem = o[:, :M, :].copy()
            outs.append(o[:, M:, :])
        return jnp.concatenate(outs, axis=1)

    def _B_ref(x, w1, w2, w3, w4):
        B, S, D = x.shape
        h = _gelu(_layernorm(x, axis=-1) @ w1)
        c = D // 4
        g0 = jnp.pad(h[:, :, 0 * c:1 * c], ((0, 0), (1, 0), (0, 0)))[:, :S, :]
        g1 = jnp.pad(h[:, :, 1 * c:2 * c], ((0, 0), (0, 1), (0, 0)))[:, 1:, :]
        g2 = jnp.pad(h[:, :, 2 * c:3 * c], ((0, 0), (2, 0), (0, 0)))[:, :S, :]
        g3 = jnp.pad(h[:, :, 3 * c:], ((0, 0), (0, 2), (0, 0)))[:, 2:, :]
        hs = jnp.concatenate([g0, g1, g2, g3], axis=-1) @ w2
        x1 = x + hs
        h2 = _gelu(_layernorm(x1, axis=-1) @ w3) @ w4
        return x1 + h2
    x = A_x
    x = x + _A_ref(_layernorm(x, axis=-1), A_mem0, A_Wq, A_Wk, A_Wv, A_Wo, A_seg_len)
    x = x + _B_ref(_layernorm(x, axis=-1), B_w1, B_w2, B_w3, B_w4)
    x = x + _A_ref(_layernorm(x, axis=-1), A_mem0, A_Wq, A_Wk, A_Wv, A_Wo, A_seg_len)
    x = x + _B_ref(_layernorm(x, axis=-1), B_w1, B_w2, B_w3, B_w4)
    return x
```

```python
import functools

import jax
import jax.numpy as jnp
from jax import lax
import jax.experimental.pallas as pl
import jax.experimental.pallas.tpu as pltpu

_SEG = 32
_MEM = 8
_LAG = 3
_NEG = -1000000000.0
_EPS = 1e-05

_F32 = jnp.float32
_BF16 = jnp.bfloat16

_NT = (((1,), (1,)), ((), ()))
_NN = (((1,), (0,)), ((), ()))


def _dot(a, b, dims=_NN):
    return lax.dot_general(a, b, dims, preferred_element_type=_F32)


def _ln(x):
    m = jnp.mean(x, axis=-1, keepdims=True)
    d = x - m
    v = jnp.mean(d * d, axis=-1, keepdims=True)
    return d * lax.rsqrt(v + _EPS)


def _gelu(x):
    return jax.nn.gelu(x, approximate=True)


def _attend(q, k, v, consts, scale):
    lo, seg0, allowed = consts
    zero = jnp.zeros_like(k)
    kb = jnp.concatenate([jnp.where(lo, k, zero), jnp.where(lo, zero, k)], axis=0).astype(_BF16)
    s = _dot(q, kb, _NT) * scale
    s = jnp.where(allowed, s, _NEG)
    m0 = jnp.max(jnp.where(seg0, s, -jnp.inf), axis=1, keepdims=True)
    m1 = jnp.max(jnp.where(seg0, -jnp.inf, s), axis=1, keepdims=True)
    p = jnp.exp(s - jnp.where(seg0, m0, m1))
    l0 = jnp.sum(jnp.where(seg0, p, 0.0), axis=1, keepdims=True)
    l1 = jnp.sum(jnp.where(seg0, 0.0, p), axis=1, keepdims=True)
    p = p / jnp.where(seg0, l0, l1)
    vb = jnp.concatenate([jnp.where(lo, v, zero), jnp.where(lo, zero, v)], axis=0).astype(_BF16)
    return _dot(p, vb)


def _kernel(x_ref, mem0_ref, wqt_ref, wkt_ref, wvt_ref, wo_ref,
            w1_ref, w2_ref, w3_ref, w4_ref, o_ref,
            ha_ref, acc_ref, ycur_ref, yprev_ref, nprev_ref, hprev_ref,
            htail_ref, y2res_ref, *, n_seg, n_heads, d_head):
    D = x_ref.shape[1]
    PW = 2 * d_head
    n_pairs = n_heads // 2
    scale = d_head ** -0.5
    L = _MEM + _SEG
    C = D // 4

    def xseg(s):
        return x_ref[pl.ds(pl.multiple_of(s * _SEG, _SEG), _SEG), :].astype(_F32)

    mem0 = mem0_ref[...]
    ha_ref[...] = jnp.zeros(ha_ref.shape, _BF16)
    ha_ref[0:2 * _MEM, :] = jnp.concatenate([mem0, mem0], axis=0).astype(_BF16)
    ha_ref[2 * _MEM:2 * _MEM + _SEG, :] = _ln(xseg(0)).astype(_BF16)
    for r in (ycur_ref, yprev_ref, nprev_ref, hprev_ref, htail_ref, y2res_ref):
        r[...] = jnp.zeros(r.shape, _F32)

    def step(t, carry):
        lo = lax.broadcasted_iota(jnp.int32, (L, PW), 1) < d_head
        lane = lax.broadcasted_iota(jnp.int32, (L, 2 * L), 1)
        row = lax.broadcasted_iota(jnp.int32, (L, 2 * L), 0)
        seg0 = lane < L
        key = jnp.where(seg0, lane, lane - L)
        allowed = (row < _MEM) | (row >= key)
        consts = (lo, seg0, allowed)

        ycur = ycur_ref[...]
        ncur = _ln(ycur)
        hcur = _gelu(_dot(_ln(ncur).astype(_BF16), w1_ref[...]))

        hprev = hprev_ref[...]
        htail = htail_ref[...]
        col = lax.broadcasted_iota(jnp.int32, (_SEG, D), 1)
        shifted = []
        for c, s in ((0, t - 2), (1, t - 2 - _LAG)):
            pt = jnp.where(s == 0, 0.0, htail[8 * c:8 * c + 8])
            nh = jnp.where(s == n_seg - 1, 0.0, hcur[_SEG * c:_SEG * c + 8])
            win = jnp.concatenate([pt, hprev[_SEG * c:_SEG * (c + 1)], nh], axis=0)
            g = jnp.where(col < C, win[7:7 + _SEG],
                          jnp.where(col < 2 * C, win[9:9 + _SEG],
                                    jnp.where(col < 3 * C, win[6:6 + _SEG], win[10:10 + _SEG])))
            shifted.append(g)
        hs = _dot(jnp.concatenate(shifted, axis=0).astype(_BF16), w2_ref[...])
        x1 = nprev_ref[...] + hs
        h2 = _dot(_gelu(_dot(_ln(x1).astype(_BF16), w3_ref[...])).astype(_BF16), w4_ref[...])
        ynew = yprev_ref[...] + x1 + h2
        so = jnp.maximum(t - 2 - _LAG, 0)
        o_ref[pl.ds(pl.multiple_of(so * _SEG, _SEG), _SEG), :] = ynew[_SEG:].astype(o_ref.dtype)
        y2new = ynew[:_SEG]
        tok2_next = _ln(y2new).astype(_BF16)
        tok1_next = _ln(xseg(jnp.minimum(t + 1, n_seg - 1))).astype(_BF16)

        htail_ref[...] = jnp.concatenate([hprev[_SEG - 8:_SEG], hprev[2 * _SEG - 8:]], axis=0)
        hprev_ref[...] = hcur
        nprev_ref[...] = ncur
        yprev_ref[...] = ycur

        acc = None
        for p in range(n_pairs):
            hb = ha_ref[...]
            q = _dot(hb, wqt_ref[p * PW:(p + 1) * PW, :], _NT)
            k = _dot(hb, wkt_ref[p * PW:(p + 1) * PW, :], _NT)
            v = _dot(hb, wvt_ref[p * PW:(p + 1) * PW, :], _NT)
            outs = []
            for c in (0, 1):
                def rows(a):
                    return jnp.concatenate(
                        [a[_MEM * c:_MEM * (c + 1)],
                         a[2 * _MEM + _SEG * c:2 * _MEM + _SEG * (c + 1)]], axis=0)
                outs.append(_attend(rows(q), rows(k), rows(v), consts, scale))
            o = jnp.concatenate([outs[0][:_MEM], outs[1][:_MEM], outs[0][_MEM:], outs[1][_MEM:]],
                                axis=0).astype(_BF16)
            part = _dot(o, wo_ref[p * PW:(p + 1) * PW, :])
            if p == 0:
                acc_ref[...] = part
            elif p < n_pairs - 1:
                acc_ref[...] += part
            else:
                acc = acc_ref[...] + part

        mem1 = acc[0:_MEM]
        mem2 = jnp.where(t + 1 <= _LAG, mem0_ref[...].astype(_F32), acc[_MEM:2 * _MEM])
        ha_ref[0:2 * _MEM, :] = jnp.concatenate([mem1, mem2], axis=0).astype(_BF16)
        ha_ref[2 * _MEM:2 * _MEM + _SEG, :] = tok1_next
        ha_ref[2 * _MEM + _SEG:, :] = tok2_next
        y1 = xseg(jnp.minimum(t, n_seg - 1)) + acc[2 * _MEM:2 * _MEM + _SEG]
        y3 = y2res_ref[...] + acc[2 * _MEM + _SEG:]
        ycur_ref[0:_SEG, :] = y1
        ycur_ref[_SEG:, :] = y3
        y2res_ref[...] = y2new
        return carry

    lax.fori_loop(0, n_seg + _LAG + 2, step, 0)


@functools.partial(jax.jit, static_argnames=("A_seg_len",))
def pallas_interleave_layers__memory_aug_recurrent_mem_tr__mixer_s_mlp__prompt_kernel(
    A_x: jax.Array,
    A_mem0: jax.Array,
    A_Wq: jax.Array,
    A_Wk: jax.Array,
    A_Wv: jax.Array,
    A_Wo: jax.Array,
    A_seg_len,
    B_x: jax.Array,
    B_w1: jax.Array,
    B_w2: jax.Array,
    B_w3: jax.Array,
    B_w4: jax.Array,
):
    del B_x
    _, S, D = A_x.shape
    _, H, Dh = A_Wq.shape
    assert A_seg_len == _SEG and A_mem0.shape[1] == _MEM and A_x.shape[0] == 1
    n_seg = S // _SEG

    def wt(w):
        return jnp.transpose(w, (1, 2, 0)).reshape(H * Dh, D)

    R = 2 * (_MEM + _SEG)
    out = pl.pallas_call(
        functools.partial(_kernel, n_seg=n_seg, n_heads=H, d_head=Dh),
        out_shape=jax.ShapeDtypeStruct((S, D), A_x.dtype),
        scratch_shapes=[
            pltpu.VMEM((R, D), _BF16),
            pltpu.VMEM((R, D), _F32),
            pltpu.VMEM((2 * _SEG, D), _F32),
            pltpu.VMEM((2 * _SEG, D), _F32),
            pltpu.VMEM((2 * _SEG, D), _F32),
            pltpu.VMEM((2 * _SEG, D), _F32),
            pltpu.VMEM((16, D), _F32),
            pltpu.VMEM((_SEG, D), _F32),
        ],
        compiler_params=pltpu.CompilerParams(vmem_limit_bytes=100 * 1024 * 1024),
    )(A_x.reshape(S, D), A_mem0.reshape(_MEM, D), wt(A_Wq), wt(A_Wk), wt(A_Wv),
      A_Wo.reshape(H * Dh, D), B_w1, B_w2, B_w3, B_w4)
    return out.reshape(1, S, D)
```

```python
import functools

import jax
import jax.numpy as jnp
from jax import lax
import jax.experimental.pallas as pl
import jax.experimental.pallas.tpu as pltpu

_SEG = 32
_MEM = 8
_LAG = 3
_NEG = -1000000000.0
_EPS = 1e-05

_F32 = jnp.float32
_BF16 = jnp.bfloat16

_NT = (((1,), (1,)), ((), ()))
_NN = (((1,), (0,)), ((), ()))


def _dot(a, b, dims=_NN):
    return lax.dot_general(a, b, dims, preferred_element_type=_F32)


def _ln(x):
    m = jnp.mean(x, axis=-1, keepdims=True)
    d = x - m
    v = jnp.mean(d * d, axis=-1, keepdims=True)
    return d * lax.rsqrt(v + _EPS)


def _gelu(x):
    return jax.nn.gelu(x, approximate=True)


def _kernel(x_ref, mem0_ref, wqt_ref, wkt_ref, wvt_ref, wo_ref,
            w1_ref, w2_ref, w3_ref, w4_ref, o_ref,
            ha_ref, acc_ref, ycur_ref, yprev_ref, nprev_ref, hprev_ref,
            htail_ref, y2res_ref, *, n_seg, n_heads, d_head, sched):
    D = x_ref.shape[1]
    PW = 2 * d_head
    n_pairs = n_heads // 2
    scale = d_head ** -0.5
    L = _MEM + _SEG
    C = D // 4

    def xseg(s):
        return x_ref[pl.ds(pl.multiple_of(s * _SEG, _SEG), _SEG), :].astype(_F32)

    mem0 = mem0_ref[...]
    ha_ref[...] = jnp.zeros(ha_ref.shape, _BF16)
    ha_ref[0:2 * _MEM, :] = jnp.concatenate([mem0, mem0], axis=0).astype(_BF16)
    ha_ref[2 * _MEM:2 * _MEM + _SEG, :] = _ln(xseg(0)).astype(_BF16)
    for r in (ycur_ref, yprev_ref, nprev_ref, hprev_ref, htail_ref, y2res_ref):
        r[...] = jnp.zeros(r.shape, _F32)

    def step(t, carry):
        lo = lax.broadcasted_iota(jnp.int32, (L, PW), 1) < d_head
        lane = lax.broadcasted_iota(jnp.int32, (L, 2 * L), 1)
        row = lax.broadcasted_iota(jnp.int32, (L, 2 * L), 0)
        seg0 = lane < L
        key = jnp.where(seg0, lane, lane - L)
        allowed = (row < _MEM) | (row >= key)
        col = lax.broadcasted_iota(jnp.int32, (_SEG, D), 1)

        st = {}

        def rows(a, c):
            return jnp.concatenate(
                [a[_MEM * c:_MEM * (c + 1)],
                 a[2 * _MEM + _SEG * c:2 * _MEM + _SEG * (c + 1)]], axis=0)

        def blockdiag(a):
            zero = jnp.zeros_like(a)
            return jnp.concatenate([jnp.where(lo, a, zero), jnp.where(lo, zero, a)],
                                   axis=0).astype(_BF16)

        def a_q(p):
            st["q", p] = _dot(ha_ref[...], wqt_ref[p * PW:(p + 1) * PW, :], _NT)

        def a_k(p):
            st["k", p] = _dot(ha_ref[...], wkt_ref[p * PW:(p + 1) * PW, :], _NT)

        def a_v(p):
            st["v", p] = _dot(ha_ref[...], wvt_ref[p * PW:(p + 1) * PW, :], _NT)

        def a_s(p):
            q, k = st.pop(("q", p)), st.pop(("k", p))
            for c in (0, 1):
                s = _dot(rows(q, c), blockdiag(rows(k, c)), _NT) * scale
                s = jnp.where(allowed, s, _NEG)
                m0 = jnp.max(jnp.where(seg0, s, -jnp.inf), axis=1, keepdims=True)
                m1 = jnp.max(jnp.where(seg0, -jnp.inf, s), axis=1, keepdims=True)
                e = jnp.exp(s - jnp.where(seg0, m0, m1))
                l0 = jnp.sum(jnp.where(seg0, e, 0.0), axis=1, keepdims=True)
                l1 = jnp.sum(jnp.where(seg0, 0.0, e), axis=1, keepdims=True)
                st["p", p, c] = e / jnp.where(seg0, l0, l1)

        def a_pv(p):
            v = st.pop(("v", p))
            outs = [_dot(st.pop(("p", p, c)), blockdiag(rows(v, c))) for c in (0, 1)]
            st["o", p] = jnp.concatenate(
                [outs[0][:_MEM], outs[1][:_MEM], outs[0][_MEM:], outs[1][_MEM:]],
                axis=0).astype(_BF16)

        def a_o(p):
            part = _dot(st.pop(("o", p)), wo_ref[p * PW:(p + 1) * PW, :])
            if p == 0:
                acc_ref[...] = part
            elif p < n_pairs - 1:
                acc_ref[...] += part
            else:
                st["acc"] = acc_ref[...] + part

        def rs(c):
            return slice(_SEG * c, _SEG * (c + 1))

        def b_1(c):
            ycur = ycur_ref[rs(c), :]
            ncur = _ln(ycur)
            st["ycur", c], st["ncur", c] = ycur, ncur
            st["h", c] = _gelu(_dot(_ln(ncur).astype(_BF16), w1_ref[...]))

        def b_2(c):
            s = t - 2 - _LAG * c
            hprev = hprev_ref[rs(c), :]
            hcur = st.pop(("h", c))
            pt = jnp.where(s == 0, 0.0, htail_ref[8 * c:8 * c + 8, :])
            nh = jnp.where(s == n_seg - 1, 0.0, hcur[0:8])
            win = jnp.concatenate([pt, hprev, nh], axis=0)
            g = jnp.where(col < C, win[7:7 + _SEG],
                          jnp.where(col < 2 * C, win[9:9 + _SEG],
                                    jnp.where(col < 3 * C, win[6:6 + _SEG], win[10:10 + _SEG])))
            htail_ref[8 * c:8 * c + 8, :] = hprev[_SEG - 8:]
            hprev_ref[rs(c), :] = hcur
            st["x1", c] = nprev_ref[rs(c), :] + _dot(g.astype(_BF16), w2_ref[...])
            nprev_ref[rs(c), :] = st.pop(("ncur", c))

        def b_3(c):
            st["f", c] = _gelu(_dot(_ln(st["x1", c]).astype(_BF16), w3_ref[...])).astype(_BF16)

        def b_4(c):
            ynew = yprev_ref[rs(c), :] + st.pop(("x1", c)) + _dot(st.pop(("f", c)), w4_ref[...])
            yprev_ref[rs(c), :] = st.pop(("ycur", c))
            if c == 0:
                st["y2new"] = ynew
                st["tok2"] = _ln(ynew).astype(_BF16)
            else:
                so = jnp.maximum(t - 2 - _LAG, 0)
                o_ref[pl.ds(pl.multiple_of(so * _SEG, _SEG), _SEG), :] = ynew.astype(o_ref.dtype)

        stages = dict(q=a_q, k=a_k, v=a_v, s=a_s, pv=a_pv, o=a_o, b1=b_1, b2=b_2, b3=b_3, b4=b_4)
        for name, arg in sched:
            stages[name](arg)

        acc = st.pop("acc")
        mem1 = acc[0:_MEM]
        mem2 = jnp.where(t + 1 <= _LAG, mem0_ref[...].astype(_F32), acc[_MEM:2 * _MEM])
        ha_ref[0:2 * _MEM, :] = jnp.concatenate([mem1, mem2], axis=0).astype(_BF16)
        ha_ref[2 * _MEM:2 * _MEM + _SEG, :] = _ln(xseg(jnp.minimum(t + 1, n_seg - 1))).astype(_BF16)
        ha_ref[2 * _MEM + _SEG:, :] = st.pop("tok2")
        ycur_ref[0:_SEG, :] = xseg(jnp.minimum(t, n_seg - 1)) + acc[2 * _MEM:2 * _MEM + _SEG]
        ycur_ref[_SEG:, :] = y2res_ref[...] + acc[2 * _MEM + _SEG:]
        y2res_ref[...] = st.pop("y2new")
        return carry

    lax.fori_loop(0, n_seg + _LAG + 2, step, 0)


def _schedule(n_pairs):
    extra = {1: [("b1", 0)], 3: [("b2", 0)], 5: [("b3", 0)], 7: [("b4", 0)],
             9: [("b1", 1)], 11: [("b2", 1)], n_pairs: [("b3", 1)], n_pairs + 1: [("b4", 1)]}
    sched = []
    for i in range(n_pairs + 3):
        if i < n_pairs:
            sched += [("q", i), ("k", i)]
        if 0 <= i - 1 < n_pairs:
            sched.append(("s", i - 1))
        if i < n_pairs:
            sched.append(("v", i))
        sched += extra.get(i, [])
        if 0 <= i - 2 < n_pairs:
            sched.append(("pv", i - 2))
        if 0 <= i - 3 < n_pairs:
            sched.append(("o", i - 3))
    return tuple(sched)


@functools.partial(jax.jit, static_argnames=("A_seg_len",))
def pallas_interleave_layers__memory_aug_recurrent_mem_tr__mixer_s_mlp__prompt_kernel(
    A_x: jax.Array,
    A_mem0: jax.Array,
    A_Wq: jax.Array,
    A_Wk: jax.Array,
    A_Wv: jax.Array,
    A_Wo: jax.Array,
    A_seg_len,
    B_x: jax.Array,
    B_w1: jax.Array,
    B_w2: jax.Array,
    B_w3: jax.Array,
    B_w4: jax.Array,
):
    del B_x
    _, S, D = A_x.shape
    _, H, Dh = A_Wq.shape
    assert A_seg_len == _SEG and A_mem0.shape[1] == _MEM and A_x.shape[0] == 1
    n_seg = S // _SEG

    def wt(w):
        return jnp.transpose(w, (1, 2, 0)).reshape(H * Dh, D)

    R = 2 * (_MEM + _SEG)
    out = pl.pallas_call(
        functools.partial(_kernel, n_seg=n_seg, n_heads=H, d_head=Dh,
                          sched=_schedule(H // 2)),
        out_shape=jax.ShapeDtypeStruct((S, D), A_x.dtype),
        scratch_shapes=[
            pltpu.VMEM((R, D), _BF16),
            pltpu.VMEM((R, D), _F32),
            pltpu.VMEM((2 * _SEG, D), _F32),
            pltpu.VMEM((2 * _SEG, D), _F32),
            pltpu.VMEM((2 * _SEG, D), _F32),
            pltpu.VMEM((2 * _SEG, D), _F32),
            pltpu.VMEM((16, D), _F32),
            pltpu.VMEM((_SEG, D), _F32),
        ],
        compiler_params=pltpu.CompilerParams(vmem_limit_bytes=100 * 1024 * 1024),
    )(A_x.reshape(S, D), A_mem0.reshape(_MEM, D), wt(A_Wq), wt(A_Wk), wt(A_Wv),
      A_Wo.reshape(H * Dh, D), B_w1, B_w2, B_w3, B_w4)
    return out.reshape(1, S, D)
```

```python
import functools

import jax
import jax.numpy as jnp
from jax import lax
import jax.experimental.pallas as pl
import jax.experimental.pallas.tpu as pltpu

_SEG = 32
_MEM = 8
_LAG = 3
_NSTAGE = 3
_NEG = -1000000000.0
_EPS = 1e-05

_F32 = jnp.float32
_BF16 = jnp.bfloat16

_NT = (((1,), (1,)), ((), ()))
_NN = (((1,), (0,)), ((), ()))


def _dot(a, b, dims=_NN):
    return lax.dot_general(a, b, dims, preferred_element_type=_F32)


def _ln(x):
    m = jnp.mean(x, axis=-1, keepdims=True)
    d = x - m
    v = jnp.mean(d * d, axis=-1, keepdims=True)
    return d * lax.rsqrt(v + _EPS)


def _gelu(x):
    return jax.nn.gelu(x, approximate=True)


def _schedule(n_pairs, a_chains, b_stages):
    slots = {("b1", 0): 1, ("b2", 0): 3, ("b3", 0): 5, ("b4", 0): 7,
             ("b1", 1): 9, ("b2", 1): 11, ("b3", 1): n_pairs, ("b4", 1): n_pairs + 1}
    b_list = [(n, c) for c in (0, 1) for n in ("b1", "b2", "b3", "b4") if (n, c) in b_stages]
    if not a_chains:
        return tuple(b_list)
    sched = []
    for i in range(n_pairs + 3):
        if i < n_pairs:
            sched += [("q", i), ("k", i)]
        if 0 <= i - 1 < n_pairs:
            sched.append(("s", i - 1))
        if i < n_pairs:
            sched.append(("v", i))
        sched += [b for b in b_list if slots[b] == i]
        if 0 <= i - 2 < n_pairs:
            sched.append(("pv", i - 2))
        if 0 <= i - 3 < n_pairs:
            sched.append(("o", i - 3))
    return tuple(sched)


def _kernel(x_hbm, mem0_hbm, wqt_hbm, wkt_hbm, wvt_hbm, wo_hbm,
            w1_hbm, w2_hbm, w3_hbm, w4_hbm, o_hbm,
            x_ref, mem0_ref, wq_ref, wk_ref, wv_ref, wo_ref,
            w1_ref, w2_ref, w3_ref, w4_ref, o_ref, stage_ref,
            ha_ref, acc_ref, ycur_ref, yprev_ref, nprev_ref, hprev_ref,
            htail_ref, y2res_ref, sems, *, n_seg, n_heads, d_head):
    S, D = x_ref.shape
    PW = 2 * d_head
    n_pairs = n_heads // 2
    scale = d_head ** -0.5
    L = _MEM + _SEG
    C = D // 4
    X0 = 4 * _SEG

    def pair_in(p, j):
        rows = pl.ds(p * PW, PW)
        sem = sems.at[4 * p + j]
        if j < 3:
            src = (wqt_hbm, wkt_hbm, wvt_hbm)[j]
            return pltpu.make_async_copy(src.at[rows, :], stage_ref.at[p % _NSTAGE, j], sem)
        return pltpu.make_async_copy(wo_hbm.at[rows, :], wo_ref.at[rows, :], sem)

    nb = 4 * n_pairs
    misc = dict(
        x0=pltpu.make_async_copy(x_hbm.at[pl.ds(0, X0), :], x_ref.at[pl.ds(0, X0), :], sems.at[nb]),
        x1=pltpu.make_async_copy(x_hbm.at[pl.ds(X0, S - X0), :], x_ref.at[pl.ds(X0, S - X0), :],
                                 sems.at[nb + 1]),
        mem0=pltpu.make_async_copy(mem0_hbm, mem0_ref, sems.at[nb + 2]),
        w1=pltpu.make_async_copy(w1_hbm, w1_ref, sems.at[nb + 3]),
        w2=pltpu.make_async_copy(w2_hbm, w2_ref, sems.at[nb + 4]),
        w3=pltpu.make_async_copy(w3_hbm, w3_ref, sems.at[nb + 5]),
        w4=pltpu.make_async_copy(w4_hbm, w4_ref, sems.at[nb + 6]),
    )
    n_early = (n_seg - _LAG - 2) * _SEG
    out_a = pltpu.make_async_copy(o_ref.at[pl.ds(0, n_early), :], o_hbm.at[pl.ds(0, n_early), :],
                                  sems.at[nb + 7])
    out_b = pltpu.make_async_copy(o_ref.at[pl.ds(n_early, S - n_early), :],
                                  o_hbm.at[pl.ds(n_early, S - n_early), :], sems.at[nb + 8])

    def xseg(s):
        if isinstance(s, int):
            return x_ref[s * _SEG:(s + 1) * _SEG, :].astype(_F32)
        return x_ref[pl.ds(pl.multiple_of(s * _SEG, _SEG), _SEG), :].astype(_F32)

    def pick(cond, a, b):
        if isinstance(cond, bool):
            return a if cond else b()
        return jnp.where(cond, a, b())

    T1 = slice(2 * _MEM, 2 * _MEM + _SEG)
    T2 = slice(2 * _MEM + _SEG, 2 * _MEM + 2 * _SEG)

    def step(t, a_chains, b_stages, first=False):
        both = len(a_chains) == 2
        lo = lax.broadcasted_iota(jnp.int32, (L, PW), 1) < d_head
        lane = lax.broadcasted_iota(jnp.int32, (L, 2 * L), 1)
        row = lax.broadcasted_iota(jnp.int32, (L, 2 * L), 0)
        seg0 = lane < L
        key = jnp.where(seg0, lane, lane - L)
        allowed = (row < _MEM) | (row >= key)
        col = lax.broadcasted_iota(jnp.int32, (_SEG, D), 1)

        st = {}

        def rows(a, c):
            if not both:
                return a
            return jnp.concatenate(
                [a[_MEM * c:_MEM * (c + 1)], a[2 * _MEM + _SEG * c:2 * _MEM + _SEG * (c + 1)]], axis=0)

        def blockdiag(a):
            zero = jnp.zeros_like(a)
            return jnp.concatenate([jnp.where(lo, a, zero), jnp.where(lo, zero, a)],
                                   axis=0).astype(_BF16)

        if len(a_chains) == 1:
            c0 = a_chains[0]
            hload = lambda: jnp.concatenate(
                [ha_ref[_MEM * c0:_MEM * (c0 + 1), :].astype(_F32),
                 ha_ref[(T1, T2)[c0], :].astype(_F32)], axis=0)
            h32 = hload()
            lhs = lambda: h32
        else:
            lhs = lambda: ha_ref[...]

        def proj(p, j):
            w_ref = (wq_ref, wk_ref, wv_ref)[j]
            if first:
                if j == 0:
                    if p + 2 < n_pairs:
                        for jj in range(4):
                            pair_in(p + 2, jj).start()
                pair_in(p, j).wait()
                w_ref[p] = stage_ref[p % _NSTAGE, j].T
            return _dot(lhs(), w_ref[p])

        def a_q(p):
            st["q", p] = proj(p, 0)

        def a_k(p):
            st["k", p] = proj(p, 1)

        def a_v(p):
            st["v", p] = proj(p, 2)

        def a_s(p):
            q, k = st.pop(("q", p)), st.pop(("k", p))
            for c in a_chains:
                s = _dot(rows(q, c), blockdiag(rows(k, c)), _NT) * scale
                s = jnp.where(allowed, s, _NEG)
                m0 = jnp.max(jnp.where(seg0, s, -jnp.inf), axis=1, keepdims=True)
                m1 = jnp.max(jnp.where(seg0, -jnp.inf, s), axis=1, keepdims=True)
                e = jnp.exp(s - jnp.where(seg0, m0, m1))
                l0 = jnp.sum(jnp.where(seg0, e, 0.0), axis=1, keepdims=True)
                l1 = jnp.sum(jnp.where(seg0, 0.0, e), axis=1, keepdims=True)
                st["p", p, c] = e / jnp.where(seg0, l0, l1)

        def a_pv(p):
            v = st.pop(("v", p))
            outs = [_dot(st.pop(("p", p, c)), blockdiag(rows(v, c))) for c in a_chains]
            if both:
                st["o", p] = jnp.concatenate(
                    [outs[0][:_MEM], outs[1][:_MEM], outs[0][_MEM:], outs[1][_MEM:]],
                    axis=0).astype(_BF16)
            else:
                st["o", p] = outs[0]

        def a_o(p):
            if first:
                pair_in(p, 3).wait()
            part = _dot(st.pop(("o", p)), wo_ref[p * PW:(p + 1) * PW, :])
            n = part.shape[0]
            if p == 0:
                acc_ref[0:n, :] = part
            elif p < n_pairs - 1:
                acc_ref[0:n, :] += part
            else:
                st["acc"] = acc_ref[0:n, :] + part

        def rs(c):
            return slice(_SEG * c, _SEG * (c + 1))

        def rotate(c):
            htail_ref[8 * c:8 * c + 8, :] = hprev_ref[_SEG * (c + 1) - 8:_SEG * (c + 1), :]
            hprev_ref[rs(c), :] = st.pop(("h", c))
            nprev_ref[rs(c), :] = st.pop(("ncur", c))
            yprev_ref[rs(c), :] = st.pop(("ycur", c))

        def b_1(c):
            ycur = ycur_ref[rs(c), :]
            ncur = _ln(ycur)
            st["ycur", c], st["ncur", c] = ycur, ncur
            st["h", c] = _gelu(_dot(_ln(ncur).astype(_BF16), w1_ref[...]))
            if ("b2", c) not in b_stages:
                rotate(c)

        def b_2(c):
            s = t - 2 - _LAG * c
            hprev = hprev_ref[rs(c), :]
            pt = pick(s == 0, jnp.zeros((8, D), _F32), lambda: htail_ref[8 * c:8 * c + 8, :])
            nh = pick(s == n_seg - 1, jnp.zeros((8, D), _F32), lambda: st["h", c][0:8])
            win = jnp.concatenate([pt, hprev, nh], axis=0)
            g = jnp.where(col < C, win[7:7 + _SEG],
                          jnp.where(col < 2 * C, win[9:9 + _SEG],
                                    jnp.where(col < 3 * C, win[6:6 + _SEG], win[10:10 + _SEG])))
            st["x1", c] = nprev_ref[rs(c), :] + _dot(g.astype(_BF16), w2_ref[...])
            st["yres", c] = yprev_ref[rs(c), :]
            if ("b1", c) in b_stages:
                rotate(c)

        def b_3(c):
            st["f", c] = _gelu(_dot(_ln(st["x1", c]).astype(_BF16), w3_ref[...])).astype(_BF16)

        def b_4(c):
            ynew = st.pop(("yres", c)) + st.pop(("x1", c)) + _dot(st.pop(("f", c)), w4_ref[...])
            if c == 0:
                st["y2new"] = ynew
                st["tok2"] = _ln(ynew).astype(_BF16)
            else:
                so = t - 2 - _LAG
                if isinstance(so, int):
                    o_ref[so * _SEG:(so + 1) * _SEG, :] = ynew.astype(o_ref.dtype)
                else:
                    so = jnp.maximum(so, 0)
                    o_ref[pl.ds(pl.multiple_of(so * _SEG, _SEG), _SEG), :] = ynew.astype(o_ref.dtype)

        stages = dict(q=a_q, k=a_k, v=a_v, s=a_s, pv=a_pv, o=a_o, b1=b_1, b2=b_2, b3=b_3, b4=b_4)
        for name, arg in _schedule(n_pairs, a_chains, b_stages):
            stages[name](arg)

        if "tok2" in st:
            ha_ref[T2, :] = st.pop("tok2")
        if a_chains:
            acc = st.pop("acc")
            if both:
                mem1, mem2 = acc[0:_MEM], acc[_MEM:2 * _MEM]
                a1, a2 = acc[T1], acc[T2]
            elif a_chains == (0,):
                mem1, mem2 = acc[0:_MEM], mem0_ref[...].astype(_F32)
                a1, a2 = acc[_MEM:L], None
            else:
                mem1, mem2 = mem0_ref[...].astype(_F32), acc[0:_MEM]
                a1, a2 = None, acc[_MEM:L]
            ha_ref[0:2 * _MEM, :] = jnp.concatenate([mem1, mem2], axis=0).astype(_BF16)
            if a1 is not None:
                nxt = min(t + 1, n_seg - 1) if isinstance(t, int) else jnp.minimum(t + 1, n_seg - 1)
                ha_ref[T1, :] = _ln(xseg(nxt)).astype(_BF16)
                ycur_ref[0:_SEG, :] = xseg(t) + a1
            if a2 is not None:
                ycur_ref[_SEG:, :] = y2res_ref[...] + a2
        if "y2new" in st:
            y2res_ref[...] = st.pop("y2new")
        assert not st, list(st)

    misc["x0"].start()
    misc["mem0"].start()
    for p in (0, 1):
        for j in range(4):
            pair_in(p, j).start()
    for r in (ycur_ref, yprev_ref, nprev_ref, hprev_ref, htail_ref, y2res_ref):
        r[...] = jnp.zeros(r.shape, _F32)
    misc["x0"].wait()
    misc["mem0"].wait()
    mem0 = mem0_ref[...]
    ha_ref[0:2 * _MEM, :] = jnp.concatenate([mem0, mem0], axis=0).astype(_BF16)
    ha_ref[T1, :] = _ln(xseg(0)).astype(_BF16)
    ha_ref[T2, :] = jnp.zeros((_SEG, D), _BF16)

    B = lambda c, which: {(n, c) for n in which}
    ALL = ("b1", "b2", "b3", "b4")
    step(0, (0,), set(), first=True)
    for k in ("w1", "w2", "w3", "w4", "x1"):
        misc[k].start()
    misc["w1"].wait()
    step(1, (0,), B(0, ALL[:1]))
    for k in ("w2", "w3", "w4"):
        misc[k].wait()
    step(2, (0,), B(0, ALL))
    misc["x1"].wait()

    def body(t, carry):
        step(t, (0, 1), B(0, ALL) | B(1, ALL))
        return carry
    lax.fori_loop(_LAG, n_seg, body, 0)

    out_a.start()
    step(n_seg, (1,), B(0, ALL) | B(1, ALL))
    step(n_seg + 1, (1,), B(0, ALL[1:]) | B(1, ALL))
    step(n_seg + 2, (1,), B(1, ALL))
    step(n_seg + 3, (), B(1, ALL))
    step(n_seg + 4, (), B(1, ALL[1:]))
    out_b.start()
    out_a.wait()
    out_b.wait()


@functools.partial(jax.jit, static_argnames=("A_seg_len",))
def pallas_interleave_layers__memory_aug_recurrent_mem_tr__mixer_s_mlp__prompt_kernel(
    A_x: jax.Array,
    A_mem0: jax.Array,
    A_Wq: jax.Array,
    A_Wk: jax.Array,
    A_Wv: jax.Array,
    A_Wo: jax.Array,
    A_seg_len,
    B_x: jax.Array,
    B_w1: jax.Array,
    B_w2: jax.Array,
    B_w3: jax.Array,
    B_w4: jax.Array,
):
    del B_x
    _, S, D = A_x.shape
    _, H, Dh = A_Wq.shape
    F = B_w3.shape[1]
    assert A_seg_len == _SEG and A_mem0.shape[1] == _MEM and A_x.shape[0] == 1
    n_seg = S // _SEG
    assert n_seg * _SEG == S and n_seg >= 2 * _LAG + 2 and H % 2 == 0

    def wt(w):
        return jnp.transpose(w, (1, 2, 0)).reshape(H * Dh, D)

    R = 2 * (_MEM + _SEG)
    NP, PW = H // 2, 2 * Dh
    hbm = pl.BlockSpec(memory_space=pl.ANY)
    out = pl.pallas_call(
        functools.partial(_kernel, n_seg=n_seg, n_heads=H, d_head=Dh),
        out_shape=jax.ShapeDtypeStruct((S, D), A_x.dtype),
        in_specs=[hbm] * 10,
        out_specs=hbm,
        scratch_shapes=[
            pltpu.VMEM((S, D), _BF16),
            pltpu.VMEM((_MEM, D), _BF16),
            pltpu.VMEM((NP, D, PW), _BF16),
            pltpu.VMEM((NP, D, PW), _BF16),
            pltpu.VMEM((NP, D, PW), _BF16),
            pltpu.VMEM((H * Dh, D), _BF16),
            pltpu.VMEM((D, D), _BF16),
            pltpu.VMEM((D, D), _BF16),
            pltpu.VMEM((D, F), _BF16),
            pltpu.VMEM((F, D), _BF16),
            pltpu.VMEM((S, D), A_x.dtype),
            pltpu.VMEM((_NSTAGE, 3, PW, D), _BF16),
            pltpu.VMEM((R, D), _BF16),
            pltpu.VMEM((R, D), _F32),
            pltpu.VMEM((2 * _SEG, D), _F32),
            pltpu.VMEM((2 * _SEG, D), _F32),
            pltpu.VMEM((2 * _SEG, D), _F32),
            pltpu.VMEM((2 * _SEG, D), _F32),
            pltpu.VMEM((16, D), _F32),
            pltpu.VMEM((_SEG, D), _F32),
            pltpu.SemaphoreType.DMA((4 * NP + 9,)),
        ],
        compiler_params=pltpu.CompilerParams(vmem_limit_bytes=100 * 1024 * 1024),
    )(A_x.reshape(S, D), A_mem0.reshape(_MEM, D), wt(A_Wq), wt(A_Wk), wt(A_Wv),
      A_Wo.reshape(H * Dh, D), B_w1, B_w2, B_w3, B_w4)
    return out.reshape(1, S, D)
```

```python
import contextlib
import functools

import jax
import jax.numpy as jnp
from jax import lax
import jax.experimental.pallas as pl
import jax.experimental.pallas.tpu as pltpu

_SEG = 32
_MEM = 8
_LAG = 3
_AHEAD = 9
_UNROLL = 1
_NEG = -1000000000.0
_EPS = 1e-05

_F32 = jnp.float32
_BF16 = jnp.bfloat16

_NT = (((1,), (1,)), ((), ()))
_NN = (((1,), (0,)), ((), ()))


_PROFILE_SCOPES = False


def _scope(name):
    return jax.named_scope(name) if _PROFILE_SCOPES else contextlib.nullcontext()


def _dot(a, b, dims=_NN):
    return lax.dot_general(a, b, dims, preferred_element_type=_F32)


def _ln(x):
    m = jnp.mean(x, axis=-1, keepdims=True)
    d = x - m
    v = jnp.mean(d * d, axis=-1, keepdims=True)
    return d * lax.rsqrt(v + _EPS)


def _gelu(x):
    return jax.nn.gelu(x, approximate=True)


def _schedule(n_pairs, a_chains, b_stages, mode, last_in_body):
    slots = {("b1", 0): 1, ("b2", 0): 3, ("b3", 0): 5, ("b4", 0): 7,
             ("b1", 1): 9, ("b2", 1): 11, ("b3", 1): n_pairs, ("b4", 1): n_pairs + 1}
    if not last_in_body:
        slots[("b3", 1)] = n_pairs + 1
        slots[("b4", 1)] = n_pairs + 3
    b_list = [(n, c) for c in (0, 1) for n in ("b1", "b2", "b3", "b4") if (n, c) in b_stages]
    if not a_chains:
        return tuple(b_list)
    sched = []
    last = n_pairs - 1
    for i in range(n_pairs + 4):
        if i < n_pairs:
            sched += [("q", i), ("k", i)]
        if mode == "first" and i == n_pairs:
            sched.append(("bulk", 0))
        if 0 <= i - 1 < n_pairs:
            sched.append(("s", i - 1))
        if i < n_pairs:
            sched.append(("v", i))
        sched += [b for b in b_list if slots[b] == i]
        if 0 <= i - 2 < n_pairs:
            sched.append(("pv", i - 2))
        if 0 <= i - 3 < n_pairs:
            sched.append(("o", i - 3))
        if mode == "first" and i == n_pairs:
            sched.append(("bulk", 1))
        if mode == "first" and i == n_pairs + 1:
            sched.append(("bulk", 2))
    return tuple(sched)


def _kernel(x_hbm, mem0_hbm, wqt_hbm, wkt_hbm, wvt_hbm, wo_hbm,
            w1_hbm, w2_hbm, w3_hbm, w4_hbm, o_hbm,
            x_ref, mem0_ref, wq_ref, wk_ref, wv_ref, wo_ref,
            w1_ref, w2_ref, w3_ref, w4_ref, o_ref, stage_ref,
            ha_ref, h0_ref, pre_ref, acc_ref, ycur_ref, yprev_ref, nprev_ref, hprev_ref,
            htail_ref, y2res_ref, sems, *, n_seg, n_heads, d_head):
    S, D = x_ref.shape
    PW = 2 * d_head
    n_pairs = n_heads // 2
    scale = d_head ** -0.5
    L = _MEM + _SEG
    C = D // 4
    NA = _AHEAD * _SEG
    X0 = (_AHEAD + _LAG) * _SEG

    def pair_in(p, j):
        rows = pl.ds(p * PW, PW)
        sem = sems.at[4 * p + j]
        if j < 3:
            src = (wqt_hbm, wkt_hbm, wvt_hbm)[j]
            return pltpu.make_async_copy(src.at[rows, :], stage_ref.at[j, p], sem)
        return pltpu.make_async_copy(wo_hbm.at[rows, :], wo_ref.at[rows, :], sem)

    nb = 4 * n_pairs
    misc = dict(
        x0=pltpu.make_async_copy(x_hbm.at[pl.ds(0, X0), :], x_ref.at[pl.ds(0, X0), :], sems.at[nb]),
        x1=pltpu.make_async_copy(x_hbm.at[pl.ds(X0, S - X0), :], x_ref.at[pl.ds(X0, S - X0), :],
                                 sems.at[nb + 1]),
        mem0=pltpu.make_async_copy(mem0_hbm, mem0_ref, sems.at[nb + 2]),
        w1=pltpu.make_async_copy(w1_hbm, w1_ref, sems.at[nb + 3]),
        w2=pltpu.make_async_copy(w2_hbm, w2_ref, sems.at[nb + 4]),
        w3=pltpu.make_async_copy(w3_hbm, w3_ref, sems.at[nb + 5]),
        w4=pltpu.make_async_copy(w4_hbm, w4_ref, sems.at[nb + 6]),
    )
    n_early = (n_seg - _LAG - 2) * _SEG
    out_a = pltpu.make_async_copy(o_ref.at[pl.ds(0, n_early), :], o_hbm.at[pl.ds(0, n_early), :],
                                  sems.at[nb + 7])
    out_b = pltpu.make_async_copy(o_ref.at[pl.ds(n_early, S - n_early), :],
                                  o_hbm.at[pl.ds(n_early, S - n_early), :], sems.at[nb + 8])

    def xseg(s):
        if isinstance(s, int):
            return x_ref[s * _SEG:(s + 1) * _SEG, :].astype(_F32)
        return x_ref[pl.ds(pl.multiple_of(s * _SEG, _SEG), _SEG), :].astype(_F32)

    def pick(cond, a, b):
        if isinstance(cond, bool):
            return a if cond else b()
        return jnp.where(cond, a, b())

    T1 = slice(2 * _MEM, 2 * _MEM + _SEG)
    T2 = slice(2 * _MEM + _SEG, 2 * _MEM + 2 * _SEG)

    def step(t, a_chains, b_stages, mode="norm", last_in_body=True):
        both = len(a_chains) == 2
        first = mode == "first"
        last_pair = n_pairs - 1
        lo = lax.broadcasted_iota(jnp.int32, (L, PW), 1) < d_head
        lane = lax.broadcasted_iota(jnp.int32, (L, 2 * L), 1)
        row = lax.broadcasted_iota(jnp.int32, (L, 2 * L), 0)
        seg0 = lane < L
        key = jnp.where(seg0, lane, lane - L)
        allowed = (row < _MEM) | (row >= key)
        col = lax.broadcasted_iota(jnp.int32, (_SEG, D), 1)

        st = {}

        def blockdiag(a):
            zero = jnp.zeros_like(a)
            return jnp.concatenate([jnp.where(lo, a, zero), jnp.where(lo, zero, a)],
                                   axis=0).astype(_BF16)

        if len(a_chains) == 1:
            c0 = a_chains[0]
            h32 = jnp.concatenate(
                [ha_ref[_MEM * c0:_MEM * (c0 + 1), :].astype(_F32),
                 ha_ref[(T1, T2)[c0], :].astype(_F32)], axis=0)

        def pre_at(j, p, s):
            if isinstance(s, int):
                return pre_ref.at[j, p, (s - 1) * _SEG:s * _SEG, :]
            return pre_ref.at[j, p, pl.ds(pl.multiple_of((s - 1) * _SEG, _SEG), _SEG), :]

        def proj(p, j):
            w_ref = (wq_ref, wk_ref, wv_ref)[j]
            if first:
                if j == 0:
                    for jj in range(4):
                        pair_in(p, jj).wait()
                wt = stage_ref[j, p]
                w_ref[p] = wt.T
                if p == last_pair:
                    return {0: _dot(h32, wt, _NT)}
                res = _dot(h0_ref[...], wt, _NT)
                pre_ref[j, p, 0:NA, :] = res[0:NA].astype(_BF16)
                return {0: res[NA:NA + L]}
            if mode == "ahead":
                res = _dot(h32, w_ref[p])
                pre_at(j, p, t + _AHEAD)[...] = res[_MEM:L].astype(_BF16)
                return {0: jnp.concatenate([res[0:_MEM], pre_at(j, p, t)[...].astype(_F32)], axis=0)}
            if mode == "pre":
                h = jnp.concatenate([ha_ref[0:2 * _MEM, :], ha_ref[T2, :]], axis=0)
                res = _dot(h, w_ref[p])
                return {0: jnp.concatenate([res[0:_MEM], pre_at(j, p, t)[...].astype(_F32)], axis=0),
                        1: res[_MEM:_MEM + L]}
            if both:
                res = _dot(ha_ref[...], w_ref[p])
                return {c: jnp.concatenate([res[_MEM * c:_MEM * (c + 1)], res[(T1, T2)[c]]], axis=0)
                        for c in (0, 1)}
            return {c0: _dot(h32, w_ref[p])}

        def bulk(j):
            wt = stage_ref[j, last_pair]
            pre_ref[j, last_pair, 0:NA, :] = _dot(h0_ref[0:NA, :], wt, _NT).astype(_BF16)

        def a_q(p):
            st["q", p] = proj(p, 0)

        def a_k(p):
            st["k", p] = proj(p, 1)

        def a_v(p):
            st["v", p] = proj(p, 2)

        def a_s(p):
            q, k = st.pop(("q", p)), st.pop(("k", p))
            for c in a_chains:
                s = _dot(q[c], blockdiag(k[c]), _NT) * scale
                s = jnp.where(allowed, s, _NEG)
                m0 = jnp.max(jnp.where(seg0, s, -jnp.inf), axis=1, keepdims=True)
                m1 = jnp.max(jnp.where(seg0, -jnp.inf, s), axis=1, keepdims=True)
                e = jnp.exp(s - jnp.where(seg0, m0, m1))
                l0 = jnp.sum(jnp.where(seg0, e, 0.0), axis=1, keepdims=True)
                l1 = jnp.sum(jnp.where(seg0, 0.0, e), axis=1, keepdims=True)
                st["p", p, c] = e / jnp.where(seg0, l0, l1)

        def a_pv(p):
            v = st.pop(("v", p))
            outs = [_dot(st.pop(("p", p, c)), blockdiag(v[c])) for c in a_chains]
            if both:
                st["o", p] = jnp.concatenate(
                    [outs[0][:_MEM], outs[1][:_MEM], outs[0][_MEM:], outs[1][_MEM:]],
                    axis=0).astype(_BF16)
            else:
                st["o", p] = outs[0]

        def a_o(p):
            part = _dot(st.pop(("o", p)), wo_ref[p * PW:(p + 1) * PW, :])
            n = part.shape[0]
            if p == 0:
                acc_ref[0:n, :] = part
            elif p < n_pairs - 1:
                acc_ref[0:n, :] += part
            else:
                st["acc"] = acc_ref[0:n, :] + part

        def rs(c):
            return slice(_SEG * c, _SEG * (c + 1))

        def rotate(c):
            htail_ref[8 * c:8 * c + 8, :] = hprev_ref[_SEG * (c + 1) - 8:_SEG * (c + 1), :]
            hprev_ref[rs(c), :] = st.pop(("h", c))
            nprev_ref[rs(c), :] = st.pop(("ncur", c))
            yprev_ref[rs(c), :] = st.pop(("ycur", c))

        def b_1(c):
            ycur = ycur_ref[rs(c), :]
            ncur = _ln(ycur)
            st["ycur", c], st["ncur", c] = ycur, ncur
            st["h", c] = _gelu(_dot(_ln(ncur).astype(_BF16), w1_ref[...]))
            if ("b2", c) not in b_stages:
                rotate(c)

        def b_2(c):
            s = t - 2 - _LAG * c
            hprev = hprev_ref[rs(c), :]
            pt = pick(s == 0, jnp.zeros((8, D), _F32), lambda: htail_ref[8 * c:8 * c + 8, :])
            nh = pick(s == n_seg - 1, jnp.zeros((8, D), _F32), lambda: st["h", c][0:8])
            win = jnp.concatenate([pt, hprev, nh], axis=0)
            g = jnp.where(col < C, win[7:7 + _SEG],
                          jnp.where(col < 2 * C, win[9:9 + _SEG],
                                    jnp.where(col < 3 * C, win[6:6 + _SEG], win[10:10 + _SEG])))
            st["x1", c] = nprev_ref[rs(c), :] + _dot(g.astype(_BF16), w2_ref[...])
            st["yres", c] = yprev_ref[rs(c), :]
            if ("b1", c) in b_stages:
                rotate(c)

        def b_3(c):
            st["f", c] = _gelu(_dot(_ln(st["x1", c]).astype(_BF16), w3_ref[...])).astype(_BF16)

        def b_4(c):
            ynew = st.pop(("yres", c)) + st.pop(("x1", c)) + _dot(st.pop(("f", c)), w4_ref[...])
            if c == 0:
                st["y2new"] = ynew
                st["tok2"] = _ln(ynew).astype(_BF16)
            else:
                so = t - 2 - _LAG
                if isinstance(so, int):
                    o_ref[so * _SEG:(so + 1) * _SEG, :] = ynew.astype(o_ref.dtype)
                else:
                    so = jnp.maximum(so, 0)
                    o_ref[pl.ds(pl.multiple_of(so * _SEG, _SEG), _SEG), :] = ynew.astype(o_ref.dtype)

        stages = dict(q=a_q, k=a_k, v=a_v, s=a_s, pv=a_pv, o=a_o, bulk=bulk,
                      b1=b_1, b2=b_2, b3=b_3, b4=b_4)
        for name, arg in _schedule(n_pairs, a_chains, b_stages, mode, last_in_body):
            stages[name](arg)

        if "tok2" in st:
            ha_ref[T2, :] = st.pop("tok2")
        if a_chains:
            acc = st.pop("acc")
            if both:
                mem1, mem2 = acc[0:_MEM], acc[_MEM:2 * _MEM]
                a1, a2 = acc[T1], acc[T2]
            elif a_chains == (0,):
                mem1, mem2 = acc[0:_MEM], mem0_ref[...].astype(_F32)
                a1, a2 = acc[_MEM:L], None
            else:
                mem1, mem2 = mem0_ref[...].astype(_F32), acc[0:_MEM]
                a1, a2 = None, acc[_MEM:L]
            ha_ref[0:2 * _MEM, :] = jnp.concatenate([mem1, mem2], axis=0).astype(_BF16)
            if a1 is not None:
                if isinstance(t, int):
                    nxt = t + 1 + _AHEAD if t + 1 < _LAG else min(t + 1, n_seg - 1)
                else:
                    nxt = jnp.minimum(t + 1, n_seg - 1)
                ha_ref[T1, :] = _ln(xseg(nxt)).astype(_BF16)
                ycur_ref[0:_SEG, :] = xseg(t) + a1
            if a2 is not None:
                ycur_ref[_SEG:, :] = y2res_ref[...] + a2
        if "y2new" in st:
            y2res_ref[...] = st.pop("y2new")
        assert not st, list(st)

    misc["x0"].start()
    misc["mem0"].start()
    for p in range(n_pairs):
        for j in range(4):
            pair_in(p, j).start()
    for k in ("w1", "w2", "w3", "w4", "x1"):
        misc[k].start()
    for r in (ycur_ref, yprev_ref, nprev_ref, hprev_ref, htail_ref, y2res_ref):
        r[...] = jnp.zeros(r.shape, _F32)
    misc["x0"].wait()
    misc["mem0"].wait()
    mem0 = mem0_ref[...]
    ha_ref[0:2 * _MEM, :] = jnp.concatenate([mem0, mem0], axis=0).astype(_BF16)
    n0 = _ln(xseg(0))
    ha_ref[T1, :] = n0.astype(_BF16)
    ha_ref[T2, :] = jnp.zeros((_SEG, D), _BF16)
    for s in range(1, _AHEAD + 1):
        h0_ref[(s - 1) * _SEG:s * _SEG, :] = _ln(xseg(s)).astype(_BF16)
    h0_ref[NA:NA + L + _MEM, :] = jnp.concatenate(
        [mem0.astype(_F32), n0, jnp.zeros((_MEM, D), _F32)], axis=0).astype(_BF16)

    B = lambda c, which: {(n, c) for n in which}
    ALL = ("b1", "b2", "b3", "b4")

    with _scope("step0"):
        step(0, (0,), set(), "first")
    with _scope("step1"):
        misc["w1"].wait()
        step(1, (0,), B(0, ALL[:1]), "ahead")
    with _scope("step2"):
        for k in ("w2", "w3", "w4"):
            misc[k].wait()
        step(2, (0,), B(0, ALL), "ahead")
        misc["x1"].wait()

    def run(lo_t, hi_t, mode, unroll):
        assert (hi_t - lo_t) % unroll == 0

        def body(i, carry):
            for u in range(unroll):
                step(lo_t + i * unroll + u, (0, 1), B(0, ALL) | B(1, ALL), mode,
                     last_in_body=u == unroll - 1)
            return carry
        lax.fori_loop(0, (hi_t - lo_t) // unroll, body, 0)

    with _scope("loop_pre"):
        run(_LAG, _LAG + _AHEAD, "pre", 1)
    with _scope("loop"):
        n_main = n_seg - _LAG - _AHEAD
        run(_LAG + _AHEAD, n_seg, "norm", _UNROLL if n_main % _UNROLL == 0 else 1)

    with _scope("tailA"):
        out_a.start()
        step(n_seg, (1,), B(0, ALL) | B(1, ALL))
        step(n_seg + 1, (1,), B(0, ALL[1:]) | B(1, ALL))
        step(n_seg + 2, (1,), B(1, ALL))
    with _scope("tailB"):
        step(n_seg + 3, (), B(1, ALL))
        step(n_seg + 4, (), B(1, ALL[1:]))
    with _scope("out"):
        out_b.start()
        out_a.wait()
        out_b.wait()


@functools.partial(jax.jit, static_argnames=("A_seg_len",))
def pallas_interleave_layers__memory_aug_recurrent_mem_tr__mixer_s_mlp__prompt_kernel(
    A_x: jax.Array,
    A_mem0: jax.Array,
    A_Wq: jax.Array,
    A_Wk: jax.Array,
    A_Wv: jax.Array,
    A_Wo: jax.Array,
    A_seg_len,
    B_x: jax.Array,
    B_w1: jax.Array,
    B_w2: jax.Array,
    B_w3: jax.Array,
    B_w4: jax.Array,
):
    del B_x
    _, S, D = A_x.shape
    _, H, Dh = A_Wq.shape
    F = B_w3.shape[1]
    assert A_seg_len == _SEG and A_mem0.shape[1] == _MEM and A_x.shape[0] == 1
    n_seg = S // _SEG
    assert n_seg * _SEG == S and n_seg >= 2 * _LAG + 2 + _AHEAD and H % 2 == 0

    def wt(w):
        return jnp.transpose(w, (1, 2, 0)).reshape(H * Dh, D)

    R = 2 * (_MEM + _SEG)
    NP, PW = H // 2, 2 * Dh
    hbm = pl.BlockSpec(memory_space=pl.ANY)
    out = pl.pallas_call(
        functools.partial(_kernel, n_seg=n_seg, n_heads=H, d_head=Dh),
        out_shape=jax.ShapeDtypeStruct((S, D), A_x.dtype),
        in_specs=[hbm] * 10,
        out_specs=hbm,
        scratch_shapes=[
            pltpu.VMEM((S, D), _BF16),
            pltpu.VMEM((_MEM, D), _BF16),
            pltpu.VMEM((NP, D, PW), _BF16),
            pltpu.VMEM((NP, D, PW), _BF16),
            pltpu.VMEM((NP, D, PW), _BF16),
            pltpu.VMEM((H * Dh, D), _BF16),
            pltpu.VMEM((D, D), _BF16),
            pltpu.VMEM((D, D), _BF16),
            pltpu.VMEM((D, F), _BF16),
            pltpu.VMEM((F, D), _BF16),
            pltpu.VMEM((S, D), A_x.dtype),
            pltpu.VMEM((3, NP, PW, D), _BF16),
            pltpu.VMEM((R, D), _BF16),
            pltpu.VMEM((_AHEAD * _SEG + 48, D), _BF16),
            pltpu.VMEM((3, NP, (_AHEAD + _LAG - 1) * _SEG, PW), _BF16),
            pltpu.VMEM((R, D), _F32),
            pltpu.VMEM((2 * _SEG, D), _F32),
            pltpu.VMEM((2 * _SEG, D), _F32),
            pltpu.VMEM((2 * _SEG, D), _F32),
            pltpu.VMEM((2 * _SEG, D), _F32),
            pltpu.VMEM((16, D), _F32),
            pltpu.VMEM((_SEG, D), _F32),
            pltpu.SemaphoreType.DMA((4 * NP + 9,)),
        ],
        compiler_params=pltpu.CompilerParams(vmem_limit_bytes=100 * 1024 * 1024),
    )(A_x.reshape(S, D), A_mem0.reshape(_MEM, D), wt(A_Wq), wt(A_Wk), wt(A_Wv),
      A_Wo.reshape(H * Dh, D), B_w1, B_w2, B_w3, B_w4)
    return out.reshape(1, S, D)
```

```python
import contextlib
import functools

import jax
import jax.numpy as jnp
from jax import lax
import jax.experimental.pallas as pl
import jax.experimental.pallas.tpu as pltpu

_SEG = 32
_MEM = 8
_LAG = 3
_AHEAD = 9
_UNROLL = 1
_NEG = -1000000000.0
_EPS = 1e-05

_F32 = jnp.float32
_BF16 = jnp.bfloat16

_NT = (((1,), (1,)), ((), ()))
_NN = (((1,), (0,)), ((), ()))


_PROFILE_SCOPES = False


def _scope(name):
    return jax.named_scope(name) if _PROFILE_SCOPES else contextlib.nullcontext()


def _dot(a, b, dims=_NN):
    return lax.dot_general(a, b, dims, preferred_element_type=_F32)


def _ln(x):
    m = jnp.mean(x, axis=-1, keepdims=True)
    d = x - m
    v = jnp.mean(d * d, axis=-1, keepdims=True)
    return d * lax.rsqrt(v + _EPS)


def _gelu(x):
    return jax.nn.gelu(x, approximate=True)


def _token_shift(win):
    n, D = win.shape[0] - 16, win.shape[1]
    C = D // 4
    col = lax.broadcasted_iota(jnp.int32, (n, D), 1)
    return jnp.where(col < C, win[7:7 + n],
                     jnp.where(col < 2 * C, win[9:9 + n],
                               jnp.where(col < 3 * C, win[6:6 + n], win[10:10 + n])))


def _schedule(n_pairs, a_chains, b_stages, mode, last_in_body):
    slots = {("b1", 0): 1, ("b2", 0): 3, ("b3", 0): 5, ("b4", 0): 7,
             ("b1", 1): 9, ("b2", 1): 11, ("b3", 1): n_pairs, ("b4", 1): n_pairs + 1}
    if not last_in_body:
        slots[("b3", 1)] = n_pairs + 1
        slots[("b4", 1)] = n_pairs + 3
    b_list = [(n, c) for c in (0, 1) for n in ("b1", "b2", "b3", "b4") if (n, c) in b_stages]
    if not a_chains:
        return tuple(b_list)
    sched = []
    last = n_pairs - 1
    for i in range(n_pairs + 4):
        if i < n_pairs:
            sched += [("q", i), ("k", i)]
        if mode == "first" and i == n_pairs:
            sched.append(("bulk", 0))
        if 0 <= i - 1 < n_pairs:
            sched.append(("s", i - 1))
        if i < n_pairs:
            sched.append(("v", i))
        sched += [b for b in b_list if slots[b] == i]
        if 0 <= i - 2 < n_pairs:
            sched.append(("pv", i - 2))
        if 0 <= i - 3 < n_pairs:
            sched.append(("o", i - 3))
        if mode == "first" and i == n_pairs:
            sched.append(("bulk", 1))
        if mode == "first" and i == n_pairs + 1:
            sched.append(("bulk", 2))
    return tuple(sched)


def _kernel(x_hbm, mem0_hbm, wqt_hbm, wkt_hbm, wvt_hbm, wo_hbm,
            w1_hbm, w2_hbm, w3_hbm, w4_hbm, o_hbm,
            x_ref, mem0_ref, wq_ref, wk_ref, wv_ref, wo_ref,
            w1_ref, w2_ref, w3_ref, w4_ref, o_ref, stage_ref,
            ha_ref, h0_ref, pre_ref, acc_ref, ycur_ref, yprev_ref, nprev_ref, hprev_ref,
            htail_ref, y2res_ref, sems, *, n_seg, n_heads, d_head):
    S, D = x_ref.shape
    PW = 2 * d_head
    n_pairs = n_heads // 2
    scale = d_head ** -0.5
    L = _MEM + _SEG
    NA = _AHEAD * _SEG
    X0 = (_AHEAD + _LAG) * _SEG

    def pair_in(p, j):
        rows = pl.ds(p * PW, PW)
        sem = sems.at[4 * p + j]
        if j < 3:
            src = (wqt_hbm, wkt_hbm, wvt_hbm)[j]
            return pltpu.make_async_copy(src.at[rows, :], stage_ref.at[j, p], sem)
        return pltpu.make_async_copy(wo_hbm.at[rows, :], wo_ref.at[rows, :], sem)

    nb = 4 * n_pairs
    misc = dict(
        x0=pltpu.make_async_copy(x_hbm.at[pl.ds(0, X0), :], x_ref.at[pl.ds(0, X0), :], sems.at[nb]),
        x1=pltpu.make_async_copy(x_hbm.at[pl.ds(X0, S - X0), :], x_ref.at[pl.ds(X0, S - X0), :],
                                 sems.at[nb + 1]),
        mem0=pltpu.make_async_copy(mem0_hbm, mem0_ref, sems.at[nb + 2]),
        w1=pltpu.make_async_copy(w1_hbm, w1_ref, sems.at[nb + 3]),
        w2=pltpu.make_async_copy(w2_hbm, w2_ref, sems.at[nb + 4]),
        w3=pltpu.make_async_copy(w3_hbm, w3_ref, sems.at[nb + 5]),
        w4=pltpu.make_async_copy(w4_hbm, w4_ref, sems.at[nb + 6]),
    )
    n_early = (n_seg - _LAG - 2) * _SEG
    out_a = pltpu.make_async_copy(o_ref.at[pl.ds(0, n_early), :], o_hbm.at[pl.ds(0, n_early), :],
                                  sems.at[nb + 7])
    out_b = pltpu.make_async_copy(o_ref.at[pl.ds(n_early, S - n_early), :],
                                  o_hbm.at[pl.ds(n_early, S - n_early), :], sems.at[nb + 8])

    def xseg(s):
        if isinstance(s, int):
            return x_ref[s * _SEG:(s + 1) * _SEG, :].astype(_F32)
        return x_ref[pl.ds(pl.multiple_of(s * _SEG, _SEG), _SEG), :].astype(_F32)

    def pick(cond, a, b):
        if isinstance(cond, bool):
            return a if cond else b()
        return jnp.where(cond, a, b())

    T1 = slice(2 * _MEM, 2 * _MEM + _SEG)
    T2 = slice(2 * _MEM + _SEG, 2 * _MEM + 2 * _SEG)

    def step(t, a_chains, b_stages, mode="norm", last_in_body=True):
        both = len(a_chains) == 2
        first = mode == "first"
        last_pair = n_pairs - 1
        lo = lax.broadcasted_iota(jnp.int32, (L, PW), 1) < d_head
        lane = lax.broadcasted_iota(jnp.int32, (L, 2 * L), 1)
        row = lax.broadcasted_iota(jnp.int32, (L, 2 * L), 0)
        seg0 = lane < L
        key = jnp.where(seg0, lane, lane - L)
        allowed = (row < _MEM) | (row >= key)

        st = {}

        def blockdiag(a):
            zero = jnp.zeros_like(a)
            return jnp.concatenate([jnp.where(lo, a, zero), jnp.where(lo, zero, a)],
                                   axis=0).astype(_BF16)

        if len(a_chains) == 1:
            c0 = a_chains[0]
            h32 = jnp.concatenate(
                [ha_ref[_MEM * c0:_MEM * (c0 + 1), :].astype(_F32),
                 ha_ref[(T1, T2)[c0], :].astype(_F32)], axis=0)

        def pre_at(j, p, s):
            if isinstance(s, int):
                return pre_ref.at[j, p, (s - 1) * _SEG:s * _SEG, :]
            return pre_ref.at[j, p, pl.ds(pl.multiple_of((s - 1) * _SEG, _SEG), _SEG), :]

        def proj(p, j):
            w_ref = (wq_ref, wk_ref, wv_ref)[j]
            if first:
                if j == 0:
                    for jj in range(3):
                        pair_in(p, jj).wait()
                    if p > 0:
                        pair_in(p - 1, 3).wait()
                wt = stage_ref[j, p]
                w_ref[p] = wt.T
                if p == last_pair:
                    return {0: _dot(h32, wt, _NT)}
                res = _dot(h0_ref[...], wt, _NT)
                pre_ref[j, p, 0:NA, :] = res[0:NA].astype(_BF16)
                return {0: res[NA:NA + L]}
            if mode == "ahead":
                res = _dot(h32, w_ref[p])
                pre_at(j, p, t + _AHEAD)[...] = res[_MEM:L].astype(_BF16)
                return {0: jnp.concatenate([res[0:_MEM], pre_at(j, p, t)[...].astype(_F32)], axis=0)}
            if mode == "pre":
                h = jnp.concatenate([ha_ref[0:2 * _MEM, :], ha_ref[T2, :]], axis=0)
                res = _dot(h, w_ref[p])
                return {0: jnp.concatenate([res[0:_MEM], pre_at(j, p, t)[...].astype(_F32)], axis=0),
                        1: res[_MEM:_MEM + L]}
            if both:
                res = _dot(ha_ref[...], w_ref[p])
                return {c: jnp.concatenate([res[_MEM * c:_MEM * (c + 1)], res[(T1, T2)[c]]], axis=0)
                        for c in (0, 1)}
            return {c0: _dot(h32, w_ref[p])}

        def bulk(j):
            wt = stage_ref[j, last_pair]
            pre_ref[j, last_pair, 0:NA, :] = _dot(h0_ref[0:NA, :], wt, _NT).astype(_BF16)

        def a_q(p):
            st["q", p] = proj(p, 0)

        def a_k(p):
            st["k", p] = proj(p, 1)

        def a_v(p):
            st["v", p] = proj(p, 2)

        def a_s(p):
            q, k = st.pop(("q", p)), st.pop(("k", p))
            for c in a_chains:
                s = _dot(q[c], blockdiag(k[c]), _NT) * scale
                s = jnp.where(allowed, s, _NEG)
                m0 = jnp.max(jnp.where(seg0, s, -jnp.inf), axis=1, keepdims=True)
                m1 = jnp.max(jnp.where(seg0, -jnp.inf, s), axis=1, keepdims=True)
                e = jnp.exp(s - jnp.where(seg0, m0, m1))
                l0 = jnp.sum(jnp.where(seg0, e, 0.0), axis=1, keepdims=True)
                l1 = jnp.sum(jnp.where(seg0, 0.0, e), axis=1, keepdims=True)
                st["p", p, c] = e / jnp.where(seg0, l0, l1)

        def a_pv(p):
            v = st.pop(("v", p))
            outs = [_dot(st.pop(("p", p, c)), blockdiag(v[c])) for c in a_chains]
            if both:
                st["o", p] = jnp.concatenate(
                    [outs[0][:_MEM], outs[1][:_MEM], outs[0][_MEM:], outs[1][_MEM:]],
                    axis=0).astype(_BF16)
            else:
                st["o", p] = outs[0]

        def a_o(p):
            if first and p == last_pair:
                pair_in(p, 3).wait()
            part = _dot(st.pop(("o", p)), wo_ref[p * PW:(p + 1) * PW, :])
            n = part.shape[0]
            if p == 0:
                acc_ref[0:n, :] = part
            elif p < n_pairs - 1:
                acc_ref[0:n, :] += part
            else:
                st["acc"] = acc_ref[0:n, :] + part

        def rs(c):
            return slice(_SEG * c, _SEG * (c + 1))

        def rotate(c):
            htail_ref[8 * c:8 * c + 8, :] = hprev_ref[_SEG * (c + 1) - 8:_SEG * (c + 1), :]
            hprev_ref[rs(c), :] = st.pop(("h", c))
            nprev_ref[rs(c), :] = st.pop(("ncur", c))
            yprev_ref[rs(c), :] = st.pop(("ycur", c))

        def b_1(c):
            ycur = ycur_ref[rs(c), :]
            ncur = _ln(ycur)
            st["ycur", c], st["ncur", c] = ycur, ncur
            st["h", c] = _gelu(_dot(_ln(ncur).astype(_BF16), w1_ref[...]))
            if ("b2", c) not in b_stages:
                rotate(c)

        def b_2(c):
            s = t - 2 - _LAG * c
            hprev = hprev_ref[rs(c), :]
            pt = pick(s == 0, jnp.zeros((8, D), _F32), lambda: htail_ref[8 * c:8 * c + 8, :])
            nh = pick(s == n_seg - 1, jnp.zeros((8, D), _F32), lambda: st["h", c][0:8])
            g = _token_shift(jnp.concatenate([pt, hprev, nh], axis=0))
            st["x1", c] = nprev_ref[rs(c), :] + _dot(g.astype(_BF16), w2_ref[...])
            st["yres", c] = yprev_ref[rs(c), :]
            if ("b1", c) in b_stages:
                rotate(c)

        def b_3(c):
            st["f", c] = _gelu(_dot(_ln(st["x1", c]).astype(_BF16), w3_ref[...])).astype(_BF16)

        def b_4(c):
            ynew = st.pop(("yres", c)) + st.pop(("x1", c)) + _dot(st.pop(("f", c)), w4_ref[...])
            if c == 0:
                st["y2new"] = ynew
                st["tok2"] = _ln(ynew).astype(_BF16)
            else:
                so = t - 2 - _LAG
                if isinstance(so, int):
                    o_ref[so * _SEG:(so + 1) * _SEG, :] = ynew.astype(o_ref.dtype)
                else:
                    o_ref[pl.ds(pl.multiple_of(so * _SEG, _SEG), _SEG), :] = ynew.astype(o_ref.dtype)

        stages = dict(q=a_q, k=a_k, v=a_v, s=a_s, pv=a_pv, o=a_o, bulk=bulk,
                      b1=b_1, b2=b_2, b3=b_3, b4=b_4)
        for name, arg in _schedule(n_pairs, a_chains, b_stages, mode, last_in_body):
            stages[name](arg)

        if "tok2" in st:
            ha_ref[T2, :] = st.pop("tok2")
        if a_chains:
            acc = st.pop("acc")
            if both:
                mem1, mem2 = acc[0:_MEM], acc[_MEM:2 * _MEM]
                a1, a2 = acc[T1], acc[T2]
            elif a_chains == (0,):
                mem1, mem2 = acc[0:_MEM], mem0_ref[...].astype(_F32)
                a1, a2 = acc[_MEM:L], None
            else:
                mem1, mem2 = mem0_ref[...].astype(_F32), acc[0:_MEM]
                a1, a2 = None, acc[_MEM:L]
            ha_ref[0:2 * _MEM, :] = jnp.concatenate([mem1, mem2], axis=0).astype(_BF16)
            if a1 is not None:
                if isinstance(t, int):
                    nxt = t + 1 + _AHEAD if t + 1 < _LAG else min(t + 1, n_seg - 1)
                else:
                    nxt = jnp.minimum(t + 1, n_seg - 1)
                ha_ref[T1, :] = _ln(xseg(nxt)).astype(_BF16)
                ycur_ref[0:_SEG, :] = xseg(t) + a1
            if a2 is not None:
                ycur_ref[_SEG:, :] = y2res_ref[...] + a2
        if "y2new" in st:
            y2res_ref[...] = st.pop("y2new")
        assert not st, list(st)

    misc["x0"].start()
    misc["mem0"].start()
    for p in range(n_pairs):
        for j in range(4):
            pair_in(p, j).start()
    for k in ("w1", "w2", "w3", "w4", "x1"):
        misc[k].start()
    for r in (ycur_ref, yprev_ref, nprev_ref, hprev_ref, htail_ref, y2res_ref):
        r[...] = jnp.zeros(r.shape, _F32)
    misc["x0"].wait()
    misc["mem0"].wait()
    mem0 = mem0_ref[...]
    ha_ref[0:2 * _MEM, :] = jnp.concatenate([mem0, mem0], axis=0).astype(_BF16)
    n0 = _ln(xseg(0))
    ha_ref[T1, :] = n0.astype(_BF16)
    ha_ref[T2, :] = jnp.zeros((_SEG, D), _BF16)
    for s in range(1, _AHEAD + 1):
        h0_ref[(s - 1) * _SEG:s * _SEG, :] = _ln(xseg(s)).astype(_BF16)
    h0_ref[NA:NA + L + _MEM, :] = jnp.concatenate(
        [mem0.astype(_F32), n0, jnp.zeros((_MEM, D), _F32)], axis=0).astype(_BF16)

    B = lambda c, which: {(n, c) for n in which}
    ALL = ("b1", "b2", "b3", "b4")

    with _scope("step0"):
        step(0, (0,), set(), "first")
    with _scope("step1"):
        misc["w1"].wait()
        step(1, (0,), B(0, ALL[:1]), "ahead")
    with _scope("step2"):
        for k in ("w2", "w3", "w4"):
            misc[k].wait()
        step(2, (0,), B(0, ALL), "ahead")
        misc["x1"].wait()

    def run(lo_t, hi_t, mode, unroll):
        assert (hi_t - lo_t) % unroll == 0

        def body(i, carry):
            for u in range(unroll):
                step(lo_t + i * unroll + u, (0, 1), B(0, ALL) | B(1, ALL), mode,
                     last_in_body=u == unroll - 1)
            return carry
        lax.fori_loop(0, (hi_t - lo_t) // unroll, body, 0)

    with _scope("loop_pre"):
        step(_LAG, (0, 1), B(0, ALL), "pre")
        step(_LAG + 1, (0, 1), B(0, ALL) | B(1, ALL[:1]), "pre")
        run(_LAG + 2, _LAG + _AHEAD, "pre", 1)
    with _scope("loop"):
        n_main = n_seg - _LAG - _AHEAD
        run(_LAG + _AHEAD, n_seg, "norm", _UNROLL if n_main % _UNROLL == 0 else 1)

    with _scope("tailA"):
        out_a.start()
        step(n_seg, (1,), B(0, ALL) | B(1, ALL))
        step(n_seg + 1, (1,), B(0, ALL[1:]) | B(1, ALL))
        step(n_seg + 2, (1,), B(1, ALL))
    with _scope("tailB"):
        C1 = slice(_SEG, 2 * _SEG)
        ycur = ycur_ref[C1, :]
        ncur = _ln(ycur)
        hcur = _gelu(_dot(_ln(ncur).astype(_BF16), w1_ref[...]))
        g = _token_shift(jnp.concatenate(
            [htail_ref[8:16, :], hprev_ref[C1, :], hcur, jnp.zeros((8, D), _F32)], axis=0))
        x1 = jnp.concatenate([nprev_ref[C1, :], ncur], axis=0) + _dot(g.astype(_BF16), w2_ref[...])
        f = _gelu(_dot(_ln(x1).astype(_BF16), w3_ref[...])).astype(_BF16)
        ynew = jnp.concatenate([yprev_ref[C1, :], ycur], axis=0) + x1 + _dot(f, w4_ref[...])
        o_ref[(n_seg - 2) * _SEG:n_seg * _SEG, :] = ynew.astype(o_ref.dtype)
    with _scope("out"):
        out_b.start()
        out_a.wait()
        out_b.wait()


@functools.partial(jax.jit, static_argnames=("A_seg_len",))
def pallas_interleave_layers__memory_aug_recurrent_mem_tr__mixer_s_mlp__prompt_kernel(
    A_x: jax.Array,
    A_mem0: jax.Array,
    A_Wq: jax.Array,
    A_Wk: jax.Array,
    A_Wv: jax.Array,
    A_Wo: jax.Array,
    A_seg_len,
    B_x: jax.Array,
    B_w1: jax.Array,
    B_w2: jax.Array,
    B_w3: jax.Array,
    B_w4: jax.Array,
):
    del B_x
    _, S, D = A_x.shape
    _, H, Dh = A_Wq.shape
    F = B_w3.shape[1]
    assert A_seg_len == _SEG and A_mem0.shape[1] == _MEM and A_x.shape[0] == 1
    n_seg = S // _SEG
    assert n_seg * _SEG == S and n_seg >= 2 * _LAG + 2 + _AHEAD and H % 2 == 0

    def wt(w):
        return jnp.transpose(w, (1, 2, 0)).reshape(H * Dh, D)

    R = 2 * (_MEM + _SEG)
    NP, PW = H // 2, 2 * Dh
    hbm = pl.BlockSpec(memory_space=pl.ANY)
    out = pl.pallas_call(
        functools.partial(_kernel, n_seg=n_seg, n_heads=H, d_head=Dh),
        out_shape=jax.ShapeDtypeStruct((S, D), A_x.dtype),
        in_specs=[hbm] * 10,
        out_specs=hbm,
        scratch_shapes=[
            pltpu.VMEM((S, D), _BF16),
            pltpu.VMEM((_MEM, D), _BF16),
            pltpu.VMEM((NP, D, PW), _BF16),
            pltpu.VMEM((NP, D, PW), _BF16),
            pltpu.VMEM((NP, D, PW), _BF16),
            pltpu.VMEM((H * Dh, D), _BF16),
            pltpu.VMEM((D, D), _BF16),
            pltpu.VMEM((D, D), _BF16),
            pltpu.VMEM((D, F), _BF16),
            pltpu.VMEM((F, D), _BF16),
            pltpu.VMEM((S, D), A_x.dtype),
            pltpu.VMEM((3, NP, PW, D), _BF16),
            pltpu.VMEM((R, D), _BF16),
            pltpu.VMEM((_AHEAD * _SEG + 48, D), _BF16),
            pltpu.VMEM((3, NP, (_AHEAD + _LAG - 1) * _SEG, PW), _BF16),
            pltpu.VMEM((R, D), _F32),
            pltpu.VMEM((2 * _SEG, D), _F32),
            pltpu.VMEM((2 * _SEG, D), _F32),
            pltpu.VMEM((2 * _SEG, D), _F32),
            pltpu.VMEM((2 * _SEG, D), _F32),
            pltpu.VMEM((16, D), _F32),
            pltpu.VMEM((_SEG, D), _F32),
            pltpu.SemaphoreType.DMA((4 * NP + 9,)),
        ],
        compiler_params=pltpu.CompilerParams(vmem_limit_bytes=100 * 1024 * 1024),
    )(A_x.reshape(S, D), A_mem0.reshape(_MEM, D), wt(A_Wq), wt(A_Wk), wt(A_Wv),
      A_Wo.reshape(H * Dh, D), B_w1, B_w2, B_w3, B_w4)
    return out.reshape(1, S, D)
```

```python
import contextlib
import functools

import jax
import jax.numpy as jnp
from jax import lax
import jax.experimental.pallas as pl
import jax.experimental.pallas.tpu as pltpu

_SEG = 32
_MEM = 8
_LAG = 3
_AHEAD = 9
_NEG = -1000000000.0
_EPS = 1e-05

_F32 = jnp.float32
_BF16 = jnp.bfloat16

_NT = (((1,), (1,)), ((), ()))
_NN = (((1,), (0,)), ((), ()))


_PROFILE_SCOPES = False


def _scope(name):
    return jax.named_scope(name) if _PROFILE_SCOPES else contextlib.nullcontext()


def _dot(a, b, dims=_NN):
    return lax.dot_general(a, b, dims, preferred_element_type=_F32)


def _ln(x):
    m = jnp.mean(x, axis=-1, keepdims=True)
    d = x - m
    v = jnp.mean(d * d, axis=-1, keepdims=True)
    return d * lax.rsqrt(v + _EPS)


def _gelu(x):
    return jax.nn.gelu(x, approximate=True)


def _token_shift(win):
    n, D = win.shape[0] - 16, win.shape[1]
    C = D // 4
    col = lax.broadcasted_iota(jnp.int32, (n, D), 1)
    return jnp.where(col < C, win[7:7 + n],
                     jnp.where(col < 2 * C, win[9:9 + n],
                               jnp.where(col < 3 * C, win[6:6 + n], win[10:10 + n])))


_DEFAULT_ORDER = (("q", "k", "s", "v", "b", "pv", "o"), (1, 2, 3), (1, 3, 5, 7, 9, 11, 16, 17))
_ORDERS = {
    ("norm", 2): (("q", "k", "s", "pv", "v", "b", "o"), (1, 3, 4), (2, 5, 7, 9, 10, 13, 15, 18)),
}
_MIXER = tuple((n, c) for c in (0, 1) for n in ("b1", "b2", "b3", "b4"))


def _schedule(n_pairs, a_chains, b_stages, mode):
    order, (lag_s, lag_pv, lag_o), slots = _ORDERS.get((mode, len(a_chains)), _DEFAULT_ORDER)
    scale = n_pairs / 16.0
    slots = {b: int(round(s * scale)) for b, s in zip(_MIXER, slots)}
    lag = dict(q=0, k=0, v=0, s=lag_s, pv=lag_pv, o=lag_o)
    sched = []
    for i in range(max(n_pairs + lag_o, max(slots.values()) + 1)):
        for item in order:
            if item == "b":
                sched += [b for b in _MIXER if b in b_stages and slots[b] == i]
            elif 0 <= i - lag[item] < n_pairs:
                sched.append((item, i - lag[item]))
    if mode == "first":
        last = n_pairs - 1
        for j, before in enumerate((("s", last), ("pv", last), ("o", last))):
            sched.insert(sched.index(before), ("bulk", j))
    return tuple(sched)


def _kernel(x_hbm, mem0_hbm, wqt_hbm, wkt_hbm, wvt_hbm, wo_hbm,
            w1_hbm, w2_hbm, w3_hbm, w4_hbm, o_hbm,
            x_ref, mem0_ref, wq_ref, wk_ref, wv_ref, wo_ref,
            w1_ref, w2_ref, w3_ref, w4_ref, o_ref, stage_ref,
            ha_ref, h0_ref, pre_ref, acc_ref, ycur_ref, yprev_ref, nprev_ref, hprev_ref,
            htail_ref, y2res_ref, sems, *, n_seg, n_heads, d_head):
    S, D = x_ref.shape
    PW = 2 * d_head
    n_pairs = n_heads // 2
    scale = d_head ** -0.5
    L = _MEM + _SEG
    NA = _AHEAD * _SEG
    X0 = (_AHEAD + _LAG) * _SEG

    def pair_in(p, j):
        rows = pl.ds(p * PW, PW)
        sem = sems.at[4 * p + j]
        if j < 3:
            src = (wqt_hbm, wkt_hbm, wvt_hbm)[j]
            return pltpu.make_async_copy(src.at[rows, :], stage_ref.at[j, p], sem)
        return pltpu.make_async_copy(wo_hbm.at[rows, :], wo_ref.at[rows, :], sem)

    nb = 4 * n_pairs
    misc = dict(
        x0=pltpu.make_async_copy(x_hbm.at[pl.ds(0, X0), :], x_ref.at[pl.ds(0, X0), :], sems.at[nb]),
        x1=pltpu.make_async_copy(x_hbm.at[pl.ds(X0, S - X0), :], x_ref.at[pl.ds(X0, S - X0), :],
                                 sems.at[nb + 1]),
        mem0=pltpu.make_async_copy(mem0_hbm, mem0_ref, sems.at[nb + 2]),
        w1=pltpu.make_async_copy(w1_hbm, w1_ref, sems.at[nb + 3]),
        w2=pltpu.make_async_copy(w2_hbm, w2_ref, sems.at[nb + 4]),
        w3=pltpu.make_async_copy(w3_hbm, w3_ref, sems.at[nb + 5]),
        w4=pltpu.make_async_copy(w4_hbm, w4_ref, sems.at[nb + 6]),
    )
    n_early = (n_seg - _LAG - 2) * _SEG
    out_a = pltpu.make_async_copy(o_ref.at[pl.ds(0, n_early), :], o_hbm.at[pl.ds(0, n_early), :],
                                  sems.at[nb + 7])
    out_b = pltpu.make_async_copy(o_ref.at[pl.ds(n_early, S - n_early), :],
                                  o_hbm.at[pl.ds(n_early, S - n_early), :], sems.at[nb + 8])

    def xseg(s):
        if isinstance(s, int):
            return x_ref[s * _SEG:(s + 1) * _SEG, :].astype(_F32)
        return x_ref[pl.ds(pl.multiple_of(s * _SEG, _SEG), _SEG), :].astype(_F32)

    def pick(cond, a, b):
        if isinstance(cond, bool):
            return a if cond else b()
        return jnp.where(cond, a, b())

    T1 = slice(2 * _MEM, 2 * _MEM + _SEG)
    T2 = slice(2 * _MEM + _SEG, 2 * _MEM + 2 * _SEG)

    def step(t, a_chains, b_stages, mode="norm"):
        both = len(a_chains) == 2
        first = mode == "first"
        last_pair = n_pairs - 1
        lo = lax.broadcasted_iota(jnp.int32, (L, PW), 1) < d_head
        lane = lax.broadcasted_iota(jnp.int32, (L, 2 * L), 1)
        row = lax.broadcasted_iota(jnp.int32, (L, 2 * L), 0)
        seg0 = lane < L
        key = jnp.where(seg0, lane, lane - L)
        allowed = (row < _MEM) | (row >= key)

        st = {}

        def blockdiag(a):
            zero = jnp.zeros_like(a)
            return jnp.concatenate([jnp.where(lo, a, zero), jnp.where(lo, zero, a)],
                                   axis=0).astype(_BF16)

        if len(a_chains) == 1:
            c0 = a_chains[0]
            h32 = jnp.concatenate(
                [ha_ref[_MEM * c0:_MEM * (c0 + 1), :].astype(_F32),
                 ha_ref[(T1, T2)[c0], :].astype(_F32)], axis=0)

        def pre_at(j, p, s):
            if isinstance(s, int):
                return pre_ref.at[j, p, (s - 1) * _SEG:s * _SEG, :]
            return pre_ref.at[j, p, pl.ds(pl.multiple_of((s - 1) * _SEG, _SEG), _SEG), :]

        def proj(p, j):
            w_ref = (wq_ref, wk_ref, wv_ref)[j]
            if first:
                if j == 0:
                    for jj in range(3):
                        pair_in(p, jj).wait()
                    if p > 0:
                        pair_in(p - 1, 3).wait()
                wt = stage_ref[j, p]
                w_ref[p] = wt.T
                if p == last_pair:
                    return {0: _dot(h32, wt, _NT)}
                res = _dot(h0_ref[...], wt, _NT)
                pre_ref[j, p, 0:NA, :] = res[0:NA].astype(_BF16)
                return {0: res[NA:NA + L]}
            if mode == "ahead":
                res = _dot(h32, w_ref[p])
                pre_at(j, p, t + _AHEAD)[...] = res[_MEM:L].astype(_BF16)
                return {0: jnp.concatenate([res[0:_MEM], pre_at(j, p, t)[...].astype(_F32)], axis=0)}
            if mode == "pre":
                h = jnp.concatenate([ha_ref[0:2 * _MEM, :], ha_ref[T2, :]], axis=0)
                res = _dot(h, w_ref[p])
                return {0: jnp.concatenate([res[0:_MEM], pre_at(j, p, t)[...].astype(_F32)], axis=0),
                        1: res[_MEM:_MEM + L]}
            if both:
                res = _dot(ha_ref[...], w_ref[p])
                return {c: jnp.concatenate([res[_MEM * c:_MEM * (c + 1)], res[(T1, T2)[c]]], axis=0)
                        for c in (0, 1)}
            return {c0: _dot(h32, w_ref[p])}

        def bulk(j):
            wt = stage_ref[j, last_pair]
            pre_ref[j, last_pair, 0:NA, :] = _dot(h0_ref[0:NA, :], wt, _NT).astype(_BF16)

        def a_q(p):
            st["q", p] = proj(p, 0)

        def a_k(p):
            st["k", p] = proj(p, 1)

        def a_v(p):
            st["v", p] = proj(p, 2)

        def a_s(p):
            q, k = st.pop(("q", p)), st.pop(("k", p))
            for c in a_chains:
                s = _dot(q[c], blockdiag(k[c]), _NT) * scale
                s = jnp.where(allowed, s, _NEG)
                m0 = jnp.max(jnp.where(seg0, s, -jnp.inf), axis=1, keepdims=True)
                m1 = jnp.max(jnp.where(seg0, -jnp.inf, s), axis=1, keepdims=True)
                e = jnp.exp(s - jnp.where(seg0, m0, m1))
                l0 = jnp.sum(jnp.where(seg0, e, 0.0), axis=1, keepdims=True)
                l1 = jnp.sum(jnp.where(seg0, 0.0, e), axis=1, keepdims=True)
                st["p", p, c] = e / jnp.where(seg0, l0, l1)

        def a_pv(p):
            v = st.pop(("v", p))
            outs = [_dot(st.pop(("p", p, c)), blockdiag(v[c])) for c in a_chains]
            if both:
                st["o", p] = jnp.concatenate(
                    [outs[0][:_MEM], outs[1][:_MEM], outs[0][_MEM:], outs[1][_MEM:]],
                    axis=0).astype(_BF16)
            else:
                st["o", p] = outs[0]

        def a_o(p):
            if first and p == last_pair:
                pair_in(p, 3).wait()
            part = _dot(st.pop(("o", p)), wo_ref[p * PW:(p + 1) * PW, :])
            n = part.shape[0]
            if p == 0:
                acc_ref[0:n, :] = part
            elif p < n_pairs - 1:
                acc_ref[0:n, :] += part
            else:
                st["acc"] = acc_ref[0:n, :] + part

        def rs(c):
            return slice(_SEG * c, _SEG * (c + 1))

        def rotate(c):
            htail_ref[8 * c:8 * c + 8, :] = hprev_ref[_SEG * (c + 1) - 8:_SEG * (c + 1), :]
            hprev_ref[rs(c), :] = st.pop(("h", c))
            nprev_ref[rs(c), :] = st.pop(("ncur", c))
            yprev_ref[rs(c), :] = st.pop(("ycur", c))

        def b_1(c):
            ycur = ycur_ref[rs(c), :]
            ncur = _ln(ycur)
            st["ycur", c], st["ncur", c] = ycur, ncur
            st["h", c] = _gelu(_dot(_ln(ncur).astype(_BF16), w1_ref[...]))
            if ("b2", c) not in b_stages:
                rotate(c)

        def b_2(c):
            s = t - 2 - _LAG * c
            hprev = hprev_ref[rs(c), :]
            pt = pick(s == 0, jnp.zeros((8, D), _F32), lambda: htail_ref[8 * c:8 * c + 8, :])
            nh = pick(s == n_seg - 1, jnp.zeros((8, D), _F32), lambda: st["h", c][0:8])
            g = _token_shift(jnp.concatenate([pt, hprev, nh], axis=0))
            st["x1", c] = nprev_ref[rs(c), :] + _dot(g.astype(_BF16), w2_ref[...])
            st["yres", c] = yprev_ref[rs(c), :]
            if ("b1", c) in b_stages:
                rotate(c)

        def b_3(c):
            st["f", c] = _gelu(_dot(_ln(st["x1", c]).astype(_BF16), w3_ref[...])).astype(_BF16)

        def b_4(c):
            ynew = st.pop(("yres", c)) + st.pop(("x1", c)) + _dot(st.pop(("f", c)), w4_ref[...])
            if c == 0:
                st["y2new"] = ynew
                st["tok2"] = _ln(ynew).astype(_BF16)
            else:
                so = t - 2 - _LAG
                if isinstance(so, int):
                    o_ref[so * _SEG:(so + 1) * _SEG, :] = ynew.astype(o_ref.dtype)
                else:
                    o_ref[pl.ds(pl.multiple_of(so * _SEG, _SEG), _SEG), :] = ynew.astype(o_ref.dtype)

        stages = dict(q=a_q, k=a_k, v=a_v, s=a_s, pv=a_pv, o=a_o, bulk=bulk,
                      b1=b_1, b2=b_2, b3=b_3, b4=b_4)
        for name, arg in _schedule(n_pairs, a_chains, b_stages, mode):
            stages[name](arg)

        if "tok2" in st:
            ha_ref[T2, :] = st.pop("tok2")
        if a_chains:
            acc = st.pop("acc")
            if both:
                mem1, mem2 = acc[0:_MEM], acc[_MEM:2 * _MEM]
                a1, a2 = acc[T1], acc[T2]
            elif a_chains == (0,):
                mem1, mem2 = acc[0:_MEM], mem0_ref[...].astype(_F32)
                a1, a2 = acc[_MEM:L], None
            else:
                mem1, mem2 = mem0_ref[...].astype(_F32), acc[0:_MEM]
                a1, a2 = None, acc[_MEM:L]
            ha_ref[0:2 * _MEM, :] = jnp.concatenate([mem1, mem2], axis=0).astype(_BF16)
            if a1 is not None:
                if isinstance(t, int):
                    nxt = t + 1 + _AHEAD if t + 1 < _LAG else min(t + 1, n_seg - 1)
                else:
                    nxt = jnp.minimum(t + 1, n_seg - 1)
                ha_ref[T1, :] = _ln(xseg(nxt)).astype(_BF16)
                ycur_ref[0:_SEG, :] = xseg(t) + a1
            if a2 is not None:
                ycur_ref[_SEG:, :] = y2res_ref[...] + a2
        if "y2new" in st:
            y2res_ref[...] = st.pop("y2new")
        assert not st, list(st)

    misc["x0"].start()
    misc["mem0"].start()
    for p in range(n_pairs):
        for j in range(4):
            pair_in(p, j).start()
    for k in ("w1", "w2", "w3", "w4", "x1"):
        misc[k].start()
    for r in (ycur_ref, yprev_ref, nprev_ref, hprev_ref, htail_ref, y2res_ref):
        r[...] = jnp.zeros(r.shape, _F32)
    misc["x0"].wait()
    misc["mem0"].wait()
    mem0 = mem0_ref[...]
    ha_ref[0:2 * _MEM, :] = jnp.concatenate([mem0, mem0], axis=0).astype(_BF16)
    n0 = _ln(xseg(0))
    ha_ref[T1, :] = n0.astype(_BF16)
    ha_ref[T2, :] = jnp.zeros((_SEG, D), _BF16)
    for s in range(1, _AHEAD + 1):
        h0_ref[(s - 1) * _SEG:s * _SEG, :] = _ln(xseg(s)).astype(_BF16)
    h0_ref[NA:NA + L + _MEM, :] = jnp.concatenate(
        [mem0.astype(_F32), n0, jnp.zeros((_MEM, D), _F32)], axis=0).astype(_BF16)

    B = lambda c, which: {(n, c) for n in which}
    ALL = ("b1", "b2", "b3", "b4")

    with _scope("step0"):
        step(0, (0,), set(), "first")
    with _scope("step1"):
        misc["w1"].wait()
        step(1, (0,), B(0, ALL[:1]), "ahead")
    with _scope("step2"):
        for k in ("w2", "w3", "w4"):
            misc[k].wait()
        step(2, (0,), B(0, ALL), "ahead")
        misc["x1"].wait()

    def run(lo_t, hi_t, mode):
        def body(t, carry):
            step(t, (0, 1), B(0, ALL) | B(1, ALL), mode)
            return carry
        lax.fori_loop(lo_t, hi_t, body, 0)

    with _scope("loop_pre"):
        step(_LAG, (0, 1), B(0, ALL), "pre")
        step(_LAG + 1, (0, 1), B(0, ALL) | B(1, ALL[:1]), "pre")
        run(_LAG + 2, _LAG + _AHEAD, "pre")
    with _scope("loop"):
        run(_LAG + _AHEAD, n_seg, "norm")

    with _scope("tailA"):
        out_a.start()
        step(n_seg, (1,), B(0, ALL) | B(1, ALL))
        step(n_seg + 1, (1,), B(0, ALL[1:]) | B(1, ALL))
        step(n_seg + 2, (1,), B(1, ALL))
    with _scope("tailB"):
        C1 = slice(_SEG, 2 * _SEG)
        ycur = ycur_ref[C1, :]
        ncur = _ln(ycur)
        hcur = _gelu(_dot(_ln(ncur).astype(_BF16), w1_ref[...]))
        g = _token_shift(jnp.concatenate(
            [htail_ref[8:16, :], hprev_ref[C1, :], hcur, jnp.zeros((8, D), _F32)], axis=0))
        x1 = jnp.concatenate([nprev_ref[C1, :], ncur], axis=0) + _dot(g.astype(_BF16), w2_ref[...])
        f = _gelu(_dot(_ln(x1).astype(_BF16), w3_ref[...])).astype(_BF16)
        ynew = jnp.concatenate([yprev_ref[C1, :], ycur], axis=0) + x1 + _dot(f, w4_ref[...])
        o_ref[(n_seg - 2) * _SEG:n_seg * _SEG, :] = ynew.astype(o_ref.dtype)
    with _scope("out"):
        out_b.start()
        out_a.wait()
        out_b.wait()


@functools.partial(jax.jit, static_argnames=("A_seg_len",))
def pallas_interleave_layers__memory_aug_recurrent_mem_tr__mixer_s_mlp__prompt_kernel(
    A_x: jax.Array,
    A_mem0: jax.Array,
    A_Wq: jax.Array,
    A_Wk: jax.Array,
    A_Wv: jax.Array,
    A_Wo: jax.Array,
    A_seg_len,
    B_x: jax.Array,
    B_w1: jax.Array,
    B_w2: jax.Array,
    B_w3: jax.Array,
    B_w4: jax.Array,
):
    del B_x
    _, S, D = A_x.shape
    _, H, Dh = A_Wq.shape
    F = B_w3.shape[1]
    assert A_seg_len == _SEG and A_mem0.shape[1] == _MEM and A_x.shape[0] == 1
    n_seg = S // _SEG
    assert n_seg * _SEG == S and n_seg >= 2 * _LAG + 2 + _AHEAD and H % 2 == 0

    def wt(w):
        return jnp.transpose(w, (1, 2, 0)).reshape(H * Dh, D)

    R = 2 * (_MEM + _SEG)
    NP, PW = H // 2, 2 * Dh
    hbm = pl.BlockSpec(memory_space=pl.ANY)
    out = pl.pallas_call(
        functools.partial(_kernel, n_seg=n_seg, n_heads=H, d_head=Dh),
        out_shape=jax.ShapeDtypeStruct((S, D), A_x.dtype),
        in_specs=[hbm] * 10,
        out_specs=hbm,
        scratch_shapes=[
            pltpu.VMEM((S, D), _BF16),
            pltpu.VMEM((_MEM, D), _BF16),
            pltpu.VMEM((NP, D, PW), _BF16),
            pltpu.VMEM((NP, D, PW), _BF16),
            pltpu.VMEM((NP, D, PW), _BF16),
            pltpu.VMEM((H * Dh, D), _BF16),
            pltpu.VMEM((D, D), _BF16),
            pltpu.VMEM((D, D), _BF16),
            pltpu.VMEM((D, F), _BF16),
            pltpu.VMEM((F, D), _BF16),
            pltpu.VMEM((S, D), A_x.dtype),
            pltpu.VMEM((3, NP, PW, D), _BF16),
            pltpu.VMEM((R, D), _BF16),
            pltpu.VMEM((_AHEAD * _SEG + 48, D), _BF16),
            pltpu.VMEM((3, NP, (_AHEAD + _LAG - 1) * _SEG, PW), _BF16),
            pltpu.VMEM((R, D), _F32),
            pltpu.VMEM((2 * _SEG, D), _F32),
            pltpu.VMEM((2 * _SEG, D), _F32),
            pltpu.VMEM((2 * _SEG, D), _F32),
            pltpu.VMEM((2 * _SEG, D), _F32),
            pltpu.VMEM((16, D), _F32),
            pltpu.VMEM((_SEG, D), _F32),
            pltpu.SemaphoreType.DMA((4 * NP + 9,)),
        ],
        compiler_params=pltpu.CompilerParams(vmem_limit_bytes=100 * 1024 * 1024),
    )(A_x.reshape(S, D), A_mem0.reshape(_MEM, D), wt(A_Wq), wt(A_Wk), wt(A_Wv),
      A_Wo.reshape(H * Dh, D), B_w1, B_w2, B_w3, B_w4)
    return out.reshape(1, S, D)
```

```python
import contextlib
import functools

import jax
import jax.numpy as jnp
from jax import lax
import jax.experimental.pallas as pl
import jax.experimental.pallas.tpu as pltpu

_SEG = 32
_MEM = 8
_LAG = 3
_AHEAD = 9
_NEG = -1000000000.0
_EPS = 1e-05

_F32 = jnp.float32
_BF16 = jnp.bfloat16

_NT = (((1,), (1,)), ((), ()))
_NN = (((1,), (0,)), ((), ()))


_PROFILE_SCOPES = False


def _scope(name):
    return jax.named_scope(name) if _PROFILE_SCOPES else contextlib.nullcontext()


def _dot(a, b, dims=_NN):
    return lax.dot_general(a, b, dims, preferred_element_type=_F32)


def _ln(x):
    m = jnp.mean(x, axis=-1, keepdims=True)
    d = x - m
    v = jnp.mean(d * d, axis=-1, keepdims=True)
    return d * lax.rsqrt(v + _EPS)


def _gelu(x):
    return jax.nn.gelu(x, approximate=True)


def _token_shift(win):
    n, D = win.shape[0] - 16, win.shape[1]
    C = D // 4
    col = lax.broadcasted_iota(jnp.int32, (n, D), 1)
    return jnp.where(col < C, win[7:7 + n],
                     jnp.where(col < 2 * C, win[9:9 + n],
                               jnp.where(col < 3 * C, win[6:6 + n], win[10:10 + n])))


_DEFAULT_ORDER = (("q", "k", "s", "v", "b", "pv", "o"), (1, 2, 3), (1, 3, 5, 7, 9, 11, 16, 17))
_ORDERS = {
    ("norm", 2): (("q", "k", "s", "pv", "v", "b", "o"), (1, 3, 4), (2, 5, 7, 9, 10, 13, 15, 18)),
    ("pre", 2): (("q", "k", "s", "pv", "o", "v", "b"), (1, 3, 5), (0, 2, 4, 6, 8, 10, 12, 20)),
    ("ahead", 1): (("q", "o", "k", "s", "pv", "v", "b"), (1, 3, 5), (2, 3, 14, 17, 9, 11, 16, 19)),
    ("norm", 1): (("q", "k", "pv", "s", "v", "b", "o"), (1, 3, 5), (1, 4, 5, 7, 8, 11, 16, 20)),
}
_MIXER = tuple((n, c) for c in (0, 1) for n in ("b1", "b2", "b3", "b4"))


def _schedule(n_pairs, a_chains, b_stages, mode):
    key = (mode, len(a_chains))
    key_b = key + (len({c for _, c in b_stages}),)
    order, (lag_s, lag_pv, lag_o), slots = _ORDERS.get(key_b, _ORDERS.get(key, _DEFAULT_ORDER))
    scale = n_pairs / 16.0
    slots = {b: int(round(s * scale)) for b, s in zip(_MIXER, slots)}
    lag = dict(q=0, k=0, v=0, s=lag_s, pv=lag_pv, o=lag_o)
    sched = []
    for i in range(max(n_pairs + lag_o, max(slots.values()) + 1)):
        for item in order:
            if item == "b":
                sched += [b for b in _MIXER if b in b_stages and slots[b] == i]
            elif 0 <= i - lag[item] < n_pairs:
                sched.append((item, i - lag[item]))
    if mode == "first":
        last = n_pairs - 1
        for j, before in enumerate((("s", last), ("pv", last), ("o", last))):
            sched.insert(sched.index(before), ("bulk", j))
    return tuple(sched)


def _kernel(x_hbm, mem0_hbm, wqt_hbm, wkt_hbm, wvt_hbm, wo_hbm,
            w1_hbm, w2_hbm, w3_hbm, w4_hbm, o_hbm,
            x_ref, mem0_ref, wq_ref, wk_ref, wv_ref, wo_ref,
            w1_ref, w2_ref, w3_ref, w4_ref, o_ref, stage_ref,
            ha_ref, h0_ref, pre_ref, acc_ref, ycur_ref, yprev_ref, nprev_ref, hprev_ref,
            htail_ref, y2res_ref, sems, *, n_seg, n_heads, d_head):
    S, D = x_ref.shape
    PW = 2 * d_head
    n_pairs = n_heads // 2
    scale = d_head ** -0.5
    L = _MEM + _SEG
    NA = _AHEAD * _SEG
    X0 = (_AHEAD + _LAG) * _SEG

    def pair_in(p, j):
        rows = pl.ds(p * PW, PW)
        sem = sems.at[4 * p + j]
        if j < 3:
            src = (wqt_hbm, wkt_hbm, wvt_hbm)[j]
            return pltpu.make_async_copy(src.at[rows, :], stage_ref.at[j, p], sem)
        return pltpu.make_async_copy(wo_hbm.at[rows, :], wo_ref.at[rows, :], sem)

    nb = 4 * n_pairs
    misc = dict(
        x0=pltpu.make_async_copy(x_hbm.at[pl.ds(0, X0), :], x_ref.at[pl.ds(0, X0), :], sems.at[nb]),
        x1=pltpu.make_async_copy(x_hbm.at[pl.ds(X0, S - X0), :], x_ref.at[pl.ds(X0, S - X0), :],
                                 sems.at[nb + 1]),
        mem0=pltpu.make_async_copy(mem0_hbm, mem0_ref, sems.at[nb + 2]),
        w1=pltpu.make_async_copy(w1_hbm, w1_ref, sems.at[nb + 3]),
        w2=pltpu.make_async_copy(w2_hbm, w2_ref, sems.at[nb + 4]),
        w3=pltpu.make_async_copy(w3_hbm, w3_ref, sems.at[nb + 5]),
        w4=pltpu.make_async_copy(w4_hbm, w4_ref, sems.at[nb + 6]),
    )
    n_early = (n_seg - _LAG - 2) * _SEG
    out_a = pltpu.make_async_copy(o_ref.at[pl.ds(0, n_early), :], o_hbm.at[pl.ds(0, n_early), :],
                                  sems.at[nb + 7])
    out_b = pltpu.make_async_copy(o_ref.at[pl.ds(n_early, S - n_early), :],
                                  o_hbm.at[pl.ds(n_early, S - n_early), :], sems.at[nb + 8])

    def xseg(s):
        if isinstance(s, int):
            return x_ref[s * _SEG:(s + 1) * _SEG, :].astype(_F32)
        return x_ref[pl.ds(pl.multiple_of(s * _SEG, _SEG), _SEG), :].astype(_F32)

    def pick(cond, a, b):
        if isinstance(cond, bool):
            return a if cond else b()
        return jnp.where(cond, a, b())

    T1 = slice(2 * _MEM, 2 * _MEM + _SEG)
    T2 = slice(2 * _MEM + _SEG, 2 * _MEM + 2 * _SEG)

    def step(t, a_chains, b_stages, mode="norm"):
        both = len(a_chains) == 2
        first = mode == "first"
        last_pair = n_pairs - 1
        lo = lax.broadcasted_iota(jnp.int32, (L, PW), 1) < d_head
        lane = lax.broadcasted_iota(jnp.int32, (L, 2 * L), 1)
        row = lax.broadcasted_iota(jnp.int32, (L, 2 * L), 0)
        seg0 = lane < L
        key = jnp.where(seg0, lane, lane - L)
        allowed = (row < _MEM) | (row >= key)

        st = {}

        def blockdiag(a):
            zero = jnp.zeros_like(a)
            return jnp.concatenate([jnp.where(lo, a, zero), jnp.where(lo, zero, a)],
                                   axis=0).astype(_BF16)

        if len(a_chains) == 1:
            c0 = a_chains[0]
            h32 = jnp.concatenate(
                [ha_ref[_MEM * c0:_MEM * (c0 + 1), :].astype(_F32),
                 ha_ref[(T1, T2)[c0], :].astype(_F32)], axis=0)

        def pre_at(j, p, s):
            if isinstance(s, int):
                return pre_ref.at[j, p, (s - 1) * _SEG:s * _SEG, :]
            return pre_ref.at[j, p, pl.ds(pl.multiple_of((s - 1) * _SEG, _SEG), _SEG), :]

        def proj(p, j):
            w_ref = (wq_ref, wk_ref, wv_ref)[j]
            if first:
                if j == 0:
                    for jj in range(3):
                        pair_in(p, jj).wait()
                    if p > 0:
                        pair_in(p - 1, 3).wait()
                wt = stage_ref[j, p]
                w_ref[p] = wt.T
                if p == last_pair:
                    return {0: _dot(h32, wt, _NT)}
                res = _dot(h0_ref[...], wt, _NT)
                pre_ref[j, p, 0:NA, :] = res[0:NA].astype(_BF16)
                return {0: res[NA:NA + L]}
            if mode == "ahead":
                res = _dot(h32, w_ref[p])
                pre_at(j, p, t + _AHEAD)[...] = res[_MEM:L].astype(_BF16)
                return {0: jnp.concatenate([res[0:_MEM], pre_at(j, p, t)[...].astype(_F32)], axis=0)}
            if mode == "pre":
                h = jnp.concatenate([ha_ref[0:2 * _MEM, :], ha_ref[T2, :]], axis=0)
                res = _dot(h, w_ref[p])
                return {0: jnp.concatenate([res[0:_MEM], pre_at(j, p, t)[...].astype(_F32)], axis=0),
                        1: res[_MEM:_MEM + L]}
            if both:
                res = _dot(ha_ref[...], w_ref[p])
                return {c: jnp.concatenate([res[_MEM * c:_MEM * (c + 1)], res[(T1, T2)[c]]], axis=0)
                        for c in (0, 1)}
            return {c0: _dot(h32, w_ref[p])}

        def bulk(j):
            wt = stage_ref[j, last_pair]
            pre_ref[j, last_pair, 0:NA, :] = _dot(h0_ref[0:NA, :], wt, _NT).astype(_BF16)

        def a_q(p):
            st["q", p] = proj(p, 0)

        def a_k(p):
            st["k", p] = proj(p, 1)

        def a_v(p):
            st["v", p] = proj(p, 2)

        def a_s(p):
            q, k = st.pop(("q", p)), st.pop(("k", p))
            for c in a_chains:
                s = _dot(q[c], blockdiag(k[c]), _NT) * scale
                s = jnp.where(allowed, s, _NEG)
                m0 = jnp.max(jnp.where(seg0, s, -jnp.inf), axis=1, keepdims=True)
                m1 = jnp.max(jnp.where(seg0, -jnp.inf, s), axis=1, keepdims=True)
                e = jnp.exp(s - jnp.where(seg0, m0, m1))
                l0 = jnp.sum(jnp.where(seg0, e, 0.0), axis=1, keepdims=True)
                l1 = jnp.sum(jnp.where(seg0, 0.0, e), axis=1, keepdims=True)
                st["p", p, c] = e / jnp.where(seg0, l0, l1)

        def a_pv(p):
            v = st.pop(("v", p))
            outs = [_dot(st.pop(("p", p, c)), blockdiag(v[c])) for c in a_chains]
            if both:
                st["o", p] = jnp.concatenate(
                    [outs[0][:_MEM], outs[1][:_MEM], outs[0][_MEM:], outs[1][_MEM:]],
                    axis=0).astype(_BF16)
            else:
                st["o", p] = outs[0]

        def a_o(p):
            if first and p == last_pair:
                pair_in(p, 3).wait()
            part = _dot(st.pop(("o", p)), wo_ref[p * PW:(p + 1) * PW, :])
            n = part.shape[0]
            if p == 0:
                acc_ref[0:n, :] = part
            elif p < n_pairs - 1:
                acc_ref[0:n, :] += part
            else:
                st["acc"] = acc_ref[0:n, :] + part

        def rs(c):
            return slice(_SEG * c, _SEG * (c + 1))

        def rotate(c):
            htail_ref[8 * c:8 * c + 8, :] = hprev_ref[_SEG * (c + 1) - 8:_SEG * (c + 1), :]
            hprev_ref[rs(c), :] = st.pop(("h", c))
            nprev_ref[rs(c), :] = st.pop(("ncur", c))
            yprev_ref[rs(c), :] = st.pop(("ycur", c))

        def b_1(c):
            ycur = ycur_ref[rs(c), :]
            ncur = _ln(ycur)
            st["ycur", c], st["ncur", c] = ycur, ncur
            st["h", c] = _gelu(_dot(_ln(ncur).astype(_BF16), w1_ref[...]))
            if ("b2", c) not in b_stages:
                rotate(c)

        def b_2(c):
            s = t - 2 - _LAG * c
            hprev = hprev_ref[rs(c), :]
            pt = pick(s == 0, jnp.zeros((8, D), _F32), lambda: htail_ref[8 * c:8 * c + 8, :])
            nh = pick(s == n_seg - 1, jnp.zeros((8, D), _F32), lambda: st["h", c][0:8])
            g = _token_shift(jnp.concatenate([pt, hprev, nh], axis=0))
            st["x1", c] = nprev_ref[rs(c), :] + _dot(g.astype(_BF16), w2_ref[...])
            st["yres", c] = yprev_ref[rs(c), :]
            if ("b1", c) in b_stages:
                rotate(c)

        def b_3(c):
            st["f", c] = _gelu(_dot(_ln(st["x1", c]).astype(_BF16), w3_ref[...])).astype(_BF16)

        def b_4(c):
            ynew = st.pop(("yres", c)) + st.pop(("x1", c)) + _dot(st.pop(("f", c)), w4_ref[...])
            if c == 0:
                st["y2new"] = ynew
                st["tok2"] = _ln(ynew).astype(_BF16)
            else:
                so = t - 2 - _LAG
                if isinstance(so, int):
                    o_ref[so * _SEG:(so + 1) * _SEG, :] = ynew.astype(o_ref.dtype)
                else:
                    o_ref[pl.ds(pl.multiple_of(so * _SEG, _SEG), _SEG), :] = ynew.astype(o_ref.dtype)

        stages = dict(q=a_q, k=a_k, v=a_v, s=a_s, pv=a_pv, o=a_o, bulk=bulk,
                      b1=b_1, b2=b_2, b3=b_3, b4=b_4)
        for name, arg in _schedule(n_pairs, a_chains, b_stages, mode):
            stages[name](arg)

        if "tok2" in st:
            ha_ref[T2, :] = st.pop("tok2")
        if a_chains:
            acc = st.pop("acc")
            if both:
                mem1, mem2 = acc[0:_MEM], acc[_MEM:2 * _MEM]
                a1, a2 = acc[T1], acc[T2]
            elif a_chains == (0,):
                mem1, mem2 = acc[0:_MEM], mem0_ref[...].astype(_F32)
                a1, a2 = acc[_MEM:L], None
            else:
                mem1, mem2 = mem0_ref[...].astype(_F32), acc[0:_MEM]
                a1, a2 = None, acc[_MEM:L]
            ha_ref[0:2 * _MEM, :] = jnp.concatenate([mem1, mem2], axis=0).astype(_BF16)
            if a1 is not None:
                if isinstance(t, int):
                    nxt = t + 1 + _AHEAD if t + 1 < _LAG else min(t + 1, n_seg - 1)
                else:
                    nxt = jnp.minimum(t + 1, n_seg - 1)
                ha_ref[T1, :] = _ln(xseg(nxt)).astype(_BF16)
                ycur_ref[0:_SEG, :] = xseg(t) + a1
            if a2 is not None:
                ycur_ref[_SEG:, :] = y2res_ref[...] + a2
        if "y2new" in st:
            y2res_ref[...] = st.pop("y2new")
        assert not st, list(st)

    misc["x0"].start()
    misc["mem0"].start()
    for p in range(n_pairs):
        for j in range(4):
            pair_in(p, j).start()
    for k in ("w1", "w2", "w3", "w4", "x1"):
        misc[k].start()
    for r in (ycur_ref, yprev_ref, nprev_ref, hprev_ref, htail_ref, y2res_ref):
        r[...] = jnp.zeros(r.shape, _F32)
    misc["x0"].wait()
    misc["mem0"].wait()
    mem0 = mem0_ref[...]
    ha_ref[0:2 * _MEM, :] = jnp.concatenate([mem0, mem0], axis=0).astype(_BF16)
    n0 = _ln(xseg(0))
    ha_ref[T1, :] = n0.astype(_BF16)
    ha_ref[T2, :] = jnp.zeros((_SEG, D), _BF16)
    for s in range(1, _AHEAD + 1):
        h0_ref[(s - 1) * _SEG:s * _SEG, :] = _ln(xseg(s)).astype(_BF16)
    h0_ref[NA:NA + L + _MEM, :] = jnp.concatenate(
        [mem0.astype(_F32), n0, jnp.zeros((_MEM, D), _F32)], axis=0).astype(_BF16)

    B = lambda c, which: {(n, c) for n in which}
    ALL = ("b1", "b2", "b3", "b4")

    with _scope("step0"):
        step(0, (0,), set(), "first")
    with _scope("step1"):
        misc["w1"].wait()
        step(1, (0,), B(0, ALL[:1]), "ahead")
    with _scope("step2"):
        for k in ("w2", "w3", "w4"):
            misc[k].wait()
        step(2, (0,), B(0, ALL), "ahead")
        misc["x1"].wait()

    def run(lo_t, hi_t, mode):
        def body(t, carry):
            step(t, (0, 1), B(0, ALL) | B(1, ALL), mode)
            return carry
        lax.fori_loop(lo_t, hi_t, body, 0)

    with _scope("loop_pre"):
        step(_LAG, (0, 1), B(0, ALL), "pre")
        step(_LAG + 1, (0, 1), B(0, ALL) | B(1, ALL[:1]), "pre")
        run(_LAG + 2, _LAG + _AHEAD, "pre")
    with _scope("loop"):
        run(_LAG + _AHEAD, n_seg, "norm")

    with _scope("tailA"):
        out_a.start()
        step(n_seg, (1,), B(0, ALL) | B(1, ALL))
        step(n_seg + 1, (1,), B(0, ALL[1:]) | B(1, ALL))
        step(n_seg + 2, (1,), B(1, ALL))
    with _scope("tailB"):
        C1 = slice(_SEG, 2 * _SEG)
        ycur = ycur_ref[C1, :]
        ncur = _ln(ycur)
        hcur = _gelu(_dot(_ln(ncur).astype(_BF16), w1_ref[...]))
        g = _token_shift(jnp.concatenate(
            [htail_ref[8:16, :], hprev_ref[C1, :], hcur, jnp.zeros((8, D), _F32)], axis=0))
        x1 = jnp.concatenate([nprev_ref[C1, :], ncur], axis=0) + _dot(g.astype(_BF16), w2_ref[...])
        f = _gelu(_dot(_ln(x1).astype(_BF16), w3_ref[...])).astype(_BF16)
        ynew = jnp.concatenate([yprev_ref[C1, :], ycur], axis=0) + x1 + _dot(f, w4_ref[...])
        o_ref[(n_seg - 2) * _SEG:n_seg * _SEG, :] = ynew.astype(o_ref.dtype)
    with _scope("out"):
        out_b.start()
        out_a.wait()
        out_b.wait()


@functools.partial(jax.jit, static_argnames=("A_seg_len",))
def pallas_interleave_layers__memory_aug_recurrent_mem_tr__mixer_s_mlp__prompt_kernel(
    A_x: jax.Array,
    A_mem0: jax.Array,
    A_Wq: jax.Array,
    A_Wk: jax.Array,
    A_Wv: jax.Array,
    A_Wo: jax.Array,
    A_seg_len,
    B_x: jax.Array,
    B_w1: jax.Array,
    B_w2: jax.Array,
    B_w3: jax.Array,
    B_w4: jax.Array,
):
    del B_x
    _, S, D = A_x.shape
    _, H, Dh = A_Wq.shape
    F = B_w3.shape[1]
    assert A_seg_len == _SEG and A_mem0.shape[1] == _MEM and A_x.shape[0] == 1
    n_seg = S // _SEG
    assert n_seg * _SEG == S and n_seg >= 2 * _LAG + 2 + _AHEAD and H % 2 == 0

    def wt(w):
        return jnp.transpose(w, (1, 2, 0)).reshape(H * Dh, D)

    R = 2 * (_MEM + _SEG)
    NP, PW = H // 2, 2 * Dh
    hbm = pl.BlockSpec(memory_space=pl.ANY)
    out = pl.pallas_call(
        functools.partial(_kernel, n_seg=n_seg, n_heads=H, d_head=Dh),
        out_shape=jax.ShapeDtypeStruct((S, D), A_x.dtype),
        in_specs=[hbm] * 10,
        out_specs=hbm,
        scratch_shapes=[
            pltpu.VMEM((S, D), _BF16),
            pltpu.VMEM((_MEM, D), _BF16),
            pltpu.VMEM((NP, D, PW), _BF16),
            pltpu.VMEM((NP, D, PW), _BF16),
            pltpu.VMEM((NP, D, PW), _BF16),
            pltpu.VMEM((H * Dh, D), _BF16),
            pltpu.VMEM((D, D), _BF16),
            pltpu.VMEM((D, D), _BF16),
            pltpu.VMEM((D, F), _BF16),
            pltpu.VMEM((F, D), _BF16),
            pltpu.VMEM((S, D), A_x.dtype),
            pltpu.VMEM((3, NP, PW, D), _BF16),
            pltpu.VMEM((R, D), _BF16),
            pltpu.VMEM((_AHEAD * _SEG + 48, D), _BF16),
            pltpu.VMEM((3, NP, (_AHEAD + _LAG - 1) * _SEG, PW), _BF16),
            pltpu.VMEM((R, D), _F32),
            pltpu.VMEM((2 * _SEG, D), _F32),
            pltpu.VMEM((2 * _SEG, D), _F32),
            pltpu.VMEM((2 * _SEG, D), _F32),
            pltpu.VMEM((2 * _SEG, D), _F32),
            pltpu.VMEM((16, D), _F32),
            pltpu.VMEM((_SEG, D), _F32),
            pltpu.SemaphoreType.DMA((4 * NP + 9,)),
        ],
        compiler_params=pltpu.CompilerParams(vmem_limit_bytes=100 * 1024 * 1024),
    )(A_x.reshape(S, D), A_mem0.reshape(_MEM, D), wt(A_Wq), wt(A_Wk), wt(A_Wv),
      A_Wo.reshape(H * Dh, D), B_w1, B_w2, B_w3, B_w4)
    return out.reshape(1, S, D)
```

```python
import contextlib
import functools

import jax
import jax.numpy as jnp
from jax import lax
import jax.experimental.pallas as pl
import jax.experimental.pallas.tpu as pltpu

_SEG = 32
_MEM = 8
_LAG = 3
_AHEAD = 9
_WO_LAG = 3
_NEG = -1000000000.0
_EPS = 1e-05

_F32 = jnp.float32
_BF16 = jnp.bfloat16

_NT = (((1,), (1,)), ((), ()))
_NN = (((1,), (0,)), ((), ()))


_PROFILE_SCOPES = False


def _scope(name):
    return jax.named_scope(name) if _PROFILE_SCOPES else contextlib.nullcontext()


def _dot(a, b, dims=_NN):
    return lax.dot_general(a, b, dims, preferred_element_type=_F32)


def _ln(x):
    m = jnp.mean(x, axis=-1, keepdims=True)
    d = x - m
    v = jnp.mean(d * d, axis=-1, keepdims=True)
    return d * lax.rsqrt(v + _EPS)


def _gelu(x):
    return jax.nn.gelu(x, approximate=True)


def _token_shift(win):
    n, D = win.shape[0] - 16, win.shape[1]
    C = D // 4
    col = lax.broadcasted_iota(jnp.int32, (n, D), 1)
    return jnp.where(col < C, win[7:7 + n],
                     jnp.where(col < 2 * C, win[9:9 + n],
                               jnp.where(col < 3 * C, win[6:6 + n], win[10:10 + n])))


_DEFAULT_ORDER = (("q", "k", "s", "v", "b", "pv", "o"), (1, 2, 3), (1, 3, 5, 7, 9, 11, 16, 17))
_ORDERS = {
    ("norm", 2): (("q", "k", "s", "pv", "v", "b", "o"), (1, 3, 4), (2, 5, 7, 9, 10, 13, 15, 18)),
    ("pre", 2): (("q", "k", "s", "pv", "o", "v", "b"), (1, 3, 5), (0, 2, 4, 6, 8, 10, 12, 20)),
    ("ahead", 1): (("q", "o", "k", "s", "pv", "v", "b"), (1, 3, 5), (2, 3, 14, 17, 9, 11, 16, 19)),
    ("norm", 1): (("q", "k", "pv", "s", "v", "b", "o"), (1, 3, 5), (1, 4, 5, 7, 8, 11, 16, 20)),
}
_MIXER = tuple((n, c) for c in (0, 1) for n in ("b1", "b2", "b3", "b4"))


def _schedule(n_pairs, a_chains, b_stages, mode):
    key = (mode, len(a_chains))
    key_b = key + (len({c for _, c in b_stages}),)
    order, (lag_s, lag_pv, lag_o), slots = _ORDERS.get(key_b, _ORDERS.get(key, _DEFAULT_ORDER))
    scale = n_pairs / 16.0
    slots = {b: int(round(s * scale)) for b, s in zip(_MIXER, slots)}
    lag = dict(q=0, k=0, v=0, s=lag_s, pv=lag_pv, o=lag_o)
    sched = []
    for i in range(max(n_pairs + lag_o, max(slots.values()) + 1)):
        for item in order:
            if item == "b":
                sched += [b for b in _MIXER if b in b_stages and slots[b] == i]
            elif 0 <= i - lag[item] < n_pairs:
                sched.append((item, i - lag[item]))
    if mode == "first":
        assert lag_o >= _WO_LAG and order.index("q") < order.index("o")
        last = n_pairs - 1
        for j, before in enumerate((("s", last), ("pv", last), ("o", last))):
            sched.insert(sched.index(before), ("bulk", j))
    return tuple(sched)


def _kernel(x_hbm, mem0_hbm, wqt_hbm, wkt_hbm, wvt_hbm, wo_hbm,
            w1_hbm, w2_hbm, w3_hbm, w4_hbm, o_hbm,
            x_ref, mem0_ref, wq_ref, wk_ref, wv_ref, wo_ref,
            w1_ref, w2_ref, w3_ref, w4_ref, o_ref, stage_ref,
            ha_ref, h0_ref, pre_ref, acc_ref, ycur_ref, yprev_ref, nprev_ref, hprev_ref,
            htail_ref, y2res_ref, sems, *, n_seg, n_heads, d_head):
    S, D = x_ref.shape
    PW = 2 * d_head
    n_pairs = n_heads // 2
    scale = d_head ** -0.5
    L = _MEM + _SEG
    NA = _AHEAD * _SEG
    X0 = (_AHEAD + _LAG) * _SEG

    def pair_in(p, j):
        rows = pl.ds(p * PW, PW)
        sem = sems.at[4 * p + j]
        if j < 3:
            src = (wqt_hbm, wkt_hbm, wvt_hbm)[j]
            return pltpu.make_async_copy(src.at[rows, :], stage_ref.at[j, p], sem)
        return pltpu.make_async_copy(wo_hbm.at[rows, :], wo_ref.at[rows, :], sem)

    nb = 4 * n_pairs
    misc = dict(
        x0=pltpu.make_async_copy(x_hbm.at[pl.ds(0, X0), :], x_ref.at[pl.ds(0, X0), :], sems.at[nb]),
        x1=pltpu.make_async_copy(x_hbm.at[pl.ds(X0, S - X0), :], x_ref.at[pl.ds(X0, S - X0), :],
                                 sems.at[nb + 1]),
        mem0=pltpu.make_async_copy(mem0_hbm, mem0_ref, sems.at[nb + 2]),
        w1=pltpu.make_async_copy(w1_hbm, w1_ref, sems.at[nb + 3]),
        w2=pltpu.make_async_copy(w2_hbm, w2_ref, sems.at[nb + 4]),
        w3=pltpu.make_async_copy(w3_hbm, w3_ref, sems.at[nb + 5]),
        w4=pltpu.make_async_copy(w4_hbm, w4_ref, sems.at[nb + 6]),
    )
    n_early = (n_seg - _LAG - 2) * _SEG
    out_a = pltpu.make_async_copy(o_ref.at[pl.ds(0, n_early), :], o_hbm.at[pl.ds(0, n_early), :],
                                  sems.at[nb + 7])
    out_b = pltpu.make_async_copy(o_ref.at[pl.ds(n_early, S - n_early), :],
                                  o_hbm.at[pl.ds(n_early, S - n_early), :], sems.at[nb + 8])

    def xseg(s):
        if isinstance(s, int):
            return x_ref[s * _SEG:(s + 1) * _SEG, :].astype(_F32)
        return x_ref[pl.ds(pl.multiple_of(s * _SEG, _SEG), _SEG), :].astype(_F32)

    def pick(cond, a, b):
        if isinstance(cond, bool):
            return a if cond else b()
        return jnp.where(cond, a, b())

    T1 = slice(2 * _MEM, 2 * _MEM + _SEG)
    T2 = slice(2 * _MEM + _SEG, 2 * _MEM + 2 * _SEG)

    def step(t, a_chains, b_stages, mode="norm"):
        both = len(a_chains) == 2
        first = mode == "first"
        last_pair = n_pairs - 1
        lo = lax.broadcasted_iota(jnp.int32, (L, PW), 1) < d_head
        lane = lax.broadcasted_iota(jnp.int32, (L, 2 * L), 1)
        row = lax.broadcasted_iota(jnp.int32, (L, 2 * L), 0)
        seg0 = lane < L
        key = jnp.where(seg0, lane, lane - L)
        allowed = (row < _MEM) | (row >= key)

        st = {}

        def blockdiag(a):
            zero = jnp.zeros_like(a)
            return jnp.concatenate([jnp.where(lo, a, zero), jnp.where(lo, zero, a)],
                                   axis=0).astype(_BF16)

        if len(a_chains) == 1:
            c0 = a_chains[0]
            h32 = jnp.concatenate(
                [ha_ref[_MEM * c0:_MEM * (c0 + 1), :].astype(_F32),
                 ha_ref[(T1, T2)[c0], :].astype(_F32)], axis=0)

        def pre_at(j, p, s):
            if isinstance(s, int):
                return pre_ref.at[j, p, (s - 1) * _SEG:s * _SEG, :]
            return pre_ref.at[j, p, pl.ds(pl.multiple_of((s - 1) * _SEG, _SEG), _SEG), :]

        def proj(p, j):
            w_ref = (wq_ref, wk_ref, wv_ref)[j]
            if first:
                if p == 0 and j < 2:
                    for jj in ((0,), (1, 2))[j]:
                        pair_in(0, jj).wait()
                elif p > 0 and j == 0:
                    for jj in range(3):
                        pair_in(p, jj).wait()
                    if p >= _WO_LAG:
                        pair_in(p - _WO_LAG, 3).wait()
                wt = stage_ref[j, p]
                w_ref[p] = wt.T
                if p == last_pair:
                    return {0: _dot(h32, wt, _NT)}
                res = _dot(h0_ref[...], wt, _NT)
                pre_ref[j, p, 0:NA, :] = res[0:NA].astype(_BF16)
                return {0: res[NA:NA + L]}
            if mode == "ahead":
                res = _dot(h32, w_ref[p])
                pre_at(j, p, t + _AHEAD)[...] = res[_MEM:L].astype(_BF16)
                return {0: jnp.concatenate([res[0:_MEM], pre_at(j, p, t)[...].astype(_F32)], axis=0)}
            if mode == "pre":
                h = jnp.concatenate([ha_ref[0:2 * _MEM, :], ha_ref[T2, :]], axis=0)
                res = _dot(h, w_ref[p])
                return {0: jnp.concatenate([res[0:_MEM], pre_at(j, p, t)[...].astype(_F32)], axis=0),
                        1: res[_MEM:_MEM + L]}
            if both:
                res = _dot(ha_ref[...], w_ref[p])
                return {c: jnp.concatenate([res[_MEM * c:_MEM * (c + 1)], res[(T1, T2)[c]]], axis=0)
                        for c in (0, 1)}
            return {c0: _dot(h32, w_ref[p])}

        def bulk(j):
            wt = stage_ref[j, last_pair]
            pre_ref[j, last_pair, 0:NA, :] = _dot(h0_ref[0:NA, :], wt, _NT).astype(_BF16)

        def a_q(p):
            st["q", p] = proj(p, 0)

        def a_k(p):
            st["k", p] = proj(p, 1)

        def a_v(p):
            st["v", p] = proj(p, 2)

        def a_s(p):
            q, k = st.pop(("q", p)), st.pop(("k", p))
            for c in a_chains:
                s = _dot(q[c], blockdiag(k[c]), _NT) * scale
                s = jnp.where(allowed, s, _NEG)
                m0 = jnp.max(jnp.where(seg0, s, -jnp.inf), axis=1, keepdims=True)
                m1 = jnp.max(jnp.where(seg0, -jnp.inf, s), axis=1, keepdims=True)
                e = jnp.exp(s - jnp.where(seg0, m0, m1))
                l0 = jnp.sum(jnp.where(seg0, e, 0.0), axis=1, keepdims=True)
                l1 = jnp.sum(jnp.where(seg0, 0.0, e), axis=1, keepdims=True)
                st["p", p, c] = e / jnp.where(seg0, l0, l1)

        def a_pv(p):
            v = st.pop(("v", p))
            outs = [_dot(st.pop(("p", p, c)), blockdiag(v[c])) for c in a_chains]
            if both:
                st["o", p] = jnp.concatenate(
                    [outs[0][:_MEM], outs[1][:_MEM], outs[0][_MEM:], outs[1][_MEM:]],
                    axis=0).astype(_BF16)
            else:
                st["o", p] = outs[0]

        def a_o(p):
            if first and p == n_pairs - _WO_LAG:
                for q in range(p, n_pairs):
                    pair_in(q, 3).wait()
            part = _dot(st.pop(("o", p)), wo_ref[p * PW:(p + 1) * PW, :])
            n = part.shape[0]
            if p == 0:
                acc_ref[0:n, :] = part
            elif p < n_pairs - 1:
                acc_ref[0:n, :] += part
            else:
                st["acc"] = acc_ref[0:n, :] + part

        def rs(c):
            return slice(_SEG * c, _SEG * (c + 1))

        def rotate(c):
            htail_ref[8 * c:8 * c + 8, :] = hprev_ref[_SEG * (c + 1) - 8:_SEG * (c + 1), :]
            hprev_ref[rs(c), :] = st.pop(("h", c))
            nprev_ref[rs(c), :] = st.pop(("ncur", c))
            yprev_ref[rs(c), :] = st.pop(("ycur", c))

        def b_1(c):
            ycur = ycur_ref[rs(c), :]
            ncur = _ln(ycur)
            st["ycur", c], st["ncur", c] = ycur, ncur
            st["h", c] = _gelu(_dot(_ln(ncur).astype(_BF16), w1_ref[...]))
            if ("b2", c) not in b_stages:
                rotate(c)

        def b_2(c):
            s = t - 2 - _LAG * c
            hprev = hprev_ref[rs(c), :]
            pt = pick(s == 0, jnp.zeros((8, D), _F32), lambda: htail_ref[8 * c:8 * c + 8, :])
            nh = pick(s == n_seg - 1, jnp.zeros((8, D), _F32), lambda: st["h", c][0:8])
            g = _token_shift(jnp.concatenate([pt, hprev, nh], axis=0))
            st["x1", c] = nprev_ref[rs(c), :] + _dot(g.astype(_BF16), w2_ref[...])
            st["yres", c] = yprev_ref[rs(c), :]
            if ("b1", c) in b_stages:
                rotate(c)

        def b_3(c):
            st["f", c] = _gelu(_dot(_ln(st["x1", c]).astype(_BF16), w3_ref[...])).astype(_BF16)

        def b_4(c):
            ynew = st.pop(("yres", c)) + st.pop(("x1", c)) + _dot(st.pop(("f", c)), w4_ref[...])
            if c == 0:
                st["y2new"] = ynew
                st["tok2"] = _ln(ynew).astype(_BF16)
            else:
                so = t - 2 - _LAG
                if isinstance(so, int):
                    o_ref[so * _SEG:(so + 1) * _SEG, :] = ynew.astype(o_ref.dtype)
                else:
                    o_ref[pl.ds(pl.multiple_of(so * _SEG, _SEG), _SEG), :] = ynew.astype(o_ref.dtype)

        stages = dict(q=a_q, k=a_k, v=a_v, s=a_s, pv=a_pv, o=a_o, bulk=bulk,
                      b1=b_1, b2=b_2, b3=b_3, b4=b_4)
        for name, arg in _schedule(n_pairs, a_chains, b_stages, mode):
            stages[name](arg)

        if "tok2" in st:
            ha_ref[T2, :] = st.pop("tok2")
        if a_chains:
            acc = st.pop("acc")
            if both:
                mem1, mem2 = acc[0:_MEM], acc[_MEM:2 * _MEM]
                a1, a2 = acc[T1], acc[T2]
            elif a_chains == (0,):
                mem1, mem2 = acc[0:_MEM], mem0_ref[...].astype(_F32)
                a1, a2 = acc[_MEM:L], None
            else:
                mem1, mem2 = mem0_ref[...].astype(_F32), acc[0:_MEM]
                a1, a2 = None, acc[_MEM:L]
            ha_ref[0:2 * _MEM, :] = jnp.concatenate([mem1, mem2], axis=0).astype(_BF16)
            if a1 is not None:
                if isinstance(t, int):
                    nxt = t + 1 + _AHEAD if t + 1 < _LAG else min(t + 1, n_seg - 1)
                else:
                    nxt = jnp.minimum(t + 1, n_seg - 1)
                ha_ref[T1, :] = _ln(xseg(nxt)).astype(_BF16)
                ycur_ref[0:_SEG, :] = xseg(t) + a1
            if a2 is not None:
                ycur_ref[_SEG:, :] = y2res_ref[...] + a2
        if "y2new" in st:
            y2res_ref[...] = st.pop("y2new")
        assert not st, list(st)

    misc["x0"].start()
    misc["mem0"].start()
    for p in range(n_pairs + _WO_LAG):
        for j in range(3):
            if p < n_pairs:
                pair_in(p, j).start()
        if p >= _WO_LAG:
            pair_in(p - _WO_LAG, 3).start()
    for k in ("w1", "w2", "w3", "w4", "x1"):
        misc[k].start()
    for r in (ycur_ref, yprev_ref, nprev_ref, hprev_ref, htail_ref, y2res_ref):
        r[...] = jnp.zeros(r.shape, _F32)
    misc["x0"].wait()
    misc["mem0"].wait()
    mem0 = mem0_ref[...]
    ha_ref[0:2 * _MEM, :] = jnp.concatenate([mem0, mem0], axis=0).astype(_BF16)
    n0 = _ln(xseg(0))
    ha_ref[T1, :] = n0.astype(_BF16)
    ha_ref[T2, :] = jnp.zeros((_SEG, D), _BF16)
    for s in range(1, _AHEAD + 1):
        h0_ref[(s - 1) * _SEG:s * _SEG, :] = _ln(xseg(s)).astype(_BF16)
    h0_ref[NA:NA + L + _MEM, :] = jnp.concatenate(
        [mem0.astype(_F32), n0, jnp.zeros((_MEM, D), _F32)], axis=0).astype(_BF16)

    B = lambda c, which: {(n, c) for n in which}
    ALL = ("b1", "b2", "b3", "b4")

    with _scope("step0"):
        step(0, (0,), set(), "first")
    with _scope("step1"):
        misc["w1"].wait()
        step(1, (0,), B(0, ALL[:1]), "ahead")
    with _scope("step2"):
        for k in ("w2", "w3", "w4"):
            misc[k].wait()
        step(2, (0,), B(0, ALL), "ahead")
        misc["x1"].wait()

    def run(lo_t, hi_t, mode):
        def body(t, carry):
            step(t, (0, 1), B(0, ALL) | B(1, ALL), mode)
            return carry
        lax.fori_loop(lo_t, hi_t, body, 0)

    with _scope("loop_pre"):
        step(_LAG, (0, 1), B(0, ALL), "pre")
        step(_LAG + 1, (0, 1), B(0, ALL) | B(1, ALL[:1]), "pre")
        run(_LAG + 2, _LAG + _AHEAD, "pre")
    with _scope("loop"):
        run(_LAG + _AHEAD, n_seg, "norm")

    with _scope("tailA"):
        out_a.start()
        step(n_seg, (1,), B(0, ALL) | B(1, ALL))
        step(n_seg + 1, (1,), B(0, ALL[1:]) | B(1, ALL))
        step(n_seg + 2, (1,), B(1, ALL))
    with _scope("tailB"):
        C1 = slice(_SEG, 2 * _SEG)
        ycur = ycur_ref[C1, :]
        ncur = _ln(ycur)
        hcur = _gelu(_dot(_ln(ncur).astype(_BF16), w1_ref[...]))
        g = _token_shift(jnp.concatenate(
            [htail_ref[8:16, :], hprev_ref[C1, :], hcur, jnp.zeros((8, D), _F32)], axis=0))
        x1 = jnp.concatenate([nprev_ref[C1, :], ncur], axis=0) + _dot(g.astype(_BF16), w2_ref[...])
        f = _gelu(_dot(_ln(x1).astype(_BF16), w3_ref[...])).astype(_BF16)
        ynew = jnp.concatenate([yprev_ref[C1, :], ycur], axis=0) + x1 + _dot(f, w4_ref[...])
        o_ref[(n_seg - 2) * _SEG:n_seg * _SEG, :] = ynew.astype(o_ref.dtype)
    with _scope("out"):
        out_b.start()
        out_a.wait()
        out_b.wait()


@functools.partial(jax.jit, static_argnames=("A_seg_len",))
def pallas_interleave_layers__memory_aug_recurrent_mem_tr__mixer_s_mlp__prompt_kernel(
    A_x: jax.Array,
    A_mem0: jax.Array,
    A_Wq: jax.Array,
    A_Wk: jax.Array,
    A_Wv: jax.Array,
    A_Wo: jax.Array,
    A_seg_len,
    B_x: jax.Array,
    B_w1: jax.Array,
    B_w2: jax.Array,
    B_w3: jax.Array,
    B_w4: jax.Array,
):
    del B_x
    _, S, D = A_x.shape
    _, H, Dh = A_Wq.shape
    F = B_w3.shape[1]
    assert A_seg_len == _SEG and A_mem0.shape[1] == _MEM and A_x.shape[0] == 1
    n_seg = S // _SEG
    assert n_seg * _SEG == S and n_seg >= 2 * _LAG + 2 + _AHEAD and H % 2 == 0

    def wt(w):
        return jnp.transpose(w, (1, 2, 0)).reshape(H * Dh, D)

    R = 2 * (_MEM + _SEG)
    NP, PW = H // 2, 2 * Dh
    hbm = pl.BlockSpec(memory_space=pl.ANY)
    out = pl.pallas_call(
        functools.partial(_kernel, n_seg=n_seg, n_heads=H, d_head=Dh),
        out_shape=jax.ShapeDtypeStruct((S, D), A_x.dtype),
        in_specs=[hbm] * 10,
        out_specs=hbm,
        scratch_shapes=[
            pltpu.VMEM((S, D), _BF16),
            pltpu.VMEM((_MEM, D), _BF16),
            pltpu.VMEM((NP, D, PW), _BF16),
            pltpu.VMEM((NP, D, PW), _BF16),
            pltpu.VMEM((NP, D, PW), _BF16),
            pltpu.VMEM((H * Dh, D), _BF16),
            pltpu.VMEM((D, D), _BF16),
            pltpu.VMEM((D, D), _BF16),
            pltpu.VMEM((D, F), _BF16),
            pltpu.VMEM((F, D), _BF16),
            pltpu.VMEM((S, D), A_x.dtype),
            pltpu.VMEM((3, NP, PW, D), _BF16),
            pltpu.VMEM((R, D), _BF16),
            pltpu.VMEM((_AHEAD * _SEG + 48, D), _BF16),
            pltpu.VMEM((3, NP, (_AHEAD + _LAG - 1) * _SEG, PW), _BF16),
            pltpu.VMEM((R, D), _F32),
            pltpu.VMEM((2 * _SEG, D), _F32),
            pltpu.VMEM((2 * _SEG, D), _F32),
            pltpu.VMEM((2 * _SEG, D), _F32),
            pltpu.VMEM((2 * _SEG, D), _F32),
            pltpu.VMEM((16, D), _F32),
            pltpu.VMEM((_SEG, D), _F32),
            pltpu.SemaphoreType.DMA((4 * NP + 9,)),
        ],
        compiler_params=pltpu.CompilerParams(vmem_limit_bytes=100 * 1024 * 1024),
    )(A_x.reshape(S, D), A_mem0.reshape(_MEM, D), wt(A_Wq), wt(A_Wk), wt(A_Wv),
      A_Wo.reshape(H * Dh, D), B_w1, B_w2, B_w3, B_w4)
    return out.reshape(1, S, D)
```

```python
import contextlib
import functools

import jax
import jax.numpy as jnp
from jax import lax
import jax.experimental.pallas as pl
import jax.experimental.pallas.tpu as pltpu

_SEG = 32
_MEM = 8
_LAG = 3
_AHEAD = 9
_WO_LAG = 3
_NEG = -1000000000.0
_EPS = 1e-05

_F32 = jnp.float32
_BF16 = jnp.bfloat16

_NT = (((1,), (1,)), ((), ()))
_NN = (((1,), (0,)), ((), ()))


_PROFILE_SCOPES = False


def _scope(name):
    return jax.named_scope(name) if _PROFILE_SCOPES else contextlib.nullcontext()


def _dot(a, b, dims=_NN):
    return lax.dot_general(a, b, dims, preferred_element_type=_F32)


def _ln(x):
    m = jnp.mean(x, axis=-1, keepdims=True)
    d = x - m
    v = jnp.mean(d * d, axis=-1, keepdims=True)
    return d * lax.rsqrt(v + _EPS)


def _gelu(x):
    return jax.nn.gelu(x, approximate=True)


def _token_shift(win):
    n, D = win.shape[0] - 16, win.shape[1]
    C = D // 4
    col = lax.broadcasted_iota(jnp.int32, (n, D), 1)
    return jnp.where(col < C, win[7:7 + n],
                     jnp.where(col < 2 * C, win[9:9 + n],
                               jnp.where(col < 3 * C, win[6:6 + n], win[10:10 + n])))


_DEFAULT_ORDER = (("q", "k", "s", "v", "b", "pv", "o"), (1, 2, 3), (1, 3, 5, 7, 9, 11, 16, 17))
_ORDERS = {
    ("norm", 2): (("q", "k", "s", "pv", "v", "b", "o"), (1, 3, 4), (2, 5, 7, 9, 10, 13, 15, 18)),
    ("pre", 2): (("q", "k", "s", "pv", "o", "v", "b"), (1, 3, 5), (0, 2, 4, 6, 8, 10, 12, 20)),
    ("ahead", 1): (("q", "o", "k", "s", "pv", "v", "b"), (1, 3, 5), (2, 3, 14, 17, 9, 11, 16, 19)),
    ("norm", 1): (("q", "k", "pv", "s", "v", "b", "o"), (1, 3, 5), (1, 4, 5, 7, 8, 11, 16, 20)),
}
_MIXER = tuple((n, c) for c in (0, 1) for n in ("b1", "b2", "b3", "b4"))


def _schedule(n_pairs, a_chains, b_stages, mode):
    key = (mode, len(a_chains))
    key_b = key + (len({c for _, c in b_stages}),)
    order, (lag_s, lag_pv, lag_o), slots = _ORDERS.get(key_b, _ORDERS.get(key, _DEFAULT_ORDER))
    scale = n_pairs / 16.0
    slots = {b: int(round(s * scale)) for b, s in zip(_MIXER, slots)}
    lag = dict(q=0, k=0, v=0, s=lag_s, pv=lag_pv, o=lag_o)
    sched = []
    for i in range(max(n_pairs + lag_o, max(slots.values()) + 1)):
        for item in order:
            if item == "b":
                sched += [b for b in _MIXER if b in b_stages and slots[b] == i]
            elif 0 <= i - lag[item] < n_pairs:
                sched.append((item, i - lag[item]))
    if mode == "first":
        assert lag_o >= _WO_LAG and order.index("q") < order.index("o")
        last = n_pairs - 1
        for j, before in enumerate((("s", last), ("pv", last), ("o", last))):
            sched.insert(sched.index(before), ("bulk", j))
    return tuple(sched)


def _kernel(x_hbm, mem0_hbm, wqt_hbm, wkt_hbm, wvt_hbm, wo_hbm,
            w1_hbm, w2_hbm, w3_hbm, w4_hbm, o_hbm,
            x_ref, mem0_ref, wq_ref, wk_ref, wv_ref, wo_ref,
            w1_ref, w2_ref, w3_ref, w4_ref, o_ref, stage_ref,
            ha_ref, h0_ref, pre_ref, acc_ref, ycur_ref, yprev_ref, nprev_ref, hprev_ref,
            htail_ref, y2res_ref, sems, *, n_seg, n_heads, d_head):
    S, D = x_ref.shape
    PW = 2 * d_head
    n_pairs = n_heads // 2
    scale = d_head ** -0.5
    L = _MEM + _SEG
    NA = _AHEAD * _SEG
    X0 = (_AHEAD + _LAG) * _SEG

    def pair_in(p, j):
        rows = pl.ds(p * PW, PW)
        sem = sems.at[4 * p + j]
        if j < 3:
            src = (wqt_hbm, wkt_hbm, wvt_hbm)[j]
            return pltpu.make_async_copy(src.at[rows, :], stage_ref.at[j, p], sem)
        return pltpu.make_async_copy(wo_hbm.at[rows, :], wo_ref.at[rows, :], sem)

    nb = 4 * n_pairs
    misc = dict(
        x0=pltpu.make_async_copy(x_hbm.at[pl.ds(0, X0), :], x_ref.at[pl.ds(0, X0), :], sems.at[nb]),
        x1=pltpu.make_async_copy(x_hbm.at[pl.ds(X0, S - X0), :], x_ref.at[pl.ds(X0, S - X0), :],
                                 sems.at[nb + 1]),
        mem0=pltpu.make_async_copy(mem0_hbm, mem0_ref, sems.at[nb + 2]),
        w1=pltpu.make_async_copy(w1_hbm, w1_ref, sems.at[nb + 3]),
        w2=pltpu.make_async_copy(w2_hbm, w2_ref, sems.at[nb + 4]),
        w3=pltpu.make_async_copy(w3_hbm, w3_ref, sems.at[nb + 5]),
        w4=pltpu.make_async_copy(w4_hbm, w4_ref, sems.at[nb + 6]),
    )
    n_early = (n_seg - _LAG - 2) * _SEG
    out_a = pltpu.make_async_copy(o_ref.at[pl.ds(0, n_early), :], o_hbm.at[pl.ds(0, n_early), :],
                                  sems.at[nb + 7])
    out_b = pltpu.make_async_copy(o_ref.at[pl.ds(n_early, S - n_early), :],
                                  o_hbm.at[pl.ds(n_early, S - n_early), :], sems.at[nb + 8])

    def xseg(s):
        if isinstance(s, int):
            return x_ref[s * _SEG:(s + 1) * _SEG, :].astype(_F32)
        return x_ref[pl.ds(pl.multiple_of(s * _SEG, _SEG), _SEG), :].astype(_F32)

    def pick(cond, a, b):
        if isinstance(cond, bool):
            return a if cond else b()
        return jnp.where(cond, a, b())

    T1 = slice(2 * _MEM, 2 * _MEM + _SEG)
    T2 = slice(2 * _MEM + _SEG, 2 * _MEM + 2 * _SEG)

    def step(t, a_chains, b_stages, mode="norm"):
        both = len(a_chains) == 2
        first = mode == "first"
        last_pair = n_pairs - 1
        lo = lax.broadcasted_iota(jnp.int32, (L, PW), 1) < d_head
        lane = lax.broadcasted_iota(jnp.int32, (L, 2 * L), 1)
        row = lax.broadcasted_iota(jnp.int32, (L, 2 * L), 0)
        seg0 = lane < L
        key = jnp.where(seg0, lane, lane - L)
        allowed = (row < _MEM) | (row >= key)

        st = {}

        def blockdiag(a):
            zero = jnp.zeros_like(a)
            return jnp.concatenate([jnp.where(lo, a, zero), jnp.where(lo, zero, a)],
                                   axis=0).astype(_BF16)

        if len(a_chains) == 1:
            c0 = a_chains[0]
            h32 = jnp.concatenate(
                [ha_ref[_MEM * c0:_MEM * (c0 + 1), :].astype(_F32),
                 ha_ref[(T1, T2)[c0], :].astype(_F32)], axis=0)

        def pre_at(j, p, s):
            if isinstance(s, int):
                return pre_ref.at[j, p, (s - 1) * _SEG:s * _SEG, :]
            return pre_ref.at[j, p, pl.ds(pl.multiple_of((s - 1) * _SEG, _SEG), _SEG), :]

        def proj(p, j):
            w_ref = (wq_ref, wk_ref, wv_ref)[j]
            if first:
                if p == 0 and j < 2:
                    for jj in ((0,), (1, 2))[j]:
                        pair_in(0, jj).wait()
                elif p > 0 and j == 0:
                    for jj in range(3):
                        pair_in(p, jj).wait()
                    if p >= _WO_LAG:
                        pair_in(p - _WO_LAG, 3).wait()
                wt = stage_ref[j, p]
                w_ref[p] = wt.T
                if p == last_pair:
                    return {0: _dot(h32, wt, _NT)}
                res = _dot(h0_ref[...], wt, _NT)
                pre_ref[j, p, 0:NA, :] = res[0:NA].astype(_BF16)
                return {0: res[NA:NA + L]}
            if mode == "ahead":
                res = _dot(h32, w_ref[p])
                pre_at(j, p, t + _AHEAD)[...] = res[_MEM:L].astype(_BF16)
                return {0: jnp.concatenate([res[0:_MEM], pre_at(j, p, t)[...].astype(_F32)], axis=0)}
            if mode == "pre":
                h = jnp.concatenate([ha_ref[0:2 * _MEM, :], ha_ref[T2, :]], axis=0)
                res = _dot(h, w_ref[p])
                return {0: jnp.concatenate([res[0:_MEM], pre_at(j, p, t)[...].astype(_F32)], axis=0),
                        1: res[_MEM:_MEM + L]}
            if both:
                res = _dot(ha_ref[...], w_ref[p])
                return {c: jnp.concatenate([res[_MEM * c:_MEM * (c + 1)], res[(T1, T2)[c]]], axis=0)
                        for c in (0, 1)}
            return {c0: _dot(h32, w_ref[p])}

        def bulk(j):
            wt = stage_ref[j, last_pair]
            pre_ref[j, last_pair, 0:NA, :] = _dot(h0_ref[0:NA, :], wt, _NT).astype(_BF16)

        def a_q(p):
            st["q", p] = proj(p, 0)

        def a_k(p):
            st["k", p] = proj(p, 1)

        def a_v(p):
            st["v", p] = proj(p, 2)

        def a_s(p):
            q, k = st.pop(("q", p)), st.pop(("k", p))
            for c in a_chains:
                s = _dot(q[c], blockdiag(k[c]), _NT) * scale
                s = jnp.where(allowed, s, _NEG)
                m0 = jnp.max(jnp.where(seg0, s, -jnp.inf), axis=1, keepdims=True)
                m1 = jnp.max(jnp.where(seg0, -jnp.inf, s), axis=1, keepdims=True)
                e = jnp.exp(s - jnp.where(seg0, m0, m1))
                l0 = jnp.sum(jnp.where(seg0, e, 0.0), axis=1, keepdims=True)
                l1 = jnp.sum(jnp.where(seg0, 0.0, e), axis=1, keepdims=True)
                st["p", p, c] = e / jnp.where(seg0, l0, l1)

        def a_pv(p):
            v = st.pop(("v", p))
            outs = [_dot(st.pop(("p", p, c)), blockdiag(v[c])) for c in a_chains]
            if both:
                st["o", p] = jnp.concatenate(
                    [outs[0][:_MEM], outs[1][:_MEM], outs[0][_MEM:], outs[1][_MEM:]],
                    axis=0).astype(_BF16)
            else:
                st["o", p] = outs[0]

        def a_o(p):
            if first and p == n_pairs - _WO_LAG:
                for q in range(p, n_pairs):
                    pair_in(q, 3).wait()
            part = _dot(st.pop(("o", p)), wo_ref[p * PW:(p + 1) * PW, :])
            n = part.shape[0]
            if p == 0:
                acc_ref[0:n, :] = part
            elif p < n_pairs - 1:
                acc_ref[0:n, :] += part
            else:
                st["acc"] = acc_ref[0:n, :] + part

        def rs(c):
            return slice(_SEG * c, _SEG * (c + 1))

        def rotate(c):
            htail_ref[8 * c:8 * c + 8, :] = hprev_ref[_SEG * (c + 1) - 8:_SEG * (c + 1), :]
            hprev_ref[rs(c), :] = st.pop(("h", c))
            nprev_ref[rs(c), :] = st.pop(("ncur", c))
            yprev_ref[rs(c), :] = st.pop(("ycur", c))

        def b_1(c):
            ycur = ycur_ref[rs(c), :]
            ncur = _ln(ycur)
            st["ycur", c], st["ncur", c] = ycur, ncur
            st["h", c] = _gelu(_dot(_ln(ncur).astype(_BF16), w1_ref[...]))
            if ("b2", c) not in b_stages:
                rotate(c)

        def b_2(c):
            s = t - 2 - _LAG * c
            hprev = hprev_ref[rs(c), :]
            pt = pick(s == 0, jnp.zeros((8, D), _F32), lambda: htail_ref[8 * c:8 * c + 8, :])
            nh = pick(s == n_seg - 1, jnp.zeros((8, D), _F32), lambda: st["h", c][0:8])
            g = _token_shift(jnp.concatenate([pt, hprev, nh], axis=0))
            st["x1", c] = nprev_ref[rs(c), :] + _dot(g.astype(_BF16), w2_ref[...])
            st["yres", c] = yprev_ref[rs(c), :]
            if ("b1", c) in b_stages:
                rotate(c)

        def b_3(c):
            st["f", c] = _gelu(_dot(_ln(st["x1", c]).astype(_BF16), w3_ref[...])).astype(_BF16)

        def b_4(c):
            ynew = st.pop(("yres", c)) + st.pop(("x1", c)) + _dot(st.pop(("f", c)), w4_ref[...])
            if c == 0:
                st["y2new"] = ynew
                st["tok2"] = _ln(ynew).astype(_BF16)
            else:
                so = t - 2 - _LAG
                if isinstance(so, int):
                    o_ref[so * _SEG:(so + 1) * _SEG, :] = ynew.astype(o_ref.dtype)
                else:
                    o_ref[pl.ds(pl.multiple_of(so * _SEG, _SEG), _SEG), :] = ynew.astype(o_ref.dtype)

        stages = dict(q=a_q, k=a_k, v=a_v, s=a_s, pv=a_pv, o=a_o, bulk=bulk,
                      b1=b_1, b2=b_2, b3=b_3, b4=b_4)
        for name, arg in _schedule(n_pairs, a_chains, b_stages, mode):
            stages[name](arg)

        if "tok2" in st:
            ha_ref[T2, :] = st.pop("tok2")
        if a_chains:
            acc = st.pop("acc")
            if both:
                mem1, mem2 = acc[0:_MEM], acc[_MEM:2 * _MEM]
                a1, a2 = acc[T1], acc[T2]
            elif a_chains == (0,):
                mem1, mem2 = acc[0:_MEM], mem0_ref[...].astype(_F32)
                a1, a2 = acc[_MEM:L], None
            else:
                mem1, mem2 = mem0_ref[...].astype(_F32), acc[0:_MEM]
                a1, a2 = None, acc[_MEM:L]
            ha_ref[0:2 * _MEM, :] = jnp.concatenate([mem1, mem2], axis=0).astype(_BF16)
            if a1 is not None:
                if isinstance(t, int):
                    nxt = t + 1 + _AHEAD if t + 1 < _LAG else min(t + 1, n_seg - 1)
                else:
                    nxt = jnp.minimum(t + 1, n_seg - 1)
                ha_ref[T1, :] = _ln(xseg(nxt)).astype(_BF16)
                ycur_ref[0:_SEG, :] = xseg(t) + a1
            if a2 is not None:
                ycur_ref[_SEG:, :] = y2res_ref[...] + a2
        if "y2new" in st:
            y2res_ref[...] = st.pop("y2new")
        assert not st, list(st)

    misc["x0"].start()
    misc["mem0"].start()
    for p in range(n_pairs + _WO_LAG):
        for j in range(3):
            if p < n_pairs:
                pair_in(p, j).start()
        if p >= _WO_LAG:
            pair_in(p - _WO_LAG, 3).start()
    for k in ("w1", "w2", "w3", "w4", "x1"):
        misc[k].start()
    for r in (ycur_ref, yprev_ref, nprev_ref, hprev_ref, htail_ref, y2res_ref):
        r[...] = jnp.zeros(r.shape, _F32)
    misc["x0"].wait()
    misc["mem0"].wait()
    mem0 = mem0_ref[...]
    ha_ref[0:2 * _MEM, :] = jnp.concatenate([mem0, mem0], axis=0).astype(_BF16)
    n0 = _ln(xseg(0))
    ha_ref[T1, :] = n0.astype(_BF16)
    ha_ref[T2, :] = jnp.zeros((_SEG, D), _BF16)
    for s in range(1, _AHEAD + 1):
        h0_ref[(s - 1) * _SEG:s * _SEG, :] = _ln(xseg(s))
    h0_ref[NA:NA + L, :] = jnp.concatenate([mem0.astype(_F32), n0], axis=0)

    B = lambda c, which: {(n, c) for n in which}
    ALL = ("b1", "b2", "b3", "b4")

    with _scope("step0"):
        step(0, (0,), set(), "first")
    with _scope("step1"):
        misc["w1"].wait()
        step(1, (0,), B(0, ALL[:1]), "ahead")
    with _scope("step2"):
        for k in ("w2", "w3", "w4"):
            misc[k].wait()
        step(2, (0,), B(0, ALL), "ahead")
        misc["x1"].wait()

    def run(lo_t, hi_t, mode):
        def body(t, carry):
            step(t, (0, 1), B(0, ALL) | B(1, ALL), mode)
            return carry
        lax.fori_loop(lo_t, hi_t, body, 0)

    with _scope("loop_pre"):
        step(_LAG, (0, 1), B(0, ALL), "pre")
        step(_LAG + 1, (0, 1), B(0, ALL) | B(1, ALL[:1]), "pre")
        run(_LAG + 2, _LAG + _AHEAD, "pre")
    with _scope("loop"):
        run(_LAG + _AHEAD, n_seg, "norm")

    with _scope("tailA"):
        out_a.start()
        step(n_seg, (1,), B(0, ALL) | B(1, ALL))
        step(n_seg + 1, (1,), B(0, ALL[1:]) | B(1, ALL))
        step(n_seg + 2, (1,), B(1, ALL))
    with _scope("tailB"):
        C1 = slice(_SEG, 2 * _SEG)
        ycur = ycur_ref[C1, :]
        ncur = _ln(ycur)
        hcur = _gelu(_dot(_ln(ncur).astype(_BF16), w1_ref[...]))
        g = _token_shift(jnp.concatenate(
            [htail_ref[8:16, :], hprev_ref[C1, :], hcur, jnp.zeros((8, D), _F32)], axis=0))
        x1 = jnp.concatenate([nprev_ref[C1, :], ncur], axis=0) + _dot(g.astype(_BF16), w2_ref[...])
        f = _gelu(_dot(_ln(x1).astype(_BF16), w3_ref[...])).astype(_BF16)
        ynew = jnp.concatenate([yprev_ref[C1, :], ycur], axis=0) + x1 + _dot(f, w4_ref[...])
        o_ref[(n_seg - 2) * _SEG:n_seg * _SEG, :] = ynew.astype(o_ref.dtype)
    with _scope("out"):
        out_b.start()
        out_a.wait()
        out_b.wait()


@functools.partial(jax.jit, static_argnames=("A_seg_len",))
def pallas_interleave_layers__memory_aug_recurrent_mem_tr__mixer_s_mlp__prompt_kernel(
    A_x: jax.Array,
    A_mem0: jax.Array,
    A_Wq: jax.Array,
    A_Wk: jax.Array,
    A_Wv: jax.Array,
    A_Wo: jax.Array,
    A_seg_len,
    B_x: jax.Array,
    B_w1: jax.Array,
    B_w2: jax.Array,
    B_w3: jax.Array,
    B_w4: jax.Array,
):
    del B_x
    _, S, D = A_x.shape
    _, H, Dh = A_Wq.shape
    F = B_w3.shape[1]
    assert A_seg_len == _SEG and A_mem0.shape[1] == _MEM and A_x.shape[0] == 1
    n_seg = S // _SEG
    assert n_seg * _SEG == S and n_seg >= 2 * _LAG + 2 + _AHEAD and H % 2 == 0

    def wt(w):
        return jnp.transpose(w, (1, 2, 0)).reshape(H * Dh, D)

    R = 2 * (_MEM + _SEG)
    NP, PW = H // 2, 2 * Dh
    hbm = pl.BlockSpec(memory_space=pl.ANY)
    out = pl.pallas_call(
        functools.partial(_kernel, n_seg=n_seg, n_heads=H, d_head=Dh),
        out_shape=jax.ShapeDtypeStruct((S, D), A_x.dtype),
        in_specs=[hbm] * 10,
        out_specs=hbm,
        scratch_shapes=[
            pltpu.VMEM((S, D), _BF16),
            pltpu.VMEM((_MEM, D), _BF16),
            pltpu.VMEM((NP, D, PW), _BF16),
            pltpu.VMEM((NP, D, PW), _BF16),
            pltpu.VMEM((NP, D, PW), _BF16),
            pltpu.VMEM((H * Dh, D), _BF16),
            pltpu.VMEM((D, D), _BF16),
            pltpu.VMEM((D, D), _BF16),
            pltpu.VMEM((D, F), _BF16),
            pltpu.VMEM((F, D), _BF16),
            pltpu.VMEM((S, D), A_x.dtype),
            pltpu.VMEM((3, NP, PW, D), _BF16),
            pltpu.VMEM((R, D), _BF16),
            pltpu.VMEM((_AHEAD * _SEG + _MEM + _SEG, D), _F32),
            pltpu.VMEM((3, NP, (_AHEAD + _LAG - 1) * _SEG, PW), _BF16),
            pltpu.VMEM((R, D), _F32),
            pltpu.VMEM((2 * _SEG, D), _F32),
            pltpu.VMEM((2 * _SEG, D), _F32),
            pltpu.VMEM((2 * _SEG, D), _F32),
            pltpu.VMEM((2 * _SEG, D), _F32),
            pltpu.VMEM((16, D), _F32),
            pltpu.VMEM((_SEG, D), _F32),
            pltpu.SemaphoreType.DMA((4 * NP + 9,)),
        ],
        compiler_params=pltpu.CompilerParams(vmem_limit_bytes=100 * 1024 * 1024),
    )(A_x.reshape(S, D), A_mem0.reshape(_MEM, D), wt(A_Wq), wt(A_Wk), wt(A_Wv),
      A_Wo.reshape(H * Dh, D), B_w1, B_w2, B_w3, B_w4)
    return out.reshape(1, S, D)
```

```python
import contextlib
import functools

import jax
import jax.numpy as jnp
from jax import lax
import jax.experimental.pallas as pl
import jax.experimental.pallas.tpu as pltpu

_SEG = 32
_MEM = 8
_LAG = 3
_AHEAD = 9
_WO_LAG = 3
_NEG = -1000000000.0
_EPS = 1e-05

_F32 = jnp.float32
_BF16 = jnp.bfloat16

_NT = (((1,), (1,)), ((), ()))
_NN = (((1,), (0,)), ((), ()))


_PROFILE_SCOPES = False


def _scope(name):
    return jax.named_scope(name) if _PROFILE_SCOPES else contextlib.nullcontext()


def _dot(a, b, dims=_NN):
    return lax.dot_general(a, b, dims, preferred_element_type=_F32)


def _ln(x):
    m = jnp.mean(x, axis=-1, keepdims=True)
    d = x - m
    v = jnp.mean(d * d, axis=-1, keepdims=True)
    return d * lax.rsqrt(v + _EPS)


def _gelu(x):
    return jax.nn.gelu(x, approximate=True)


def _token_shift(win):
    n, D = win.shape[0] - 16, win.shape[1]
    C = D // 4
    col = lax.broadcasted_iota(jnp.int32, (n, D), 1)
    return jnp.where(col < C, win[7:7 + n],
                     jnp.where(col < 2 * C, win[9:9 + n],
                               jnp.where(col < 3 * C, win[6:6 + n], win[10:10 + n])))


_DEFAULT_ORDER = (("q", "k", "s", "v", "b", "pv", "o"), (1, 2, 3), (1, 3, 5, 7, 9, 11, 16, 17))
_ORDERS = {
    ("norm", 2): (("q", "k", "s", "pv", "v", "b", "o"), (1, 3, 4), (2, 5, 7, 9, 10, 13, 15, 18)),
    ("pre", 2): (("q", "k", "s", "pv", "o", "v", "b"), (1, 3, 5), (0, 2, 4, 6, 8, 10, 12, 20)),
    ("ahead", 1): (("q", "o", "k", "s", "pv", "v", "b"), (1, 3, 5), (2, 3, 14, 17, 9, 11, 16, 19)),
    ("norm", 1): (("q", "k", "pv", "s", "v", "b", "o"), (1, 3, 5), (1, 4, 5, 7, 8, 11, 16, 20)),
}
_MIXER = tuple((n, c) for c in (0, 1) for n in ("b1", "b2", "b3", "b4"))


def _schedule(n_pairs, a_chains, b_stages, mode):
    key = (mode, len(a_chains))
    key_b = key + (len({c for _, c in b_stages}),)
    order, (lag_s, lag_pv, lag_o), slots = _ORDERS.get(key_b, _ORDERS.get(key, _DEFAULT_ORDER))
    scale = n_pairs / 16.0
    slots = {b: int(round(s * scale)) for b, s in zip(_MIXER, slots)}
    lag = dict(q=0, k=0, v=0, s=lag_s, pv=lag_pv, o=lag_o)
    sched = []
    for i in range(max(n_pairs + lag_o, max(slots.values()) + 1)):
        for item in order:
            if item == "b":
                sched += [b for b in _MIXER if b in b_stages and slots[b] == i]
            elif 0 <= i - lag[item] < n_pairs:
                sched.append((item, i - lag[item]))
    if mode == "first":
        assert lag_o >= _WO_LAG and order.index("q") < order.index("o")
        last = n_pairs - 1
        for j, before in enumerate((("s", last), ("pv", last), ("o", last))):
            sched.insert(sched.index(before), ("bulk", j))
    return tuple(sched)


def _kernel(x_hbm, mem0_hbm, wqt_hbm, wkt_hbm, wvt_hbm, wo_hbm,
            w1_hbm, w2_hbm, w3_hbm, w4_hbm, o_hbm,
            x_ref, mem0_ref, wq_ref, wk_ref, wv_ref, wo_ref,
            w1_ref, w2_ref, w3_ref, w4_ref, o_ref, stage_ref,
            ha_ref, h0_ref, pre_ref, acc_ref, ycur_ref, yprev_ref, nprev_ref, hprev_ref,
            htail_ref, y2res_ref, sems, *, n_seg, n_heads, d_head):
    S, D = x_ref.shape
    PW = 2 * d_head
    n_pairs = n_heads // 2
    scale = d_head ** -0.5
    L = _MEM + _SEG
    NA = _AHEAD * _SEG
    X0 = (_AHEAD + _LAG) * _SEG

    def pair_in(p, j):
        rows = pl.ds(p * PW, PW)
        sem = sems.at[4 * p + j]
        if j < 3:
            src = (wqt_hbm, wkt_hbm, wvt_hbm)[j]
            return pltpu.make_async_copy(src.at[rows, :], stage_ref.at[j, p], sem)
        return pltpu.make_async_copy(wo_hbm.at[rows, :], wo_ref.at[rows, :], sem)

    nb = 4 * n_pairs
    misc = dict(
        x0=pltpu.make_async_copy(x_hbm.at[pl.ds(0, X0), :], x_ref.at[pl.ds(0, X0), :], sems.at[nb]),
        x1=pltpu.make_async_copy(x_hbm.at[pl.ds(X0, S - X0), :], x_ref.at[pl.ds(X0, S - X0), :],
                                 sems.at[nb + 1]),
        mem0=pltpu.make_async_copy(mem0_hbm, mem0_ref, sems.at[nb + 2]),
        w1=pltpu.make_async_copy(w1_hbm, w1_ref, sems.at[nb + 3]),
        w2=pltpu.make_async_copy(w2_hbm, w2_ref, sems.at[nb + 4]),
        w3=pltpu.make_async_copy(w3_hbm, w3_ref, sems.at[nb + 5]),
        w4=pltpu.make_async_copy(w4_hbm, w4_ref, sems.at[nb + 6]),
    )
    n_early = (n_seg - _LAG - 2) * _SEG
    out_a = pltpu.make_async_copy(o_ref.at[pl.ds(0, n_early), :], o_hbm.at[pl.ds(0, n_early), :],
                                  sems.at[nb + 7])
    out_b = pltpu.make_async_copy(o_ref.at[pl.ds(n_early, S - n_early), :],
                                  o_hbm.at[pl.ds(n_early, S - n_early), :], sems.at[nb + 8])

    def xseg(s):
        if isinstance(s, int):
            return x_ref[s * _SEG:(s + 1) * _SEG, :].astype(_F32)
        return x_ref[pl.ds(pl.multiple_of(s * _SEG, _SEG), _SEG), :].astype(_F32)

    def pick(cond, a, b):
        if isinstance(cond, bool):
            return a if cond else b()
        return jnp.where(cond, a, b())

    T1 = slice(2 * _MEM, 2 * _MEM + _SEG)
    T2 = slice(2 * _MEM + _SEG, 2 * _MEM + 2 * _SEG)

    def step(t, a_chains, b_stages, mode="norm", final=False):
        both = len(a_chains) == 2
        first = mode == "first"
        last_pair = n_pairs - 1
        lo = lax.broadcasted_iota(jnp.int32, (L, PW), 1) < d_head
        nq = _SEG if final else L
        lane = lax.broadcasted_iota(jnp.int32, (nq, 2 * L), 1)
        row = lax.broadcasted_iota(jnp.int32, (nq, 2 * L), 0) + (L - nq)
        seg0 = lane < L
        key = jnp.where(seg0, lane, lane - L)
        allowed = (row < _MEM) | (row >= key)

        st = {}

        def blockdiag(a):
            zero = jnp.zeros_like(a)
            return jnp.concatenate([jnp.where(lo, a, zero), jnp.where(lo, zero, a)],
                                   axis=0).astype(_BF16)

        if len(a_chains) == 1:
            c0 = a_chains[0]
            h32 = jnp.concatenate(
                [ha_ref[_MEM * c0:_MEM * (c0 + 1), :].astype(_F32),
                 ha_ref[(T1, T2)[c0], :].astype(_F32)], axis=0)

        def pre_at(j, p, s):
            if isinstance(s, int):
                return pre_ref.at[j, p, (s - 1) * _SEG:s * _SEG, :]
            return pre_ref.at[j, p, pl.ds(pl.multiple_of((s - 1) * _SEG, _SEG), _SEG), :]

        def proj(p, j):
            w_ref = (wq_ref, wk_ref, wv_ref)[j]
            if first:
                if p == 0 and j < 2:
                    for jj in ((0,), (1, 2))[j]:
                        pair_in(0, jj).wait()
                elif p > 0 and j == 0:
                    for jj in range(3):
                        pair_in(p, jj).wait()
                    if p >= _WO_LAG:
                        pair_in(p - _WO_LAG, 3).wait()
                wt = stage_ref[j, p]
                w_ref[p] = wt.T
                if p == last_pair:
                    return {0: _dot(h32, wt, _NT)}
                res = _dot(h0_ref[...], wt, _NT)
                pre_ref[j, p, 0:NA, :] = res[0:NA].astype(_BF16)
                return {0: res[NA:NA + L]}
            if mode == "ahead":
                res = _dot(h32, w_ref[p])
                pre_at(j, p, t + _AHEAD)[...] = res[_MEM:L].astype(_BF16)
                return {0: jnp.concatenate([res[0:_MEM], pre_at(j, p, t)[...].astype(_F32)], axis=0)}
            if mode == "pre":
                h = jnp.concatenate([ha_ref[0:2 * _MEM, :], ha_ref[T2, :]], axis=0)
                res = _dot(h, w_ref[p])
                return {0: jnp.concatenate([res[0:_MEM], pre_at(j, p, t)[...].astype(_F32)], axis=0),
                        1: res[_MEM:_MEM + L]}
            if both:
                res = _dot(ha_ref[...], w_ref[p])
                return {c: jnp.concatenate([res[_MEM * c:_MEM * (c + 1)], res[(T1, T2)[c]]], axis=0)
                        for c in (0, 1)}
            return {c0: _dot(h32[_MEM:] if final and j == 0 else h32, w_ref[p])}

        def bulk(j):
            wt = stage_ref[j, last_pair]
            pre_ref[j, last_pair, 0:NA, :] = _dot(h0_ref[0:NA, :], wt, _NT).astype(_BF16)

        def a_q(p):
            st["q", p] = proj(p, 0)

        def a_k(p):
            st["k", p] = proj(p, 1)

        def a_v(p):
            st["v", p] = proj(p, 2)

        def a_s(p):
            q, k = st.pop(("q", p)), st.pop(("k", p))
            for c in a_chains:
                s = _dot(q[c], blockdiag(k[c]), _NT) * scale
                s = jnp.where(allowed, s, _NEG)
                m0 = jnp.max(jnp.where(seg0, s, -jnp.inf), axis=1, keepdims=True)
                m1 = jnp.max(jnp.where(seg0, -jnp.inf, s), axis=1, keepdims=True)
                e = jnp.exp(s - jnp.where(seg0, m0, m1))
                l0 = jnp.sum(jnp.where(seg0, e, 0.0), axis=1, keepdims=True)
                l1 = jnp.sum(jnp.where(seg0, 0.0, e), axis=1, keepdims=True)
                st["p", p, c] = e / jnp.where(seg0, l0, l1)

        def a_pv(p):
            v = st.pop(("v", p))
            outs = [_dot(st.pop(("p", p, c)), blockdiag(v[c])) for c in a_chains]
            if both:
                st["o", p] = jnp.concatenate(
                    [outs[0][:_MEM], outs[1][:_MEM], outs[0][_MEM:], outs[1][_MEM:]],
                    axis=0).astype(_BF16)
            else:
                st["o", p] = outs[0]

        def a_o(p):
            if first and p == n_pairs - _WO_LAG:
                for q in range(p, n_pairs):
                    pair_in(q, 3).wait()
            part = _dot(st.pop(("o", p)), wo_ref[p * PW:(p + 1) * PW, :])
            n = part.shape[0]
            if p == 0:
                acc_ref[0:n, :] = part
            elif p < n_pairs - 1:
                acc_ref[0:n, :] += part
            else:
                st["acc"] = acc_ref[0:n, :] + part

        def rs(c):
            return slice(_SEG * c, _SEG * (c + 1))

        def rotate(c):
            htail_ref[8 * c:8 * c + 8, :] = hprev_ref[_SEG * (c + 1) - 8:_SEG * (c + 1), :]
            hprev_ref[rs(c), :] = st.pop(("h", c))
            nprev_ref[rs(c), :] = st.pop(("ncur", c))
            yprev_ref[rs(c), :] = st.pop(("ycur", c))

        def b_1(c):
            ycur = ycur_ref[rs(c), :]
            ncur = _ln(ycur)
            st["ycur", c], st["ncur", c] = ycur, ncur
            st["h", c] = _gelu(_dot(_ln(ncur).astype(_BF16), w1_ref[...]))
            if ("b2", c) not in b_stages:
                rotate(c)

        def b_2(c):
            s = t - 2 - _LAG * c
            hprev = hprev_ref[rs(c), :]
            pt = pick(s == 0, jnp.zeros((8, D), _F32), lambda: htail_ref[8 * c:8 * c + 8, :])
            nh = pick(s == n_seg - 1, jnp.zeros((8, D), _F32), lambda: st["h", c][0:8])
            g = _token_shift(jnp.concatenate([pt, hprev, nh], axis=0))
            st["x1", c] = nprev_ref[rs(c), :] + _dot(g.astype(_BF16), w2_ref[...])
            st["yres", c] = yprev_ref[rs(c), :]
            if ("b1", c) in b_stages:
                rotate(c)

        def b_3(c):
            st["f", c] = _gelu(_dot(_ln(st["x1", c]).astype(_BF16), w3_ref[...])).astype(_BF16)

        def b_4(c):
            ynew = st.pop(("yres", c)) + st.pop(("x1", c)) + _dot(st.pop(("f", c)), w4_ref[...])
            if c == 0:
                st["y2new"] = ynew
                st["tok2"] = _ln(ynew).astype(_BF16)
            else:
                so = t - 2 - _LAG
                if isinstance(so, int):
                    o_ref[so * _SEG:(so + 1) * _SEG, :] = ynew.astype(o_ref.dtype)
                else:
                    o_ref[pl.ds(pl.multiple_of(so * _SEG, _SEG), _SEG), :] = ynew.astype(o_ref.dtype)

        stages = dict(q=a_q, k=a_k, v=a_v, s=a_s, pv=a_pv, o=a_o, bulk=bulk,
                      b1=b_1, b2=b_2, b3=b_3, b4=b_4)
        for name, arg in _schedule(n_pairs, a_chains, b_stages, mode):
            stages[name](arg)

        if "tok2" in st:
            ha_ref[T2, :] = st.pop("tok2")
        if a_chains:
            acc = st.pop("acc")
            if both:
                mem1, mem2 = acc[0:_MEM], acc[_MEM:2 * _MEM]
                a1, a2 = acc[T1], acc[T2]
            elif a_chains == (0,):
                mem1, mem2 = acc[0:_MEM], mem0_ref[...].astype(_F32)
                a1, a2 = acc[_MEM:L], None
            elif final:
                a1, a2 = None, acc
            else:
                mem1, mem2 = mem0_ref[...].astype(_F32), acc[0:_MEM]
                a1, a2 = None, acc[_MEM:L]
            if not final:
                ha_ref[0:2 * _MEM, :] = jnp.concatenate([mem1, mem2], axis=0).astype(_BF16)
            if a1 is not None:
                if isinstance(t, int):
                    nxt = t + 1 + _AHEAD if t + 1 < _LAG else min(t + 1, n_seg - 1)
                else:
                    nxt = jnp.minimum(t + 1, n_seg - 1)
                ha_ref[T1, :] = _ln(xseg(nxt)).astype(_BF16)
                ycur_ref[0:_SEG, :] = xseg(t) + a1
            if a2 is not None:
                ycur_ref[_SEG:, :] = y2res_ref[...] + a2
        if "y2new" in st:
            y2res_ref[...] = st.pop("y2new")
        assert not st, list(st)

    misc["x0"].start()
    misc["mem0"].start()
    for p in range(n_pairs + _WO_LAG):
        for j in range(3):
            if p < n_pairs:
                pair_in(p, j).start()
        if p >= _WO_LAG:
            pair_in(p - _WO_LAG, 3).start()
    for k in ("w1", "w2", "w3", "w4", "x1"):
        misc[k].start()
    for r in (ycur_ref, yprev_ref, nprev_ref, hprev_ref, htail_ref, y2res_ref):
        r[...] = jnp.zeros(r.shape, _F32)
    misc["x0"].wait()
    misc["mem0"].wait()
    mem0 = mem0_ref[...]
    ha_ref[0:2 * _MEM, :] = jnp.concatenate([mem0, mem0], axis=0).astype(_BF16)
    n0 = _ln(xseg(0))
    ha_ref[T1, :] = n0.astype(_BF16)
    ha_ref[T2, :] = jnp.zeros((_SEG, D), _BF16)
    for s in range(1, _AHEAD + 1):
        h0_ref[(s - 1) * _SEG:s * _SEG, :] = _ln(xseg(s))
    h0_ref[NA:NA + L, :] = jnp.concatenate([mem0.astype(_F32), n0], axis=0)

    B = lambda c, which: {(n, c) for n in which}
    ALL = ("b1", "b2", "b3", "b4")

    with _scope("step0"):
        step(0, (0,), set(), "first")
    with _scope("step1"):
        misc["w1"].wait()
        step(1, (0,), B(0, ALL[:1]), "ahead")
    with _scope("step2"):
        for k in ("w2", "w3", "w4"):
            misc[k].wait()
        step(2, (0,), B(0, ALL), "ahead")
        misc["x1"].wait()

    def run(lo_t, hi_t, mode):
        def body(t, carry):
            step(t, (0, 1), B(0, ALL) | B(1, ALL), mode)
            return carry
        lax.fori_loop(lo_t, hi_t, body, 0)

    with _scope("loop_pre"):
        step(_LAG, (0, 1), B(0, ALL), "pre")
        step(_LAG + 1, (0, 1), B(0, ALL) | B(1, ALL[:1]), "pre")
        run(_LAG + 2, _LAG + _AHEAD, "pre")
    with _scope("loop"):
        run(_LAG + _AHEAD, n_seg, "norm")

    with _scope("tailA"):
        out_a.start()
        step(n_seg, (1,), B(0, ALL) | B(1, ALL))
        step(n_seg + 1, (1,), B(0, ALL[1:]) | B(1, ALL))
        step(n_seg + 2, (1,), B(1, ALL), final=True)
    with _scope("tailB"):
        C1 = slice(_SEG, 2 * _SEG)
        ycur = ycur_ref[C1, :]
        ncur = _ln(ycur)
        hcur = _gelu(_dot(_ln(ncur).astype(_BF16), w1_ref[...]))
        g = _token_shift(jnp.concatenate(
            [htail_ref[8:16, :], hprev_ref[C1, :], hcur, jnp.zeros((8, D), _F32)], axis=0))
        x1 = jnp.concatenate([nprev_ref[C1, :], ncur], axis=0) + _dot(g.astype(_BF16), w2_ref[...])
        f = _gelu(_dot(_ln(x1).astype(_BF16), w3_ref[...])).astype(_BF16)
        ynew = jnp.concatenate([yprev_ref[C1, :], ycur], axis=0) + x1 + _dot(f, w4_ref[...])
        o_ref[(n_seg - 2) * _SEG:n_seg * _SEG, :] = ynew.astype(o_ref.dtype)
    with _scope("out"):
        out_b.start()
        out_a.wait()
        out_b.wait()


@functools.partial(jax.jit, static_argnames=("A_seg_len",))
def pallas_interleave_layers__memory_aug_recurrent_mem_tr__mixer_s_mlp__prompt_kernel(
    A_x: jax.Array,
    A_mem0: jax.Array,
    A_Wq: jax.Array,
    A_Wk: jax.Array,
    A_Wv: jax.Array,
    A_Wo: jax.Array,
    A_seg_len,
    B_x: jax.Array,
    B_w1: jax.Array,
    B_w2: jax.Array,
    B_w3: jax.Array,
    B_w4: jax.Array,
):
    del B_x
    _, S, D = A_x.shape
    _, H, Dh = A_Wq.shape
    F = B_w3.shape[1]
    assert A_seg_len == _SEG and A_mem0.shape[1] == _MEM and A_x.shape[0] == 1
    n_seg = S // _SEG
    assert n_seg * _SEG == S and n_seg >= 2 * _LAG + 2 + _AHEAD and H % 2 == 0

    def wt(w):
        return jnp.transpose(w, (1, 2, 0)).reshape(H * Dh, D)

    R = 2 * (_MEM + _SEG)
    NP, PW = H // 2, 2 * Dh
    hbm = pl.BlockSpec(memory_space=pl.ANY)
    out = pl.pallas_call(
        functools.partial(_kernel, n_seg=n_seg, n_heads=H, d_head=Dh),
        out_shape=jax.ShapeDtypeStruct((S, D), A_x.dtype),
        in_specs=[hbm] * 10,
        out_specs=hbm,
        scratch_shapes=[
            pltpu.VMEM((S, D), _BF16),
            pltpu.VMEM((_MEM, D), _BF16),
            pltpu.VMEM((NP, D, PW), _BF16),
            pltpu.VMEM((NP, D, PW), _BF16),
            pltpu.VMEM((NP, D, PW), _BF16),
            pltpu.VMEM((H * Dh, D), _BF16),
            pltpu.VMEM((D, D), _BF16),
            pltpu.VMEM((D, D), _BF16),
            pltpu.VMEM((D, F), _BF16),
            pltpu.VMEM((F, D), _BF16),
            pltpu.VMEM((S, D), A_x.dtype),
            pltpu.VMEM((3, NP, PW, D), _BF16),
            pltpu.VMEM((R, D), _BF16),
            pltpu.VMEM((_AHEAD * _SEG + _MEM + _SEG, D), _F32),
            pltpu.VMEM((3, NP, (_AHEAD + _LAG - 1) * _SEG, PW), _BF16),
            pltpu.VMEM((R, D), _F32),
            pltpu.VMEM((2 * _SEG, D), _F32),
            pltpu.VMEM((2 * _SEG, D), _F32),
            pltpu.VMEM((2 * _SEG, D), _F32),
            pltpu.VMEM((2 * _SEG, D), _F32),
            pltpu.VMEM((16, D), _F32),
            pltpu.VMEM((_SEG, D), _F32),
            pltpu.SemaphoreType.DMA((4 * NP + 9,)),
        ],
        compiler_params=pltpu.CompilerParams(vmem_limit_bytes=100 * 1024 * 1024),
    )(A_x.reshape(S, D), A_mem0.reshape(_MEM, D), wt(A_Wq), wt(A_Wk), wt(A_Wv),
      A_Wo.reshape(H * Dh, D), B_w1, B_w2, B_w3, B_w4)
    return out.reshape(1, S, D)
```

```python
import contextlib
import functools

import jax
import jax.numpy as jnp
from jax import lax
import jax.experimental.pallas as pl
import jax.experimental.pallas.tpu as pltpu

_SEG = 32
_MEM = 8
_LAG = 3
_AHEAD = 11
_WO_LAG = 3
_FLAGS = ({"XLA_TPU_RESCHEDULE_DMA_DONES": True}
          if tuple(int(v) for v in jax.__version__.split(".")[:2]) >= (0, 12) else None)
_NEG = -1000000000.0
_EPS = 1e-05

_F32 = jnp.float32
_BF16 = jnp.bfloat16

_NT = (((1,), (1,)), ((), ()))
_NN = (((1,), (0,)), ((), ()))


_PROFILE_SCOPES = False


def _scope(name):
    return jax.named_scope(name) if _PROFILE_SCOPES else contextlib.nullcontext()


def _dot(a, b, dims=_NN):
    return lax.dot_general(a, b, dims, preferred_element_type=_F32)


def _ln(x):
    m = jnp.mean(x, axis=-1, keepdims=True)
    d = x - m
    v = jnp.mean(d * d, axis=-1, keepdims=True)
    return d * lax.rsqrt(v + _EPS)


def _gelu(x):
    return jax.nn.gelu(x, approximate=True)


def _token_shift(win):
    n, D = win.shape[0] - 16, win.shape[1]
    C = D // 4
    col = lax.broadcasted_iota(jnp.int32, (n, D), 1)
    return jnp.where(col < C, win[7:7 + n],
                     jnp.where(col < 2 * C, win[9:9 + n],
                               jnp.where(col < 3 * C, win[6:6 + n], win[10:10 + n])))


_DEFAULT_ORDER = (("q", "k", "s", "v", "b", "pv", "o"), (1, 2, 3), (1, 3, 5, 7, 9, 11, 16, 17))
_ORDERS = {
    ("norm", 2): (("q", "k", "s", "pv", "v", "b", "o"), (1, 3, 4), (2, 5, 7, 9, 10, 13, 15, 18)),
    ("pre", 2): (("q", "k", "s", "pv", "o", "v", "b"), (1, 3, 5), (0, 2, 4, 6, 8, 10, 12, 20)),
    ("ahead", 1): (("q", "o", "k", "s", "pv", "v", "b"), (1, 3, 5), (2, 3, 14, 17, 9, 11, 16, 19)),
    ("norm", 1): (("q", "k", "pv", "s", "v", "b", "o"), (1, 3, 5), (1, 4, 5, 7, 8, 11, 16, 20)),
}
_MIXER = tuple((n, c) for c in (0, 1) for n in ("b1", "b2", "b3", "b4"))


def _schedule(n_pairs, a_chains, b_stages, mode):
    key = (mode, len(a_chains))
    key_b = key + (len({c for _, c in b_stages}),)
    order, (lag_s, lag_pv, lag_o), slots = _ORDERS.get(key_b, _ORDERS.get(key, _DEFAULT_ORDER))
    scale = n_pairs / 16.0
    slots = {b: int(round(s * scale)) for b, s in zip(_MIXER, slots)}
    lag = dict(q=0, k=0, v=0, s=lag_s, pv=lag_pv, o=lag_o)
    sched = []
    for i in range(max(n_pairs + lag_o, max(slots.values()) + 1)):
        for item in order:
            if item == "b":
                sched += [b for b in _MIXER if b in b_stages and slots[b] == i]
            elif 0 <= i - lag[item] < n_pairs:
                sched.append((item, i - lag[item]))
    if mode == "first":
        assert lag_o >= _WO_LAG and order.index("q") < order.index("o")
        last = n_pairs - 1
        for j, before in enumerate((("s", last), ("pv", last), ("o", last))):
            sched.insert(sched.index(before), ("bulk", j))
    return tuple(sched)


def _kernel(x_hbm, mem0_hbm, wqt_hbm, wkt_hbm, wvt_hbm, wo_hbm,
            w1_hbm, w2_hbm, w3_hbm, w4_hbm, o_hbm,
            x_ref, mem0_ref, wq_ref, wk_ref, wv_ref, wo_ref,
            w1_ref, w2_ref, w3_ref, w4_ref, o_ref, stage_ref,
            ha_ref, h0_ref, pre_ref, acc_ref, ycur_ref, yprev_ref, nprev_ref, hprev_ref,
            htail_ref, y2res_ref, sems, *, n_seg, n_heads, d_head):
    S, D = x_ref.shape
    PW = 2 * d_head
    n_pairs = n_heads // 2
    scale = d_head ** -0.5
    L = _MEM + _SEG
    NA = _AHEAD * _SEG
    X0 = (_AHEAD + _LAG) * _SEG

    def pair_in(p, j):
        rows = pl.ds(p * PW, PW)
        sem = sems.at[4 * p + j]
        if j < 3:
            src = (wqt_hbm, wkt_hbm, wvt_hbm)[j]
            return pltpu.make_async_copy(src.at[rows, :], stage_ref.at[j, p], sem)
        return pltpu.make_async_copy(wo_hbm.at[rows, :], wo_ref.at[rows, :], sem)

    nb = 4 * n_pairs
    misc = dict(
        x0=pltpu.make_async_copy(x_hbm.at[pl.ds(0, X0), :], x_ref.at[pl.ds(0, X0), :], sems.at[nb]),
        x1=pltpu.make_async_copy(x_hbm.at[pl.ds(X0, S - X0), :], x_ref.at[pl.ds(X0, S - X0), :],
                                 sems.at[nb + 1]),
        mem0=pltpu.make_async_copy(mem0_hbm, mem0_ref, sems.at[nb + 2]),
        w1=pltpu.make_async_copy(w1_hbm, w1_ref, sems.at[nb + 3]),
        w2=pltpu.make_async_copy(w2_hbm, w2_ref, sems.at[nb + 4]),
        w3=pltpu.make_async_copy(w3_hbm, w3_ref, sems.at[nb + 5]),
        w4=pltpu.make_async_copy(w4_hbm, w4_ref, sems.at[nb + 6]),
    )
    n_early = (n_seg - _LAG - 2) * _SEG
    out_a = pltpu.make_async_copy(o_ref.at[pl.ds(0, n_early), :], o_hbm.at[pl.ds(0, n_early), :],
                                  sems.at[nb + 7])
    out_b = pltpu.make_async_copy(o_ref.at[pl.ds(n_early, S - n_early), :],
                                  o_hbm.at[pl.ds(n_early, S - n_early), :], sems.at[nb + 8])

    def xseg(s):
        if isinstance(s, int):
            return x_ref[s * _SEG:(s + 1) * _SEG, :].astype(_F32)
        return x_ref[pl.ds(pl.multiple_of(s * _SEG, _SEG), _SEG), :].astype(_F32)

    def pick(cond, a, b):
        if isinstance(cond, bool):
            return a if cond else b()
        return jnp.where(cond, a, b())

    T1 = slice(2 * _MEM, 2 * _MEM + _SEG)
    T2 = slice(2 * _MEM + _SEG, 2 * _MEM + 2 * _SEG)

    def step(t, a_chains, b_stages, mode="norm", final=False):
        both = len(a_chains) == 2
        first = mode == "first"
        last_pair = n_pairs - 1
        lo = lax.broadcasted_iota(jnp.int32, (L, PW), 1) < d_head
        nq = _SEG if final else L
        lane = lax.broadcasted_iota(jnp.int32, (nq, 2 * L), 1)
        row = lax.broadcasted_iota(jnp.int32, (nq, 2 * L), 0) + (L - nq)
        seg0 = lane < L
        key = jnp.where(seg0, lane, lane - L)
        allowed = (row < _MEM) | (row >= key)

        st = {}

        def blockdiag(a):
            zero = jnp.zeros_like(a)
            return jnp.concatenate([jnp.where(lo, a, zero), jnp.where(lo, zero, a)],
                                   axis=0).astype(_BF16)

        if len(a_chains) == 1:
            c0 = a_chains[0]
            h32 = jnp.concatenate(
                [ha_ref[_MEM * c0:_MEM * (c0 + 1), :].astype(_F32),
                 ha_ref[(T1, T2)[c0], :].astype(_F32)], axis=0)

        def pre_at(j, p, s):
            if isinstance(s, int):
                return pre_ref.at[j, p, (s - 1) * _SEG:s * _SEG, :]
            return pre_ref.at[j, p, pl.ds(pl.multiple_of((s - 1) * _SEG, _SEG), _SEG), :]

        def proj(p, j):
            w_ref = (wq_ref, wk_ref, wv_ref)[j]
            if first:
                if p == 0 and j < 2:
                    for jj in ((0,), (1, 2))[j]:
                        pair_in(0, jj).wait()
                elif p > 0 and j == 0:
                    for jj in range(3):
                        pair_in(p, jj).wait()
                    if p >= _WO_LAG:
                        pair_in(p - _WO_LAG, 3).wait()
                wt = stage_ref[j, p]
                w_ref[p] = wt.T
                if p == last_pair:
                    return {0: _dot(h32, wt, _NT)}
                res = _dot(h0_ref[...], wt, _NT)
                pre_ref[j, p, 0:NA, :] = res[0:NA].astype(_BF16)
                return {0: res[NA:NA + L]}
            if mode == "ahead":
                res = _dot(h32, w_ref[p])
                pre_at(j, p, t + _AHEAD)[...] = res[_MEM:L].astype(_BF16)
                return {0: jnp.concatenate([res[0:_MEM], pre_at(j, p, t)[...].astype(_F32)], axis=0)}
            if mode == "pre":
                h = jnp.concatenate([ha_ref[0:2 * _MEM, :], ha_ref[T2, :]], axis=0)
                res = _dot(h, w_ref[p])
                return {0: jnp.concatenate([res[0:_MEM], pre_at(j, p, t)[...].astype(_F32)], axis=0),
                        1: res[_MEM:_MEM + L]}
            if both:
                res = _dot(ha_ref[...], w_ref[p])
                return {c: jnp.concatenate([res[_MEM * c:_MEM * (c + 1)], res[(T1, T2)[c]]], axis=0)
                        for c in (0, 1)}
            return {c0: _dot(h32[_MEM:] if final and j == 0 else h32, w_ref[p])}

        def bulk(j):
            wt = stage_ref[j, last_pair]
            pre_ref[j, last_pair, 0:NA, :] = _dot(h0_ref[0:NA, :], wt, _NT).astype(_BF16)

        def a_q(p):
            st["q", p] = proj(p, 0)

        def a_k(p):
            st["k", p] = proj(p, 1)

        def a_v(p):
            st["v", p] = proj(p, 2)

        def a_s(p):
            q, k = st.pop(("q", p)), st.pop(("k", p))
            for c in a_chains:
                s = _dot(q[c], blockdiag(k[c]), _NT) * scale
                s = jnp.where(allowed, s, _NEG)
                m0 = jnp.max(jnp.where(seg0, s, -jnp.inf), axis=1, keepdims=True)
                m1 = jnp.max(jnp.where(seg0, -jnp.inf, s), axis=1, keepdims=True)
                e = jnp.exp(s - jnp.where(seg0, m0, m1))
                l0 = jnp.sum(jnp.where(seg0, e, 0.0), axis=1, keepdims=True)
                l1 = jnp.sum(jnp.where(seg0, 0.0, e), axis=1, keepdims=True)
                st["p", p, c] = e / jnp.where(seg0, l0, l1)

        def a_pv(p):
            v = st.pop(("v", p))
            outs = [_dot(st.pop(("p", p, c)), blockdiag(v[c])) for c in a_chains]
            if both:
                st["o", p] = jnp.concatenate(
                    [outs[0][:_MEM], outs[1][:_MEM], outs[0][_MEM:], outs[1][_MEM:]],
                    axis=0).astype(_BF16)
            else:
                st["o", p] = outs[0]

        def a_o(p):
            if first and p == n_pairs - _WO_LAG:
                for q in range(p, n_pairs):
                    pair_in(q, 3).wait()
            part = _dot(st.pop(("o", p)), wo_ref[p * PW:(p + 1) * PW, :])
            n = part.shape[0]
            if p == 0:
                acc_ref[0:n, :] = part
            elif p < n_pairs - 1:
                acc_ref[0:n, :] += part
            else:
                st["acc"] = acc_ref[0:n, :] + part

        def rs(c):
            return slice(_SEG * c, _SEG * (c + 1))

        def rotate(c):
            htail_ref[8 * c:8 * c + 8, :] = hprev_ref[_SEG * (c + 1) - 8:_SEG * (c + 1), :]
            hprev_ref[rs(c), :] = st.pop(("h", c))
            nprev_ref[rs(c), :] = st.pop(("ncur", c))
            yprev_ref[rs(c), :] = st.pop(("ycur", c))

        def b_1(c):
            ycur = ycur_ref[rs(c), :]
            ncur = _ln(ycur)
            st["ycur", c], st["ncur", c] = ycur, ncur
            st["h", c] = _gelu(_dot(_ln(ncur).astype(_BF16), w1_ref[...]))
            if ("b2", c) not in b_stages:
                rotate(c)

        def b_2(c):
            s = t - 2 - _LAG * c
            hprev = hprev_ref[rs(c), :]
            pt = pick(s == 0, jnp.zeros((8, D), _F32), lambda: htail_ref[8 * c:8 * c + 8, :])
            nh = pick(s == n_seg - 1, jnp.zeros((8, D), _F32), lambda: st["h", c][0:8])
            g = _token_shift(jnp.concatenate([pt, hprev, nh], axis=0))
            st["x1", c] = nprev_ref[rs(c), :] + _dot(g.astype(_BF16), w2_ref[...])
            st["yres", c] = yprev_ref[rs(c), :]
            if ("b1", c) in b_stages:
                rotate(c)

        def b_3(c):
            st["f", c] = _gelu(_dot(_ln(st["x1", c]).astype(_BF16), w3_ref[...])).astype(_BF16)

        def b_4(c):
            ynew = st.pop(("yres", c)) + st.pop(("x1", c)) + _dot(st.pop(("f", c)), w4_ref[...])
            if c == 0:
                st["y2new"] = ynew
                st["tok2"] = _ln(ynew).astype(_BF16)
            else:
                so = t - 2 - _LAG
                if isinstance(so, int):
                    o_ref[so * _SEG:(so + 1) * _SEG, :] = ynew.astype(o_ref.dtype)
                else:
                    o_ref[pl.ds(pl.multiple_of(so * _SEG, _SEG), _SEG), :] = ynew.astype(o_ref.dtype)

        stages = dict(q=a_q, k=a_k, v=a_v, s=a_s, pv=a_pv, o=a_o, bulk=bulk,
                      b1=b_1, b2=b_2, b3=b_3, b4=b_4)
        for name, arg in _schedule(n_pairs, a_chains, b_stages, mode):
            stages[name](arg)

        if "tok2" in st:
            ha_ref[T2, :] = st.pop("tok2")
        if a_chains:
            acc = st.pop("acc")
            if both:
                mem1, mem2 = acc[0:_MEM], acc[_MEM:2 * _MEM]
                a1, a2 = acc[T1], acc[T2]
            elif a_chains == (0,):
                mem1, mem2 = acc[0:_MEM], mem0_ref[...].astype(_F32)
                a1, a2 = acc[_MEM:L], None
            elif final:
                a1, a2 = None, acc
            else:
                mem1, mem2 = mem0_ref[...].astype(_F32), acc[0:_MEM]
                a1, a2 = None, acc[_MEM:L]
            if not final:
                ha_ref[0:2 * _MEM, :] = jnp.concatenate([mem1, mem2], axis=0).astype(_BF16)
            if a1 is not None:
                if isinstance(t, int):
                    nxt = t + 1 + _AHEAD if t + 1 < _LAG else min(t + 1, n_seg - 1)
                else:
                    nxt = jnp.minimum(t + 1, n_seg - 1)
                ha_ref[T1, :] = _ln(xseg(nxt)).astype(_BF16)
                ycur_ref[0:_SEG, :] = xseg(t) + a1
            if a2 is not None:
                ycur_ref[_SEG:, :] = y2res_ref[...] + a2
        if "y2new" in st:
            y2res_ref[...] = st.pop("y2new")
        assert not st, list(st)

    misc["x0"].start()
    misc["mem0"].start()
    for p in range(n_pairs + _WO_LAG):
        for j in range(3):
            if p < n_pairs:
                pair_in(p, j).start()
        if p >= _WO_LAG:
            pair_in(p - _WO_LAG, 3).start()
    for k in ("w1", "w2", "w3", "w4", "x1"):
        misc[k].start()
    for r in (ycur_ref, yprev_ref, nprev_ref, hprev_ref, htail_ref, y2res_ref):
        r[...] = jnp.zeros(r.shape, _F32)
    misc["x0"].wait()
    misc["mem0"].wait()
    mem0 = mem0_ref[...]
    ha_ref[0:2 * _MEM, :] = jnp.concatenate([mem0, mem0], axis=0).astype(_BF16)
    n0 = _ln(xseg(0))
    ha_ref[T1, :] = n0.astype(_BF16)
    ha_ref[T2, :] = jnp.zeros((_SEG, D), _BF16)
    for s in range(1, _AHEAD + 1):
        h0_ref[(s - 1) * _SEG:s * _SEG, :] = _ln(xseg(s))
    h0_ref[NA:NA + L, :] = jnp.concatenate([mem0.astype(_F32), n0], axis=0)

    B = lambda c, which: {(n, c) for n in which}
    ALL = ("b1", "b2", "b3", "b4")

    with _scope("step0"):
        step(0, (0,), set(), "first")

    def own_block(f):
        def body(i, carry):
            f()
            return carry
        lax.fori_loop(0, pl.program_id(0) + 1, body, 0)

    def step1():
        misc["w1"].wait()
        step(1, (0,), B(0, ALL[:1]), "ahead")

    def step2():
        for k in ("w2", "w3", "w4"):
            misc[k].wait()
        step(2, (0,), B(0, ALL), "ahead")

    with _scope("step1"):
        own_block(step1)
    with _scope("step2"):
        own_block(step2)
        misc["x1"].wait()

    def run(lo_t, hi_t, mode):
        def body(t, carry):
            step(t, (0, 1), B(0, ALL) | B(1, ALL), mode)
            return carry
        lax.fori_loop(lo_t, hi_t, body, 0)

    with _scope("loop_pre"):
        step(_LAG, (0, 1), B(0, ALL), "pre")
        step(_LAG + 1, (0, 1), B(0, ALL) | B(1, ALL[:1]), "pre")
        run(_LAG + 2, _LAG + _AHEAD, "pre")
    with _scope("loop"):
        run(_LAG + _AHEAD, n_seg, "norm")

    with _scope("tailA"):
        out_a.start()
        step(n_seg, (1,), B(0, ALL) | B(1, ALL))
        step(n_seg + 1, (1,), B(0, ALL[1:]) | B(1, ALL))
        step(n_seg + 2, (1,), B(1, ALL), final=True)
    with _scope("tailB"):
        C1 = slice(_SEG, 2 * _SEG)
        ycur = ycur_ref[C1, :]
        ncur = _ln(ycur)
        hcur = _gelu(_dot(_ln(ncur).astype(_BF16), w1_ref[...]))
        g = _token_shift(jnp.concatenate(
            [htail_ref[8:16, :], hprev_ref[C1, :], hcur, jnp.zeros((8, D), _F32)], axis=0))
        x1 = jnp.concatenate([nprev_ref[C1, :], ncur], axis=0) + _dot(g.astype(_BF16), w2_ref[...])
        f = _gelu(_dot(_ln(x1).astype(_BF16), w3_ref[...])).astype(_BF16)
        ynew = jnp.concatenate([yprev_ref[C1, :], ycur], axis=0) + x1 + _dot(f, w4_ref[...])
        o_ref[(n_seg - 2) * _SEG:n_seg * _SEG, :] = ynew.astype(o_ref.dtype)
    with _scope("out"):
        out_b.start()
        out_a.wait()
        out_b.wait()


@functools.partial(jax.jit, static_argnames=("A_seg_len",))
def pallas_interleave_layers__memory_aug_recurrent_mem_tr__mixer_s_mlp__prompt_kernel(
    A_x: jax.Array,
    A_mem0: jax.Array,
    A_Wq: jax.Array,
    A_Wk: jax.Array,
    A_Wv: jax.Array,
    A_Wo: jax.Array,
    A_seg_len,
    B_x: jax.Array,
    B_w1: jax.Array,
    B_w2: jax.Array,
    B_w3: jax.Array,
    B_w4: jax.Array,
):
    del B_x
    _, S, D = A_x.shape
    _, H, Dh = A_Wq.shape
    F = B_w3.shape[1]
    assert A_seg_len == _SEG and A_mem0.shape[1] == _MEM and A_x.shape[0] == 1
    n_seg = S // _SEG
    assert n_seg * _SEG == S and n_seg >= 2 * _LAG + 2 + _AHEAD and H % 2 == 0

    def wt(w):
        return jnp.transpose(w, (1, 2, 0)).reshape(H * Dh, D)

    R = 2 * (_MEM + _SEG)
    NP, PW = H // 2, 2 * Dh
    hbm = pl.BlockSpec(memory_space=pl.ANY)
    out = pl.pallas_call(
        functools.partial(_kernel, n_seg=n_seg, n_heads=H, d_head=Dh),
        out_shape=jax.ShapeDtypeStruct((S, D), A_x.dtype),
        grid=(1,),
        in_specs=[hbm] * 10,
        out_specs=hbm,
        scratch_shapes=[
            pltpu.VMEM((S, D), _BF16),
            pltpu.VMEM((_MEM, D), _BF16),
            pltpu.VMEM((NP, D, PW), _BF16),
            pltpu.VMEM((NP, D, PW), _BF16),
            pltpu.VMEM((NP, D, PW), _BF16),
            pltpu.VMEM((H * Dh, D), _BF16),
            pltpu.VMEM((D, D), _BF16),
            pltpu.VMEM((D, D), _BF16),
            pltpu.VMEM((D, F), _BF16),
            pltpu.VMEM((F, D), _BF16),
            pltpu.VMEM((S, D), A_x.dtype),
            pltpu.VMEM((3, NP, PW, D), _BF16),
            pltpu.VMEM((R, D), _BF16),
            pltpu.VMEM((_AHEAD * _SEG + _MEM + _SEG, D), _F32),
            pltpu.VMEM((3, NP, (_AHEAD + _LAG - 1) * _SEG, PW), _BF16),
            pltpu.VMEM((R, D), _F32),
            pltpu.VMEM((2 * _SEG, D), _F32),
            pltpu.VMEM((2 * _SEG, D), _F32),
            pltpu.VMEM((2 * _SEG, D), _F32),
            pltpu.VMEM((2 * _SEG, D), _F32),
            pltpu.VMEM((16, D), _F32),
            pltpu.VMEM((_SEG, D), _F32),
            pltpu.SemaphoreType.DMA((4 * NP + 9,)),
        ],
        compiler_params=pltpu.CompilerParams(
            vmem_limit_bytes=100 * 1024 * 1024,
            flags=_FLAGS),
    )(A_x.reshape(S, D), A_mem0.reshape(_MEM, D), wt(A_Wq), wt(A_Wk), wt(A_Wv),
      A_Wo.reshape(H * Dh, D), B_w1, B_w2, B_w3, B_w4)
    return out.reshape(1, S, D)
```
